```python
import jax
import jax.numpy as jnp

def _softmax(x, axis=-1):
    return jax.nn.softmax(x, axis=axis)
def _gelu(x):
    return jax.nn.gelu(x, approximate=True)
def _silu(x):
    return jax.nn.silu(x)
def _sigmoid(x):
    return jax.nn.sigmoid(x)
def _layernorm(x, axis=-1, eps=1e-5):
    m = jnp.mean(x, axis=axis, keepdims=True)
    v = jnp.var(x, axis=axis, keepdims=True)
    return (x - m) / jnp.sqrt(v + eps)
def _scatter_add(tgt, idx, src, axis=0):
    return tgt.at[idx].add(src)
def _segment_sum(src, seg, n):
    return jax.ops.segment_sum(src, seg, n)
class _Rng:
    def __init__(self, key):
        self._k = key
    def _next(self):
        self._k, sub = jax.random.split(self._k)
        return sub
    def normal(self, shape):
        return jax.random.normal(self._next(), shape, dtype=jnp.bfloat16)
    def randint(self, lo, hi, shape):
        return jax.random.randint(self._next(), shape, lo, hi, dtype=jnp.int32)
    def uniform(self, shape, lo=0.0, hi=1.0):
        return jax.random.uniform(self._next(), shape, jnp.bfloat16, lo, hi)
    def permutation(self, n):
        return jax.random.permutation(self._next(), n)


kernel_name = 'sequential_preLN__compressed_kv_cla__moe_arch_mod__prompt'

def setup_inputs():
    _rng = _Rng(jax.random.key(int.from_bytes(__import__("os").urandom(4), "little")))
    _w = (lambda a: (lambda t: t.astype(jnp.bfloat16) if jnp.issubdtype(t.dtype, jnp.floating) else t)(jnp.asarray(a)))
    def _A_setup():
        B, H, Sq, Sk, D, M = 1, 32, 2048, 2048, 128, 1024
        Dc = 4 * D
        return {
            "x": _w((lambda *s: _rng.normal(s) * 0.05)(B, Sq, M)),
            "c_kv": _w((lambda *s: _rng.normal(s) * 0.05)(B, Sk, Dc)),
            "w_q": _w((lambda *s: _rng.normal(s) * 0.05)(M, H, D) * (M ** -0.5)),
            "w_uk": _w((lambda *s: _rng.normal(s) * 0.05)(Dc, H, D) * (Dc ** -0.5)),
            "w_uv": _w((lambda *s: _rng.normal(s) * 0.05)(Dc, H, D) * (Dc ** -0.5)),
            "w_o": _w((lambda *s: _rng.normal(s) * 0.05)(H, D, M) * ((H * D) ** -0.5)),
        }
    _A_in = _A_setup()

    def _B_setup():
        B, S, D, F, C = 1, 2048, 1024, 3584, 2
        return {
            "x": _w((lambda *s: _rng.normal(s) * 0.05)(B, S, D)),
            "w_r": _w((lambda *s: _rng.normal(s) * 0.05)(D)),
            "w_gate": _w((lambda *s: _rng.normal(s) * 0.05)(D, F)),
            "w_up": _w((lambda *s: _rng.normal(s) * 0.05)(D, F)),
            "w_down": _w((lambda *s: _rng.normal(s) * 0.05)(F, D)),
        }
    _B_in = _B_setup()

    return {
        "A_x": _A_in["x"],
        "A_c_kv": _A_in["c_kv"],
        "A_w_q": _A_in["w_q"],
        "A_w_uk": _A_in["w_uk"],
        "A_w_uv": _A_in["w_uv"],
        "A_w_o": _A_in["w_o"],
        "B_x": _B_in["x"],
        "B_w_r": _B_in["w_r"],
        "B_w_gate": _B_in["w_gate"],
        "B_w_up": _B_in["w_up"],
        "B_w_down": _B_in["w_down"],
    }

def reference(A_x, A_c_kv, A_w_q, A_w_uk, A_w_uv, A_w_o, B_x, B_w_r, B_w_gate, B_w_up, B_w_down):
    def _A_ref(x, c_kv, w_q, w_uk, w_uv, w_o):
        B, Sq, M = x.shape[0], x.shape[1], x.shape[2]
        Sk = c_kv.shape[1]
        H, D = w_q.shape[1], w_q.shape[2]
        q = jnp.einsum("bqm,mhd->bhqd", x, w_q)
        k = jnp.einsum("bkc,chd->bhkd", c_kv, w_uk)
        v = jnp.einsum("bkc,chd->bhkd", c_kv, w_uv)
        scores = jnp.einsum("bhqd,bhkd->bhqk", q, k) * (D ** -0.5)
        off = Sk - Sq
        qi = jnp.arange(Sq)[:, None]
        kj = jnp.arange(Sk)[None, :]
        cmask = kj <= (qi + off)
        scores = jnp.where(cmask[None, None], scores, -1e9)
        p = _softmax(scores, axis=-1)
        ctx = jnp.einsum("bhqk,bhkd->bhqd", p, v)
        return jnp.einsum("bhqd,hdm->bqm", ctx, w_o)

    def _B_ref(x, w_r, w_gate, w_up, w_down):
        B, S, D = x.shape
        C = 2
        r = x @ w_r
        idx = jnp.argsort(-r, axis=-1)[:, :C]
        idx_e = jnp.repeat(idx.reshape(B, C, 1), D, axis=2)
        x_sel = jnp.take_along_axis(x, idx_e, axis=1)
        g = _silu(x_sel @ w_gate)
        u = x_sel @ w_up
        y = (g * u) @ w_down
        r_sel = _sigmoid(jnp.take_along_axis(r, idx, axis=1))
        y = y * r_sel.reshape(B, C, 1)
        b_off = (jnp.arange(B) * S).reshape(B, 1)
        flat_idx = (idx + b_off).reshape(B * C)
        zero = (x * 0.0).reshape(B * S, D)
        upd = _scatter_add(zero, flat_idx, y.reshape(B * C, D), axis=0)
        return x + upd.reshape(B, S, D)

    x = A_x
    h = x + _A_ref(_layernorm(x, axis=-1), A_c_kv, A_w_q, A_w_uk, A_w_uv, A_w_o)
    h2 = h + _B_ref(_layernorm(h, axis=-1), B_w_r, B_w_gate, B_w_up, B_w_down)
    return h2
```

```python
import functools
import math

import jax
import jax.numpy as jnp
from jax import lax
import jax.experimental.pallas as pl
import jax.experimental.pallas.tpu as pltpu

F32 = jnp.float32
BF16 = jnp.bfloat16
NEG = -1e30
NT = (((1,), (1,)), ((), ()))
TQ = 512
SUB = 128
GRP = 4


def _rb(v):
    return v.astype(BF16).astype(F32)


def _unpack_pair(w32):
    lo = pltpu.bitcast(w32 << 16, F32)
    hi = pltpu.bitcast(w32 & jnp.uint32(0xFFFF0000), F32)
    return jnp.concatenate([lo, hi], axis=1).astype(BF16)


def _qk(q, k, i):
    r0 = i * TQ
    nb = TQ // SUB
    qb = q[r0:r0 + TQ, :]
    s_main = lax.dot_general(qb, k[0:r0 + SUB, :], NT, preferred_element_type=F32)
    s_ext = [lax.dot_general(qb[c * SUB:, :], k[r0 + c * SUB:r0 + (c + 1) * SUB, :], NT,
                             preferred_element_type=F32) for c in range(1, nb)]
    return s_main, s_ext


def _softmax(s, i):
    s_main, s_ext = s
    r0 = i * TQ
    nb = TQ // SUB
    row = lax.broadcasted_iota(jnp.int32, (SUB, SUB), 0)
    col = lax.broadcasted_iota(jnp.int32, (SUB, SUB), 1)
    tri = col <= row
    p_main, p_ext, ls = [], [[] for _ in range(1, nb)], []
    for b in range(nb):
        sm = s_main[b * SUB:(b + 1) * SUB, :]
        if b == 0:
            d = jnp.where(tri, sm[:, r0:], NEG)
            sm = jnp.concatenate([sm[:, :r0], d], axis=1) if r0 > 0 else d
        parts = [sm]
        for c in range(1, b + 1):
            e = s_ext[c - 1][(b - c) * SUB:(b - c + 1) * SUB, :]
            if c == b:
                e = jnp.where(tri, e, NEG)
            parts.append(e)
        sb = jnp.concatenate(parts, axis=1) if len(parts) > 1 else parts[0]
        m = jnp.max(sb, axis=1, keepdims=True)
        p = jnp.exp2(sb - m)
        nt = p.shape[1] // SUB
        tiles = [p[:, t * SUB:(t + 1) * SUB] for t in range(nt)]
        acc = None
        for t0 in range(0, nt, GRP):
            grp = tiles[t0:t0 + GRP]
            tot = grp[0]
            for g in grp[1:]:
                tot = tot + g
            acc = tot if acc is None else acc + tot
            last = t0 + len(grp) - 1
            if acc is not tiles[last]:
                tiles[last] = jnp.minimum(tiles[last], acc)
        p = jnp.concatenate(tiles, axis=1) if nt > 1 else tiles[0]
        ls.append(jnp.sum(acc, axis=1, keepdims=True))
        p_main.append(p[:, :r0 + SUB])
        for c in range(1, b + 1):
            p_ext[c - 1].append(p[:, r0 + c * SUB:r0 + (c + 1) * SUB])
    pm = jnp.concatenate(p_main, axis=0).astype(BF16)
    pe = [(jnp.concatenate(e, axis=0) if len(e) > 1 else e[0]).astype(BF16) for e in p_ext]
    return pm, pe, ls


def _pv(p, v, i):
    pm, pe, ls = p
    r0 = i * TQ
    nb = TQ // SUB
    o = jnp.dot(pm, v[0:r0 + SUB, :], preferred_element_type=F32)
    os_ = [o[b * SUB:(b + 1) * SUB] for b in range(nb)]
    for c in range(1, nb):
        oe = jnp.dot(pe[c - 1], v[r0 + c * SUB:r0 + (c + 1) * SUB, :], preferred_element_type=F32)
        for b in range(c, nb):
            os_[b] = os_[b] + oe[(b - c) * SUB:(b - c + 1) * SUB]
    return jnp.concatenate([os_[b] / ls[b] for b in range(nb)], axis=0)


def _kernel(x_ref, c_ref, wq_hbm, wk_hbm, wv_hbm, wo_ref, wr_ref, wg_hbm, wu_hbm, wd_hbm,
            out_ref,
            xn_s, acc_s, ln_s, r_s, wq_b, wk_b, wv_b, wg_v, wu_v, wd_v, wsem, fsem,
            *, S, M, D, NP):
    j = pl.program_id(0)
    slot = j % 2

    def wcopies(jj, sl):
        return [
            pltpu.make_async_copy(wk_hbm.bitcast(jnp.uint32).at[:, jj, :], wk_b.at[sl], wsem.at[0, sl]),
            pltpu.make_async_copy(wv_hbm.bitcast(jnp.uint32).at[:, jj, :], wv_b.at[sl], wsem.at[1, sl]),
            pltpu.make_async_copy(wq_hbm.bitcast(jnp.uint32).at[:, jj, :], wq_b.at[sl], wsem.at[2, sl]),
        ]

    def fcopies():
        return [
            pltpu.make_async_copy(wg_hbm, wg_v, fsem.at[0]),
            pltpu.make_async_copy(wu_hbm, wu_v, fsem.at[1]),
            pltpu.make_async_copy(wd_hbm, wd_v, fsem.at[2]),
        ]

    @pl.when(j == 0)
    def _():
        for cp in wcopies(0, 0):
            cp.start()
        RB = 128

        def ln1(b, carry):
            rows = pl.ds(pl.multiple_of(b * RB, RB), RB)
            xf = x_ref[0, rows, :].astype(F32)
            mu = jnp.mean(xf, axis=1, keepdims=True)
            xc = xf - mu
            var = jnp.mean(xc * xc, axis=1, keepdims=True)
            xn_s[rows, :] = (xc * lax.rsqrt(var + 1e-5)).astype(BF16)
            acc_s[rows, :] = jnp.zeros((RB, M), F32)
            return carry
        lax.fori_loop(0, S // RB, ln1, 0)

    @pl.when(j == 1)
    def _():
        for cp in fcopies():
            cp.start()

    @pl.when(j + 1 < NP)
    def _():
        for cp in wcopies(j + 1, 1 - slot):
            cp.start()

    for cp in wcopies(j, slot):
        cp.wait()

    scale = (D ** -0.5) * math.log2(math.e)
    c = c_ref[0]
    kp = jnp.dot(c, _unpack_pair(wk_b[slot]), preferred_element_type=F32).astype(BF16)
    qp = (jnp.dot(xn_s[...], _unpack_pair(wq_b[slot]), preferred_element_type=F32) * scale).astype(BF16)
    vp = jnp.dot(c, _unpack_pair(wv_b[slot]), preferred_element_type=F32).astype(BF16)
    wo = wo_ref[...].reshape(2 * D, M)

    qs = [qp[:, :D], qp[:, D:]]
    ks = [kp[:, :D], kp[:, D:]]
    vs = [vp[:, :D], vp[:, D:]]
    nq = S // TQ
    jobs = [(h, i) for i in range(nq - 1, -1, -1) for h in range(2)]
    s_next = _qk(qs[jobs[0][0]], ks[jobs[0][0]], jobs[0][1])
    ctx = {}
    pending = None
    for t, (h, i) in enumerate(jobs):
        s_cur = s_next
        if t + 1 < len(jobs):
            h2, i2 = jobs[t + 1]
            s_next = _qk(qs[h2], ks[h2], i2)
        if pending is not None:
            ii = pending
            cpair = jnp.concatenate([ctx[(0, ii)], ctx[(1, ii)]], axis=1).astype(BF16)
            acc_s[ii * TQ:(ii + 1) * TQ, :] += jnp.dot(cpair, wo, preferred_element_type=F32)
            pending = None
        p = _softmax(s_cur, i)
        ctx[(h, i)] = _pv(p, vs[h], i)
        if h == 1:
            pending = i
    ii = pending
    cpair = jnp.concatenate([ctx[(0, ii)], ctx[(1, ii)]], axis=1).astype(BF16)
    acc_s[ii * TQ:(ii + 1) * TQ, :] += jnp.dot(cpair, wo, preferred_element_type=F32)

    @pl.when(j == NP - 1)
    def _():
        RB = 128
        wr = wr_ref[...].astype(F32)
        eps = jnp.asarray(1e-5, BF16).astype(F32)

        def ln2(b, carry):
            rows = pl.ds(pl.multiple_of(b * RB, RB), RB)
            hf = _rb(x_ref[0, rows, :].astype(F32) + _rb(acc_s[rows, :]))
            mu = jnp.mean(hf, axis=1, keepdims=True)
            hc = hf - mu
            var = jnp.mean(hc * hc, axis=1, keepdims=True)
            den = _rb(jnp.sqrt(_rb(_rb(var) + eps)))
            ln = _rb(_rb(hf - _rb(mu)) / den)
            r_s[rows, :] = _rb(jnp.sum(ln * wr, axis=1, keepdims=True))
            ln_s[rows, :] = ln
            acc_s[rows, :] = hf
            out_ref[0, rows, :] = (hf + ln).astype(BF16)
            return carry
        lax.fori_loop(0, S // RB, ln2, 0)

        r = r_s[...]
        idx = lax.broadcasted_iota(jnp.int32, (S, 1), 0)
        m1 = jnp.max(r)
        i1 = jnp.min(jnp.where(r == m1, idx, S))
        r2 = jnp.where(idx == i1, -jnp.inf, r)
        m2 = jnp.max(r2)
        i2 = jnp.min(jnp.where(r2 == m2, idx, S))
        i1 = jnp.clip(i1, 0, S - 1)
        i2 = jnp.clip(i2, 0, S - 1)

        for cp in fcopies():
            cp.wait()
        x1 = ln_s[pl.ds(i1, 1), :]
        x2 = ln_s[pl.ds(i2, 1), :]
        rid = lax.broadcasted_iota(jnp.int32, (16, M), 0)
        xs = jnp.where(rid == 0, x1, x2)
        xsb = xs.astype(BF16)
        a = _rb(jnp.dot(xsb, wg_v[...], preferred_element_type=F32))
        u = _rb(jnp.dot(xsb, wu_v[...], preferred_element_type=F32))
        g = _rb(a * _rb(jax.nn.sigmoid(a)))
        y = _rb(jnp.dot((g * u).astype(BF16), wd_v[...], preferred_element_type=F32))
        rsel = jnp.where(rid == 0, m1, m2)
        y = _rb(y * _rb(jax.nn.sigmoid(rsel)))
        upd = _rb(xs + y)
        for (ii, rr) in ((i1, 0), (i2, 1)):
            base = pl.multiple_of((ii // 16) * 16, 16)
            hrow = acc_s[pl.ds(ii, 1), :]
            new = hrow + upd[rr:rr + 1, :]
            cur = out_ref[0, pl.ds(base, 16), :].astype(F32)
            out_ref[0, pl.ds(base, 16), :] = jnp.where(rid == ii - base, new, cur).astype(BF16)


@jax.jit
def pallas_sequential_preLN__compressed_kv_cla__moe_arch_mod__prompt_kernel(
    A_x: jax.Array,
    A_c_kv: jax.Array,
    A_w_q: jax.Array,
    A_w_uk: jax.Array,
    A_w_uv: jax.Array,
    A_w_o: jax.Array,
    B_x: jax.Array,
    B_w_r: jax.Array,
    B_w_gate: jax.Array,
    B_w_up: jax.Array,
    B_w_down: jax.Array,
):
    _, S, M = A_x.shape
    C = A_c_kv.shape[2]
    H, D = A_w_q.shape[1], A_w_q.shape[2]
    FF = B_w_gate.shape[1]
    NP = H // 2
    any_spec = pl.BlockSpec(memory_space=pl.ANY)
    one = pl.Buffered(1)
    return pl.pallas_call(
        functools.partial(_kernel, S=S, M=M, D=D, NP=NP),
        grid=(NP,),
        in_specs=[
            pl.BlockSpec((1, S, M), lambda j: (0, 0, 0), pipeline_mode=one),
            pl.BlockSpec((1, S, C), lambda j: (0, 0, 0), pipeline_mode=one),
            any_spec, any_spec, any_spec,
            pl.BlockSpec((2, D, M), lambda j: (j, 0, 0)),
            pl.BlockSpec((1, M), lambda j: (0, 0)),
            any_spec, any_spec, any_spec,
        ],
        out_specs=pl.BlockSpec((1, S, M), lambda j: (0, 0, 0)),
        out_shape=jax.ShapeDtypeStruct((1, S, M), BF16),
        scratch_shapes=[
            pltpu.VMEM((S, M), BF16),
            pltpu.VMEM((S, M), F32),
            pltpu.VMEM((S, M), F32),
            pltpu.VMEM((S, 1), F32),
            pltpu.VMEM((2, M, D), jnp.uint32),
            pltpu.VMEM((2, C, D), jnp.uint32),
            pltpu.VMEM((2, C, D), jnp.uint32),
            pltpu.VMEM((M, FF), BF16),
            pltpu.VMEM((M, FF), BF16),
            pltpu.VMEM((FF, M), BF16),
            pltpu.SemaphoreType.DMA((3, 2)),
            pltpu.SemaphoreType.DMA((3,)),
        ],
        compiler_params=pltpu.CompilerParams(
            dimension_semantics=("arbitrary",),
            vmem_limit_bytes=110 * 1024 * 1024,
        ),
    )(A_x, A_c_kv, A_w_q, A_w_uk, A_w_uv, A_w_o, B_w_r.reshape(1, M), B_w_gate, B_w_up, B_w_down)
```

```python
import functools
import math

import jax
import jax.numpy as jnp
from jax import lax
import jax.experimental.pallas as pl
import jax.experimental.pallas.tpu as pltpu

F32 = jnp.float32
BF16 = jnp.bfloat16
NEG = -1e30
NT = (((1,), (1,)), ((), ()))
TQ = 512
SUB = 128
GRP = 4
ODELAY = 3


def _rb(v):
    return v.astype(BF16).astype(F32)


def _recip(l):
    r = pl.reciprocal(l, approx=True)
    return r * (2.0 - l * r)


def _unpack_pair(w32):
    lo = pltpu.bitcast(w32 << 16, F32)
    hi = pltpu.bitcast(w32 & jnp.uint32(0xFFFF0000), F32)
    return jnp.concatenate([lo, hi], axis=1).astype(BF16)


def _qk(q, k, i):
    r0 = i * TQ
    nb = TQ // SUB
    qb = q[r0:r0 + TQ, :]
    s_main = lax.dot_general(qb, k[0:r0 + SUB, :], NT, preferred_element_type=F32)
    s_ext = [lax.dot_general(qb[c * SUB:, :], k[r0 + c * SUB:r0 + (c + 1) * SUB, :], NT,
                             preferred_element_type=F32) for c in range(1, nb)]
    return s_main, s_ext


def _softmax(s, i):
    s_main, s_ext = s
    r0 = i * TQ
    nb = TQ // SUB
    row = lax.broadcasted_iota(jnp.int32, (SUB, SUB), 0)
    col = lax.broadcasted_iota(jnp.int32, (SUB, SUB), 1)
    tri = col <= row
    p_main, p_ext, ls = [], [[] for _ in range(1, nb)], []
    for b in range(nb):
        sm = s_main[b * SUB:(b + 1) * SUB, :]
        if b == 0:
            d = jnp.where(tri, sm[:, r0:], NEG)
            sm = jnp.concatenate([sm[:, :r0], d], axis=1) if r0 > 0 else d
        parts = [sm]
        for c in range(1, b + 1):
            e = s_ext[c - 1][(b - c) * SUB:(b - c + 1) * SUB, :]
            if c == b:
                e = jnp.where(tri, e, NEG)
            parts.append(e)
        sb = jnp.concatenate(parts, axis=1) if len(parts) > 1 else parts[0]
        m = jnp.max(sb, axis=1, keepdims=True)
        p = jnp.exp2(sb - m)
        nt = p.shape[1] // SUB
        tiles = [p[:, t * SUB:(t + 1) * SUB] for t in range(nt)]
        acc = None
        for t0 in range(0, nt, GRP):
            grp = tiles[t0:t0 + GRP]
            tot = grp[0]
            for g in grp[1:]:
                tot = tot + g
            acc = tot if acc is None else acc + tot
            last = t0 + len(grp) - 1
            if acc is not tiles[last]:
                tiles[last] = jnp.minimum(tiles[last], acc)
        p = jnp.concatenate(tiles, axis=1) if nt > 1 else tiles[0]
        ls.append(jnp.sum(acc, axis=1, keepdims=True))
        p_main.append(p[:, :r0 + SUB])
        for c in range(1, b + 1):
            p_ext[c - 1].append(p[:, r0 + c * SUB:r0 + (c + 1) * SUB])
    pm = jnp.concatenate(p_main, axis=0).astype(BF16)
    pe = [(jnp.concatenate(e, axis=0) if len(e) > 1 else e[0]).astype(BF16) for e in p_ext]
    return pm, pe, ls


def _pv(p, v, i):
    pm, pe, ls = p
    r0 = i * TQ
    nb = TQ // SUB
    o = jnp.dot(pm, v[0:r0 + SUB, :], preferred_element_type=F32)
    os_ = [o[b * SUB:(b + 1) * SUB] for b in range(nb)]
    for c in range(1, nb):
        oe = jnp.dot(pe[c - 1], v[r0 + c * SUB:r0 + (c + 1) * SUB, :], preferred_element_type=F32)
        for b in range(c, nb):
            os_[b] = os_[b] + oe[(b - c) * SUB:(b - c + 1) * SUB]
    return jnp.concatenate([os_[b] * _recip(ls[b]) for b in range(nb)], axis=0)


def _kernel(x_ref, c_ref, wq_hbm, wk_hbm, wv_hbm, wo_ref, wr_ref, wg_hbm, wu_hbm, wd_hbm,
            out_ref,
            xn_s, acc_s, ln_s, r_s, wq_b, wk_b, wv_b, wg_v, wu_v, wd_v, wsem, fsem,
            *, S, M, D, NP):
    j = pl.program_id(0)
    slot = j % 2

    def wcopies(jj, sl):
        return [
            pltpu.make_async_copy(wk_hbm.bitcast(jnp.uint32).at[:, jj, :], wk_b.at[sl], wsem.at[0, sl]),
            pltpu.make_async_copy(wv_hbm.bitcast(jnp.uint32).at[:, jj, :], wv_b.at[sl], wsem.at[1, sl]),
            pltpu.make_async_copy(wq_hbm.bitcast(jnp.uint32).at[:, jj, :], wq_b.at[sl], wsem.at[2, sl]),
        ]

    def fcopies():
        return [
            pltpu.make_async_copy(wg_hbm, wg_v, fsem.at[0]),
            pltpu.make_async_copy(wu_hbm, wu_v, fsem.at[1]),
            pltpu.make_async_copy(wd_hbm, wd_v, fsem.at[2]),
        ]

    @pl.when(j == 0)
    def _():
        for cp in wcopies(0, 0):
            cp.start()
        RB = 128

        def ln1(b, carry):
            rows = pl.ds(pl.multiple_of(b * RB, RB), RB)
            xf = x_ref[0, rows, :].astype(F32)
            mu = jnp.mean(xf, axis=1, keepdims=True)
            xc = xf - mu
            var = jnp.mean(xc * xc, axis=1, keepdims=True)
            xn_s[rows, :] = (xc * lax.rsqrt(var + 1e-5)).astype(BF16)
            acc_s[rows, :] = jnp.zeros((RB, M), F32)
            return carry
        lax.fori_loop(0, S // RB, ln1, 0)

    @pl.when(j == 1)
    def _():
        for cp in fcopies():
            cp.start()

    @pl.when(j + 1 < NP)
    def _():
        for cp in wcopies(j + 1, 1 - slot):
            cp.start()

    for cp in wcopies(j, slot):
        cp.wait()

    scale = (D ** -0.5) * math.log2(math.e)
    c = c_ref[0]
    kp = jnp.dot(c, _unpack_pair(wk_b[slot]), preferred_element_type=F32).astype(BF16)
    qp = (jnp.dot(xn_s[...], _unpack_pair(wq_b[slot]), preferred_element_type=F32) * scale).astype(BF16)
    vp = jnp.dot(c, _unpack_pair(wv_b[slot]), preferred_element_type=F32).astype(BF16)
    wo = wo_ref[...].reshape(2 * D, M)

    qs = [qp[:, :D], qp[:, D:]]
    ks = [kp[:, :D], kp[:, D:]]
    vs = [vp[:, :D], vp[:, D:]]
    nq = S // TQ
    jobs = [(h, i) for i in range(nq - 1, -1, -1) for h in range(2)]
    ctx = {}

    def oproj(ii):
        cpair = jnp.concatenate([ctx[(0, ii)], ctx[(1, ii)]], axis=1).astype(BF16)
        acc_s[ii * TQ:(ii + 1) * TQ, :] += jnp.dot(cpair, wo, preferred_element_type=F32)

    s_next = _qk(qs[jobs[0][0]], ks[jobs[0][0]], jobs[0][1])
    pending = []
    for t, (h, i) in enumerate(jobs):
        s_cur = s_next
        if t + 1 < len(jobs):
            h2, i2 = jobs[t + 1]
            s_next = _qk(qs[h2], ks[h2], i2)
        while pending and pending[0][1] + ODELAY <= t:
            oproj(pending.pop(0)[0])
        p = _softmax(s_cur, i)
        ctx[(h, i)] = _pv(p, vs[h], i)
        if h == 1:
            pending.append((i, t))
    for ii, _ in pending:
        oproj(ii)

    @pl.when(j == NP - 1)
    def _():
        RB = 128
        wr = wr_ref[...].astype(F32)
        eps = jnp.asarray(1e-5, BF16).astype(F32)

        def ln2(b, carry):
            rows = pl.ds(pl.multiple_of(b * RB, RB), RB)
            hf = _rb(x_ref[0, rows, :].astype(F32) + _rb(acc_s[rows, :]))
            mu = jnp.mean(hf, axis=1, keepdims=True)
            hc = hf - mu
            var = jnp.mean(hc * hc, axis=1, keepdims=True)
            den = _rb(jnp.sqrt(_rb(_rb(var) + eps)))
            ln = _rb(_rb(hf - _rb(mu)) / den)
            r_s[rows, :] = _rb(jnp.sum(ln * wr, axis=1, keepdims=True))
            ln_s[rows, :] = ln
            acc_s[rows, :] = hf
            out_ref[0, rows, :] = (hf + ln).astype(BF16)
            return carry
        lax.fori_loop(0, S // RB, ln2, 0)

        r = r_s[...]
        idx = lax.broadcasted_iota(jnp.int32, (S, 1), 0)
        m1 = jnp.max(r)
        i1 = jnp.min(jnp.where(r == m1, idx, S))
        r2 = jnp.where(idx == i1, -jnp.inf, r)
        m2 = jnp.max(r2)
        i2 = jnp.min(jnp.where(r2 == m2, idx, S))
        i1 = jnp.clip(i1, 0, S - 1)
        i2 = jnp.clip(i2, 0, S - 1)

        for cp in fcopies():
            cp.wait()
        x1 = ln_s[pl.ds(i1, 1), :]
        x2 = ln_s[pl.ds(i2, 1), :]
        rid = lax.broadcasted_iota(jnp.int32, (16, M), 0)
        xs = jnp.where(rid == 0, x1, x2)
        xsb = xs.astype(BF16)
        a = _rb(jnp.dot(xsb, wg_v[...], preferred_element_type=F32))
        u = _rb(jnp.dot(xsb, wu_v[...], preferred_element_type=F32))
        g = _rb(a * _rb(jax.nn.sigmoid(a)))
        y = _rb(jnp.dot((g * u).astype(BF16), wd_v[...], preferred_element_type=F32))
        rsel = jnp.where(rid == 0, m1, m2)
        y = _rb(y * _rb(jax.nn.sigmoid(rsel)))
        upd = _rb(xs + y)
        for (ii, rr) in ((i1, 0), (i2, 1)):
            base = pl.multiple_of((ii // 16) * 16, 16)
            hrow = acc_s[pl.ds(ii, 1), :]
            new = hrow + upd[rr:rr + 1, :]
            cur = out_ref[0, pl.ds(base, 16), :].astype(F32)
            out_ref[0, pl.ds(base, 16), :] = jnp.where(rid == ii - base, new, cur).astype(BF16)


@jax.jit
def pallas_sequential_preLN__compressed_kv_cla__moe_arch_mod__prompt_kernel(
    A_x: jax.Array,
    A_c_kv: jax.Array,
    A_w_q: jax.Array,
    A_w_uk: jax.Array,
    A_w_uv: jax.Array,
    A_w_o: jax.Array,
    B_x: jax.Array,
    B_w_r: jax.Array,
    B_w_gate: jax.Array,
    B_w_up: jax.Array,
    B_w_down: jax.Array,
):
    _, S, M = A_x.shape
    C = A_c_kv.shape[2]
    H, D = A_w_q.shape[1], A_w_q.shape[2]
    FF = B_w_gate.shape[1]
    NP = H // 2
    any_spec = pl.BlockSpec(memory_space=pl.ANY)
    one = pl.Buffered(1)
    return pl.pallas_call(
        functools.partial(_kernel, S=S, M=M, D=D, NP=NP),
        grid=(NP,),
        in_specs=[
            pl.BlockSpec((1, S, M), lambda j: (0, 0, 0), pipeline_mode=one),
            pl.BlockSpec((1, S, C), lambda j: (0, 0, 0), pipeline_mode=one),
            any_spec, any_spec, any_spec,
            pl.BlockSpec((2, D, M), lambda j: (j, 0, 0)),
            pl.BlockSpec((1, M), lambda j: (0, 0)),
            any_spec, any_spec, any_spec,
        ],
        out_specs=pl.BlockSpec((1, S, M), lambda j: (0, 0, 0)),
        out_shape=jax.ShapeDtypeStruct((1, S, M), BF16),
        scratch_shapes=[
            pltpu.VMEM((S, M), BF16),
            pltpu.VMEM((S, M), F32),
            pltpu.VMEM((S, M), F32),
            pltpu.VMEM((S, 1), F32),
            pltpu.VMEM((2, M, D), jnp.uint32),
            pltpu.VMEM((2, C, D), jnp.uint32),
            pltpu.VMEM((2, C, D), jnp.uint32),
            pltpu.VMEM((M, FF), BF16),
            pltpu.VMEM((M, FF), BF16),
            pltpu.VMEM((FF, M), BF16),
            pltpu.SemaphoreType.DMA((3, 2)),
            pltpu.SemaphoreType.DMA((3,)),
        ],
        compiler_params=pltpu.CompilerParams(
            dimension_semantics=("arbitrary",),
            vmem_limit_bytes=110 * 1024 * 1024,
        ),
    )(A_x, A_c_kv, A_w_q, A_w_uk, A_w_uv, A_w_o, B_w_r.reshape(1, M), B_w_gate, B_w_up, B_w_down)
```

```python
import functools
import math

import jax
import jax.numpy as jnp
from jax import lax
import jax.experimental.pallas as pl
import jax.experimental.pallas.tpu as pltpu

F32 = jnp.float32
BF16 = jnp.bfloat16
NEG = -1e30
NT = (((1,), (1,)), ((), ()))
TQ = 512
SUB = 128
GRP = 4
ODELAY = 3
XB = 256
OB = 512
FC = 512


def _rb(v):
    return v.astype(BF16).astype(F32)


def _recip(l):
    r = pl.reciprocal(l, approx=True)
    return r * (2.0 - l * r)


def _unpack_pair(w32):
    lo = pltpu.bitcast(w32 << 16, F32)
    hi = pltpu.bitcast(w32 & jnp.uint32(0xFFFF0000), F32)
    return jnp.concatenate([lo, hi], axis=1).astype(BF16)


def _qk(q, k, i):
    r0 = i * TQ
    nb = TQ // SUB
    qb = q[r0:r0 + TQ, :]
    s_main = lax.dot_general(qb, k[0:r0 + SUB, :], NT, preferred_element_type=F32)
    s_ext = [lax.dot_general(qb[c * SUB:, :], k[r0 + c * SUB:r0 + (c + 1) * SUB, :], NT,
                             preferred_element_type=F32) for c in range(1, nb)]
    return s_main, s_ext


def _softmax(s, i):
    s_main, s_ext = s
    r0 = i * TQ
    nb = TQ // SUB
    row = lax.broadcasted_iota(jnp.int32, (SUB, SUB), 0)
    col = lax.broadcasted_iota(jnp.int32, (SUB, SUB), 1)
    tri = col <= row
    p_main, p_ext, ls = [], [[] for _ in range(1, nb)], []
    for b in range(nb):
        sm = s_main[b * SUB:(b + 1) * SUB, :]
        if b == 0:
            d = jnp.where(tri, sm[:, r0:], NEG)
            sm = jnp.concatenate([sm[:, :r0], d], axis=1) if r0 > 0 else d
        parts = [sm]
        for c in range(1, b + 1):
            e = s_ext[c - 1][(b - c) * SUB:(b - c + 1) * SUB, :]
            if c == b:
                e = jnp.where(tri, e, NEG)
            parts.append(e)
        sb = jnp.concatenate(parts, axis=1) if len(parts) > 1 else parts[0]
        m = jnp.max(sb, axis=1, keepdims=True)
        p = jnp.exp2(sb - m)
        nt = p.shape[1] // SUB
        tiles = [p[:, t * SUB:(t + 1) * SUB] for t in range(nt)]
        acc = None
        for t0 in range(0, nt, GRP):
            grp = tiles[t0:t0 + GRP]
            tot = grp[0]
            for g in grp[1:]:
                tot = tot + g
            acc = tot if acc is None else acc + tot
            last = t0 + len(grp) - 1
            if acc is not tiles[last]:
                tiles[last] = jnp.minimum(tiles[last], acc)
        p = jnp.concatenate(tiles, axis=1) if nt > 1 else tiles[0]
        ls.append(jnp.sum(acc, axis=1, keepdims=True))
        p_main.append(p[:, :r0 + SUB])
        for c in range(1, b + 1):
            p_ext[c - 1].append(p[:, r0 + c * SUB:r0 + (c + 1) * SUB])
    pm = jnp.concatenate(p_main, axis=0).astype(BF16)
    pe = [(jnp.concatenate(e, axis=0) if len(e) > 1 else e[0]).astype(BF16) for e in p_ext]
    return pm, pe, ls


def _pv(p, v, i):
    pm, pe, ls = p
    r0 = i * TQ
    nb = TQ // SUB
    o = jnp.dot(pm, v[0:r0 + SUB, :], preferred_element_type=F32)
    os_ = [o[b * SUB:(b + 1) * SUB] for b in range(nb)]
    for c in range(1, nb):
        oe = jnp.dot(pe[c - 1], v[r0 + c * SUB:r0 + (c + 1) * SUB, :], preferred_element_type=F32)
        for b in range(c, nb):
            os_[b] = os_[b] + oe[(b - c) * SUB:(b - c + 1) * SUB]
    return jnp.concatenate([os_[b] * _recip(ls[b]) for b in range(nb)], axis=0)


def _attn_pair(qp, kp, vp, wo, acc_s, S, D):
    qs = [qp[:, :D], qp[:, D:]]
    ks = [kp[:, :D], kp[:, D:]]
    vs = [vp[:, :D], vp[:, D:]]
    nq = S // TQ
    jobs = [(h, i) for i in range(nq - 1, -1, -1) for h in range(2)]
    ctx = {}

    def oproj(ii):
        cpair = jnp.concatenate([ctx[(0, ii)], ctx[(1, ii)]], axis=1).astype(BF16)
        acc_s[ii * TQ:(ii + 1) * TQ, :] += jnp.dot(cpair, wo, preferred_element_type=F32)

    s_next = _qk(qs[jobs[0][0]], ks[jobs[0][0]], jobs[0][1])
    pending = []
    for t, (h, i) in enumerate(jobs):
        s_cur = s_next
        if t + 1 < len(jobs):
            h2, i2 = jobs[t + 1]
            s_next = _qk(qs[h2], ks[h2], i2)
        while pending and pending[0][1] + ODELAY <= t:
            oproj(pending.pop(0)[0])
        p = _softmax(s_cur, i)
        ctx[(h, i)] = _pv(p, vs[h], i)
        if h == 1:
            pending.append((i, t))
    for ii, _ in pending:
        oproj(ii)


def _kernel(x_hbm, c_hbm, wq_hbm, wk_hbm, wv_hbm, wo_hbm, wr_ref, wg_hbm, wu_hbm, wd_hbm,
            out_hbm,
            io_v, c_v, xn_s, acc_s, r_s, wq_b, wk_b, wv_b, wo_b, wg_v, wu_v, wd_v,
            xsem, csem, wsem, fsem, osem,
            *, S, M, D, NP, FF):
    U32 = jnp.uint32

    def xcopy(b):
        rows = pl.ds(pl.multiple_of(b * XB, XB), XB)
        return pltpu.make_async_copy(x_hbm.at[0, rows, :], io_v.at[rows, :], xsem.at[b])

    def ccopy():
        return pltpu.make_async_copy(c_hbm.at[0], c_v, csem.at[0])

    def wcopies(jj, sl):
        return [
            pltpu.make_async_copy(wk_hbm.bitcast(U32).at[:, jj, :], wk_b.at[sl], wsem.at[0, sl]),
            pltpu.make_async_copy(wq_hbm.bitcast(U32).at[:, jj, :], wq_b.at[sl], wsem.at[1, sl]),
            pltpu.make_async_copy(wv_hbm.bitcast(U32).at[:, jj, :], wv_b.at[sl], wsem.at[2, sl]),
            pltpu.make_async_copy(wo_hbm.at[pl.ds(2 * jj, 2)], wo_b.at[sl], wsem.at[3, sl]),
        ]

    def fcopy(t):
        if t == 0:
            return pltpu.make_async_copy(wg_hbm, wg_v, fsem.at[0])
        if t == 1:
            return pltpu.make_async_copy(wu_hbm, wu_v, fsem.at[1])
        return pltpu.make_async_copy(wd_hbm, wd_v.at[:, 0:M], fsem.at[2])

    def ocopy(b):
        rows = pl.ds(pl.multiple_of(b * OB, OB), OB)
        return pltpu.make_async_copy(io_v.at[rows, :], out_hbm.at[0, rows, :], osem.at[b])

    for b in range(S // XB):
        xcopy(b).start()
    ccopy().start()
    for cp in wcopies(0, 0):
        cp.start()

    def ln1(b, carry):
        xcopy(b).wait()
        rows = pl.ds(pl.multiple_of(b * XB, XB), XB)
        xf = io_v[rows, :].astype(F32)
        mu = jnp.mean(xf, axis=1, keepdims=True)
        xc = xf - mu
        var = jnp.mean(xc * xc, axis=1, keepdims=True)
        xn_s[rows, :] = (xc * lax.rsqrt(var + 1e-5)).astype(BF16)
        acc_s[rows, :] = xf
        return carry
    lax.fori_loop(0, S // XB, ln1, 0)
    ccopy().wait()

    scale = (D ** -0.5) * math.log2(math.e)

    def step(j, carry):
        slot = j % 2

        @pl.when(j + 1 < NP)
        def _():
            for cp in wcopies(j + 1, 1 - slot):
                cp.start()

        for t in range(3):
            @pl.when(j == 2 * t + 1)
            def _():
                fcopy(t).start()

        for cp in wcopies(j, slot):
            cp.wait()

        c = c_v[...]
        kp = jnp.dot(c, _unpack_pair(wk_b[slot]), preferred_element_type=F32).astype(BF16)
        qp = (jnp.dot(xn_s[...], _unpack_pair(wq_b[slot]), preferred_element_type=F32) * scale).astype(BF16)
        vp = jnp.dot(c, _unpack_pair(wv_b[slot]), preferred_element_type=F32).astype(BF16)
        wo = wo_b[slot].reshape(2 * D, M)
        _attn_pair(qp, kp, vp, wo, acc_s, S, D)
        return carry
    lax.fori_loop(0, NP, step, 0)

    wr16 = jnp.broadcast_to(wr_ref[...].astype(F32), (16, M)).astype(BF16)
    eps = jnp.asarray(1e-5, BF16).astype(F32)

    def ln2(b, carry):
        rows = pl.ds(pl.multiple_of(b * OB, OB), OB)
        hf = _rb(acc_s[rows, :])
        mu = jnp.mean(hf, axis=1, keepdims=True)
        mub = _rb(mu)
        d = hf - mub
        dm = mu - mub
        var = jnp.maximum(jnp.mean(d * d, axis=1, keepdims=True) - dm * dm, 0.0)
        den = _rb(jnp.sqrt(_rb(_rb(var) + eps)))
        lnb = (d * (1.0 / den)).astype(BF16)
        xn_s[rows, :] = lnb
        io_v[rows, :] = (hf + lnb.astype(F32)).astype(BF16)
        ocopy(b).start()
        r = lax.dot_general(wr16, lnb, NT, preferred_element_type=F32)
        r_s[pl.ds(b, 1), :] = _rb(r[0:1, :])
        return carry
    lax.fori_loop(0, S // OB, ln2, 0)

    r = r_s[...]
    idx = (lax.broadcasted_iota(jnp.int32, r.shape, 0) * OB
           + lax.broadcasted_iota(jnp.int32, r.shape, 1)).astype(F32)
    m1 = jnp.max(r, keepdims=True)
    f1 = jnp.min(jnp.where(r == m1, idx, float(S)), keepdims=True)
    r2 = jnp.where(idx == f1, -jnp.inf, r)
    m2 = jnp.max(r2, keepdims=True)
    f2 = jnp.min(jnp.where(r2 == m2, idx, float(S)), keepdims=True)
    i1 = jnp.clip(f1[0, 0].astype(jnp.int32), 0, S - 1)
    i2 = jnp.clip(f2[0, 0].astype(jnp.int32), 0, S - 1)
    g1 = pl.multiple_of((i1 // 16) * 16, 16)
    g2 = pl.multiple_of((i2 // 16) * 16, 16)

    rid = lax.broadcasted_iota(jnp.int32, (16, M), 0)

    def pick(g, i):
        blk = xn_s[pl.ds(g, 16), :].astype(F32)
        return jnp.sum(jnp.where(rid == i - g, blk, 0.0), axis=0, keepdims=True)

    xs = jnp.where(rid == 0, pick(g1, i1), pick(g2, i2))
    xsb = xs.astype(BF16)
    for t in range(3):
        fcopy(t).wait()
    nch = FF // FC
    acts = []
    y = None
    for t in range(nch + 1):
        if t < nch:
            a = _rb(jnp.dot(xsb, wg_v[:, t * FC:(t + 1) * FC], preferred_element_type=F32))
            u = _rb(jnp.dot(xsb, wu_v[:, t * FC:(t + 1) * FC], preferred_element_type=F32))
            g = _rb(a * _rb(jax.nn.sigmoid(a)))
            acts.append((g * u).astype(BF16))
        if t > 0:
            yt = jnp.dot(acts[t - 1], wd_v[(t - 1) * FC:t * FC, 0:M], preferred_element_type=F32)
            y = yt if y is None else y + yt
    rsel = jnp.where(rid == 0, m1, m2)
    y = _rb(_rb(y) * _rb(jax.nn.sigmoid(rsel)))
    upd = _rb(xs + y)

    for b in range(S // OB):
        ocopy(b).wait()
    for (ii, gg, rr) in ((i1, g1, 0), (i2, g2, 1)):
        new = _rb(acc_s[pl.ds(ii, 1), :]) + upd[rr:rr + 1, :]
        cur = io_v[pl.ds(gg, 16), :].astype(F32)
        io_v[pl.ds(gg, 16), :] = jnp.where(rid == ii - gg, new, cur).astype(BF16)

    def pcopy(g, k):
        return pltpu.make_async_copy(io_v.at[pl.ds(g, 16), :], out_hbm.at[0, pl.ds(g, 16), :], osem.at[k])

    pcopy(g1, 0).start()

    @pl.when(g2 != g1)
    def _():
        pcopy(g2, 1).start()
        pcopy(g2, 1).wait()
    pcopy(g1, 0).wait()


@jax.jit
def pallas_sequential_preLN__compressed_kv_cla__moe_arch_mod__prompt_kernel(
    A_x: jax.Array,
    A_c_kv: jax.Array,
    A_w_q: jax.Array,
    A_w_uk: jax.Array,
    A_w_uv: jax.Array,
    A_w_o: jax.Array,
    B_x: jax.Array,
    B_w_r: jax.Array,
    B_w_gate: jax.Array,
    B_w_up: jax.Array,
    B_w_down: jax.Array,
):
    _, S, M = A_x.shape
    C = A_c_kv.shape[2]
    H, D = A_w_q.shape[1], A_w_q.shape[2]
    FF = B_w_gate.shape[1]
    NP = H // 2
    any_spec = pl.BlockSpec(memory_space=pl.ANY)
    return pl.pallas_call(
        functools.partial(_kernel, S=S, M=M, D=D, NP=NP, FF=FF),
        in_specs=[
            any_spec, any_spec, any_spec, any_spec, any_spec, any_spec,
            pl.BlockSpec(memory_space=pltpu.VMEM),
            any_spec, any_spec, any_spec,
        ],
        out_specs=any_spec,
        out_shape=jax.ShapeDtypeStruct((1, S, M), BF16),
        scratch_shapes=[
            pltpu.VMEM((S, M), BF16),
            pltpu.VMEM((S, C), BF16),
            pltpu.VMEM((S, M), BF16),
            pltpu.VMEM((S, M), F32),
            pltpu.VMEM((S // OB, OB), F32),
            pltpu.VMEM((2, M, D), jnp.uint32),
            pltpu.VMEM((2, C, D), jnp.uint32),
            pltpu.VMEM((2, C, D), jnp.uint32),
            pltpu.VMEM((2, 2, D, M), BF16),
            pltpu.VMEM((M, FF), BF16),
            pltpu.VMEM((M, FF), BF16),
            pltpu.VMEM((FF, M + 128), BF16),
            pltpu.SemaphoreType.DMA((S // XB,)),
            pltpu.SemaphoreType.DMA((1,)),
            pltpu.SemaphoreType.DMA((4, 2)),
            pltpu.SemaphoreType.DMA((3,)),
            pltpu.SemaphoreType.DMA((S // OB,)),
        ],
        compiler_params=pltpu.CompilerParams(
            vmem_limit_bytes=110 * 1024 * 1024,
        ),
    )(A_x, A_c_kv, A_w_q, A_w_uk, A_w_uv, A_w_o, B_w_r.reshape(1, M), B_w_gate, B_w_up, B_w_down)
```

```python
import functools
import math
import os

import jax
import jax.numpy as jnp
from jax import lax
import jax.experimental.pallas as pl
import jax.experimental.pallas.tpu as pltpu

F32 = jnp.float32
BF16 = jnp.bfloat16
NEG = -1e30
NT = (((1,), (1,)), ((), ()))
TQ = 512
SUB = 128
GRP = 4
ORDER_MAIN = os.environ.get("ORDER_MAIN", "S03 S13 P03 S02 P13 S12 P02 S01 P12 S11 O3 P01 S00 P11 S10 O2 P00 P10 O1 O0")
ORDER_LAST = os.environ.get("ORDER_LAST", "S03 S13 P03 S02 P13 S12 P02 S01 P12 S11 P01 S00 P11 S10 C3 P00 P10 O0 C2 C1 C0")
XB = 256
AHEAD = int(os.environ.get('AHEAD', 2))
EB = int(os.environ.get('EB', 256))
FC = 256
NF = 2


def _rb(v):
    return v.astype(BF16).astype(F32)


def _recip(l):
    r = pl.reciprocal(l, approx=True)
    return r * (2.0 - l * r)


def _unpack_pair(w32):
    lo = pltpu.bitcast(w32 << 16, F32)
    hi = pltpu.bitcast(w32 & jnp.uint32(0xFFFF0000), F32)
    return jnp.concatenate([lo, hi], axis=1).astype(BF16)


def _qk(q, k, i):
    r0 = i * TQ
    nb = TQ // SUB
    qb = q[r0:r0 + TQ, :]
    s_main = lax.dot_general(qb, k[0:r0 + SUB, :], NT, preferred_element_type=F32)
    s_ext = [lax.dot_general(qb[c * SUB:, :], k[r0 + c * SUB:r0 + (c + 1) * SUB, :], NT,
                             preferred_element_type=F32) for c in range(1, nb)]
    return s_main, s_ext


def _softmax(s, i):
    s_main, s_ext = s
    r0 = i * TQ
    nb = TQ // SUB
    row = lax.broadcasted_iota(jnp.int32, (SUB, SUB), 0)
    col = lax.broadcasted_iota(jnp.int32, (SUB, SUB), 1)
    tri = col <= row
    p_main, p_ext, ls = [], [[] for _ in range(1, nb)], []
    for b in range(nb):
        sm = s_main[b * SUB:(b + 1) * SUB, :]
        if b == 0:
            d = jnp.where(tri, sm[:, r0:], NEG)
            sm = jnp.concatenate([sm[:, :r0], d], axis=1) if r0 > 0 else d
        parts = [sm]
        for c in range(1, b + 1):
            e = s_ext[c - 1][(b - c) * SUB:(b - c + 1) * SUB, :]
            if c == b:
                e = jnp.where(tri, e, NEG)
            parts.append(e)
        sb = jnp.concatenate(parts, axis=1) if len(parts) > 1 else parts[0]
        m = jnp.max(sb, axis=1, keepdims=True)
        p = jnp.exp2(sb - m)
        nt = p.shape[1] // SUB
        tiles = [p[:, t * SUB:(t + 1) * SUB] for t in range(nt)]
        acc = None
        for t0 in range(0, nt, GRP):
            grp = tiles[t0:t0 + GRP]
            tot = grp[0]
            for g in grp[1:]:
                tot = tot + g
            acc = tot if acc is None else acc + tot
            last = t0 + len(grp) - 1
            if acc is not tiles[last]:
                tiles[last] = jnp.minimum(tiles[last], acc)
        p = jnp.concatenate(tiles, axis=1) if nt > 1 else tiles[0]
        ls.append(jnp.sum(acc, axis=1, keepdims=True))
        p_main.append(p[:, :r0 + SUB])
        for c in range(1, b + 1):
            p_ext[c - 1].append(p[:, r0 + c * SUB:r0 + (c + 1) * SUB])
    pm = jnp.concatenate(p_main, axis=0).astype(BF16)
    pe = [(jnp.concatenate(e, axis=0) if len(e) > 1 else e[0]).astype(BF16) for e in p_ext]
    return pm, pe, ls


def _pv(p, v, i):
    pm, pe, ls = p
    r0 = i * TQ
    nb = TQ // SUB
    o = jnp.dot(pm, v[0:r0 + SUB, :], preferred_element_type=F32)
    os_ = [o[b * SUB:(b + 1) * SUB] for b in range(nb)]
    for c in range(1, nb):
        oe = jnp.dot(pe[c - 1], v[r0 + c * SUB:r0 + (c + 1) * SUB, :], preferred_element_type=F32)
        for b in range(c, nb):
            os_[b] = os_[b] + oe[(b - c) * SUB:(b - c + 1) * SUB]
    return jnp.concatenate([os_[b] * _recip(ls[b]) for b in range(nb)], axis=0)


def _attn_pair(q_s, k_s, v_s, order, actions):
    sc, ctx = {}, {}

    def pair_ctx(i):
        return jnp.concatenate([ctx[(0, i)], ctx[(1, i)]], axis=1).astype(BF16)

    for tok in order.split():
        if tok[0] == 'S':
            h, i = int(tok[1]), int(tok[2])
            sc[(h, i)] = _qk(q_s.at[h], k_s.at[h], i)
        elif tok[0] == 'P':
            h, i = int(tok[1]), int(tok[2])
            ctx[(h, i)] = _pv(_softmax(sc.pop((h, i)), i), v_s.at[h], i)
        else:
            actions[tok[0]](int(tok[1:]), pair_ctx)


def _kernel(x_hbm, c_hbm, wq_hbm, wk_hbm, wv_hbm, wo_hbm, wr_ref, wg_hbm, wu_hbm, wd_hbm,
            out_hbm,
            io_v, c_v, xn_s, acc_s, h_s, r_s, ctx_s, q_s, k_s, v_s,
            wq_b, wk_b, wv_b, wo_b, wg_v, wu_v, wd_v,
            xsem, csem, wsem, osem_w, fsem, osem,
            *, S, M, D, NP, FF):
    U32 = jnp.uint32
    scale = (D ** -0.5) * math.log2(math.e)

    def xcopy(b):
        rows = pl.ds(pl.multiple_of(b * XB, XB), XB)
        return pltpu.make_async_copy(x_hbm.at[0, rows, :], io_v.at[rows, :], xsem.at[b])

    def ccopy(b):
        rows = pl.ds(pl.multiple_of(b * XB, XB), XB)
        return pltpu.make_async_copy(c_hbm.at[0, rows, :], c_v.at[rows, :], csem.at[b])

    def wcopies(jj, sl):
        return [
            pltpu.make_async_copy(wk_hbm.bitcast(U32).at[:, jj, :], wk_b.at[sl], wsem.at[0, sl]),
            pltpu.make_async_copy(wv_hbm.bitcast(U32).at[:, jj, :], wv_b.at[sl], wsem.at[1, sl]),
            pltpu.make_async_copy(wq_hbm.bitcast(U32).at[:, jj, :], wq_b.at[sl], wsem.at[2, sl]),
        ]

    def wocopy(jj, sl):
        return pltpu.make_async_copy(wo_hbm.at[pl.ds(2 * jj, 2)], wo_b.at[sl], osem_w.at[sl])

    def fcopy(t):
        if t == 0:
            return pltpu.make_async_copy(wg_hbm, wg_v, fsem.at[0])
        if t == 1:
            return pltpu.make_async_copy(wu_hbm, wu_v, fsem.at[1])
        return pltpu.make_async_copy(wd_hbm, wd_v.at[:, 0:M], fsem.at[2])

    def ocopy(b):
        rows = pl.ds(pl.multiple_of(b * EB, EB), EB)
        return pltpu.make_async_copy(io_v.at[rows, :], out_hbm.at[0, rows, :], osem.at[b])

    def project(xn, c, sl, rows):
        kp = jnp.dot(c, _unpack_pair(wk_b[sl]), preferred_element_type=F32).astype(BF16)
        k_s[0, rows, :] = kp[:, :D]
        k_s[1, rows, :] = kp[:, D:]
        vp = jnp.dot(c, _unpack_pair(wv_b[sl]), preferred_element_type=F32).astype(BF16)
        v_s[0, rows, :] = vp[:, :D]
        v_s[1, rows, :] = vp[:, D:]
        qp = (jnp.dot(xn, _unpack_pair(wq_b[sl]), preferred_element_type=F32) * scale).astype(BF16)
        q_s[0, rows, :] = qp[:, :D]
        q_s[1, rows, :] = qp[:, D:]

    NXB = S // XB
    for cp in wcopies(0, 0):
        cp.start()
    ccopy(0).start()
    xcopy(0).start()
    for cp in wcopies(0, 0):
        cp.wait()
    for b in range(1, AHEAD):
        ccopy(b).start()
        xcopy(b).start()

    def first(b, carry):
        ccopy(b).wait()
        xcopy(b).wait()

        @pl.when(b + AHEAD < NXB)
        def _():
            ccopy(b + AHEAD).start()
            xcopy(b + AHEAD).start()

        @pl.when(b + AHEAD == NXB)
        def _():
            wocopy(0, 0).start()
            for cp in wcopies(1, 1):
                cp.start()

        rows = pl.ds(pl.multiple_of(b * XB, XB), XB)
        xf = io_v[rows, :].astype(F32)
        mu = jnp.mean(xf, axis=1, keepdims=True)
        xc = xf - mu
        var = jnp.mean(xc * xc, axis=1, keepdims=True)
        xn = (xc * lax.rsqrt(var + 1e-5)).astype(BF16)
        xn_s[rows, :] = xn
        acc_s[rows, :] = xf
        project(xn, c_v[rows, :], 0, rows)
        return carry
    lax.fori_loop(0, S // XB, first, 0)

    def step(j, carry):
        slot = j % 2
        wocopy(j, slot).wait()
        for cp in wcopies(j + 1, 1 - slot):
            cp.wait()
        wocopy(j + 1, 1 - slot).start()

        @pl.when(j + 2 < NP)
        def _():
            for cp in wcopies(j + 2, slot):
                cp.start()

        for t in range(3):
            @pl.when(j == 2 * t + 1)
            def _():
                fcopy(t).start()

        wo = wo_b[slot].reshape(2 * D, M)

        def oproj(ii, pair_ctx):
            acc_s[ii * TQ:(ii + 1) * TQ, :] += jnp.dot(pair_ctx(ii), wo, preferred_element_type=F32)

        _attn_pair(q_s, k_s, v_s, ORDER_MAIN, {'O': oproj})
        project(xn_s[...], c_v[...], 1 - slot, slice(None))
        return carry
    lax.fori_loop(0, NP - 1, step, 0)

    last = (NP - 1) % 2
    wocopy(NP - 1, last).wait()
    eps = jnp.asarray(1e-5, BF16).astype(F32)

    NEB = S // EB

    def erows(b):
        return pl.ds(pl.multiple_of(b * EB, EB), EB)

    def oproj_h(b):
        rows = erows(b)
        h_s[rows, :] = (acc_s[rows, :]
                        + jnp.dot(ctx_s[rows, :], wo_b[last].reshape(2 * D, M),
                                  preferred_element_type=F32)).astype(BF16)

    def ln2(b):
        rows = erows(b)
        hf = h_s[rows, :].astype(F32)
        mu = jnp.mean(hf, axis=1, keepdims=True)
        mub = _rb(mu)
        d = hf - mub
        dm = mu - mub
        var = jnp.maximum(jnp.mean(d * d, axis=1, keepdims=True) - dm * dm, 0.0)
        ve = _rb(_rb(var) + eps)
        den = _rb(ve * lax.rsqrt(ve))
        lnb = (d * _recip(den)).astype(BF16)
        xn_s[rows, :] = lnb
        io_v[rows, :] = (hf + lnb.astype(F32)).astype(BF16)

    def router(b):
        wr16 = jnp.broadcast_to(wr_ref[...].astype(F32), (16, M)).astype(BF16)
        r = lax.dot_general(wr16, xn_s[erows(b), :], NT, preferred_element_type=F32)
        r_s[pl.ds(b, 1), :] = _rb(r[0:1, :])
        ocopy(b).start()

    def keep_ctx(ii, pair_ctx):
        ctx_s[ii * TQ:(ii + 1) * TQ, :] = pair_ctx(ii)

    _attn_pair(q_s, k_s, v_s, ORDER_LAST,
               {'C': keep_ctx, 'O': lambda ii, pc: oproj_h(NEB - 1)})

    def tail(i, carry):
        b = NEB - 1 - i
        ln2(b + 1)
        oproj_h(b)
        router(b + 1)
        return carry
    lax.fori_loop(1, NEB, tail, 0)
    ln2(0)
    router(0)

    r = r_s[...]
    idx = (lax.broadcasted_iota(jnp.int32, r.shape, 0) * EB
           + lax.broadcasted_iota(jnp.int32, r.shape, 1)).astype(F32)
    m1 = jnp.max(r, keepdims=True)
    f1 = jnp.min(jnp.where(r == m1, idx, float(S)), keepdims=True)
    r2 = jnp.where(idx == f1, -jnp.inf, r)
    m2 = jnp.max(r2, keepdims=True)
    f2 = jnp.min(jnp.where(r2 == m2, idx, float(S)), keepdims=True)
    i1 = jnp.clip(f1[0, 0].astype(jnp.int32), 0, S - 1)
    i2 = jnp.clip(f2[0, 0].astype(jnp.int32), 0, S - 1)
    g1 = pl.multiple_of((i1 // 16) * 16, 16)
    g2 = pl.multiple_of((i2 // 16) * 16, 16)

    rid = lax.broadcasted_iota(jnp.int32, (16, M), 0)

    def pick(g, i):
        blk = xn_s[pl.ds(g, 16), :].astype(F32)
        return jnp.sum(jnp.where(rid == i - g, blk, 0.0), axis=0, keepdims=True)

    xs = jnp.where(rid == 0, pick(g1, i1), pick(g2, i2))
    xsb = xs.astype(BF16)
    for t in range(3):
        fcopy(t).wait()
    FH = FF // NF

    def ffn(o, y):
        nch = FH // FC
        acts = []
        for t in range(nch + 1):
            if t < nch:
                cols = pl.ds(pl.multiple_of(o * FH + t * FC, 128), FC)
                a = _rb(jnp.dot(xsb, wg_v[:, cols], preferred_element_type=F32))
                u = _rb(jnp.dot(xsb, wu_v[:, cols], preferred_element_type=F32))
                g = _rb(a * _rb(jax.nn.sigmoid(a)))
                acts.append((g * u).astype(BF16))
            if t > 0:
                rws = pl.ds(pl.multiple_of(o * FH + (t - 1) * FC, 128), FC)
                y = y + jnp.dot(acts[t - 1], wd_v[rws, 0:M], preferred_element_type=F32)
        return y
    y = lax.fori_loop(0, NF, ffn, jnp.zeros((16, M), F32))
    rsel = jnp.where(rid == 0, m1, m2)
    y = _rb(_rb(y) * _rb(jax.nn.sigmoid(rsel)))
    upd = _rb(xs + y)

    for b in range(NEB):
        ocopy(b).wait()
    for (ii, gg, rr) in ((i1, g1, 0), (i2, g2, 1)):
        new = h_s[pl.ds(gg, 16), :].astype(F32) + upd[rr:rr + 1, :]
        cur = io_v[pl.ds(gg, 16), :].astype(F32)
        io_v[pl.ds(gg, 16), :] = jnp.where(rid == ii - gg, new, cur).astype(BF16)

    def pcopy(g, k):
        return pltpu.make_async_copy(io_v.at[pl.ds(g, 16), :], out_hbm.at[0, pl.ds(g, 16), :], osem.at[k])

    pcopy(g1, 0).start()

    @pl.when(g2 != g1)
    def _():
        pcopy(g2, 1).start()
        pcopy(g2, 1).wait()
    pcopy(g1, 0).wait()


@jax.jit
def pallas_sequential_preLN__compressed_kv_cla__moe_arch_mod__prompt_kernel(
    A_x: jax.Array,
    A_c_kv: jax.Array,
    A_w_q: jax.Array,
    A_w_uk: jax.Array,
    A_w_uv: jax.Array,
    A_w_o: jax.Array,
    B_x: jax.Array,
    B_w_r: jax.Array,
    B_w_gate: jax.Array,
    B_w_up: jax.Array,
    B_w_down: jax.Array,
):
    _, S, M = A_x.shape
    C = A_c_kv.shape[2]
    H, D = A_w_q.shape[1], A_w_q.shape[2]
    FF = B_w_gate.shape[1]
    NP = H // 2
    any_spec = pl.BlockSpec(memory_space=pl.ANY)
    return pl.pallas_call(
        functools.partial(_kernel, S=S, M=M, D=D, NP=NP, FF=FF),
        in_specs=[
            any_spec, any_spec, any_spec, any_spec, any_spec, any_spec,
            pl.BlockSpec(memory_space=pltpu.VMEM),
            any_spec, any_spec, any_spec,
        ],
        out_specs=any_spec,
        out_shape=jax.ShapeDtypeStruct((1, S, M), BF16),
        scratch_shapes=[
            pltpu.VMEM((S, M), BF16),
            pltpu.VMEM((S, C), BF16),
            pltpu.VMEM((S, M), BF16),
            pltpu.VMEM((S, M), F32),
            pltpu.VMEM((S, M), BF16),
            pltpu.VMEM((S // EB, EB), F32),
            pltpu.VMEM((S, 2 * D), BF16),
            pltpu.VMEM((2, S, D), BF16),
            pltpu.VMEM((2, S, D), BF16),
            pltpu.VMEM((2, S, D), BF16),
            pltpu.VMEM((2, M, D), jnp.uint32),
            pltpu.VMEM((2, C, D), jnp.uint32),
            pltpu.VMEM((2, C, D), jnp.uint32),
            pltpu.VMEM((2, 2, D, M), BF16),
            pltpu.VMEM((M, FF), BF16),
            pltpu.VMEM((M, FF), BF16),
            pltpu.VMEM((FF, M + 128), BF16),
            pltpu.SemaphoreType.DMA((S // XB,)),
            pltpu.SemaphoreType.DMA((S // XB,)),
            pltpu.SemaphoreType.DMA((3, 2)),
            pltpu.SemaphoreType.DMA((2,)),
            pltpu.SemaphoreType.DMA((3,)),
            pltpu.SemaphoreType.DMA((S // EB,)),
        ],
        compiler_params=pltpu.CompilerParams(
            vmem_limit_bytes=110 * 1024 * 1024,
        ),
    )(A_x, A_c_kv, A_w_q, A_w_uk, A_w_uv, A_w_o, B_w_r.reshape(1, M), B_w_gate, B_w_up, B_w_down)
```

```python
import functools
import math
import os

import jax
import jax.numpy as jnp
from jax import lax
import jax.experimental.pallas as pl
import jax.experimental.pallas.tpu as pltpu

F32 = jnp.float32
BF16 = jnp.bfloat16
NEG = -1e30
NT = (((1,), (1,)), ((), ()))
TQ = 512
SUB = 128
GRP = 4
ORDER_MAIN = os.environ.get("ORDER_MAIN", "S03 S13 P03 S02 P13 S12 P02 S01 P12 S11 O3 P01 S00 P11 S10 O2 P00 P10 O1 O0")
ORDER_LAST = os.environ.get("ORDER_LAST", "S3 S2 P3 S1 P2 S0 P1 P0")
XB = 256
AHEAD = int(os.environ.get('AHEAD', 2))
EBLOCKS = tuple(int(t) for t in os.environ.get('EBLOCKS', '256,256,256,256,256,256,256,128,128').split(','))
RLAG = int(os.environ.get('RLAG', 2))
FC = 256
NF = 2


def _rb(v):
    return v.astype(BF16).astype(F32)


def _recip(l):
    r = pl.reciprocal(l, approx=True)
    return r * (2.0 - l * r)


def _unpack_pair(w32):
    lo = pltpu.bitcast(w32 << 16, F32)
    hi = pltpu.bitcast(w32 & jnp.uint32(0xFFFF0000), F32)
    return jnp.concatenate([lo, hi], axis=1).astype(BF16)


def _qk(q, k, i):
    r0 = i * TQ
    nb = TQ // SUB
    qb = q[r0:r0 + TQ, :]
    s_main = lax.dot_general(qb, k[0:r0 + SUB, :], NT, preferred_element_type=F32)
    s_ext = [lax.dot_general(qb[c * SUB:, :], k[r0 + c * SUB:r0 + (c + 1) * SUB, :], NT,
                             preferred_element_type=F32) for c in range(1, nb)]
    return s_main, s_ext


def _softmax(s, i):
    s_main, s_ext = s
    r0 = i * TQ
    nb = TQ // SUB
    row = lax.broadcasted_iota(jnp.int32, (SUB, SUB), 0)
    col = lax.broadcasted_iota(jnp.int32, (SUB, SUB), 1)
    tri = col <= row
    p_main, p_ext, ls = [], [[] for _ in range(1, nb)], []
    for b in range(nb):
        sm = s_main[b * SUB:(b + 1) * SUB, :]
        if b == 0:
            d = jnp.where(tri, sm[:, r0:], NEG)
            sm = jnp.concatenate([sm[:, :r0], d], axis=1) if r0 > 0 else d
        parts = [sm]
        for c in range(1, b + 1):
            e = s_ext[c - 1][(b - c) * SUB:(b - c + 1) * SUB, :]
            if c == b:
                e = jnp.where(tri, e, NEG)
            parts.append(e)
        sb = jnp.concatenate(parts, axis=1) if len(parts) > 1 else parts[0]
        m = jnp.max(sb, axis=1, keepdims=True)
        p = jnp.exp2(sb - m)
        nt = p.shape[1] // SUB
        tiles = [p[:, t * SUB:(t + 1) * SUB] for t in range(nt)]
        acc = None
        for t0 in range(0, nt, GRP):
            grp = tiles[t0:t0 + GRP]
            tot = grp[0]
            for g in grp[1:]:
                tot = tot + g
            acc = tot if acc is None else acc + tot
            last = t0 + len(grp) - 1
            if acc is not tiles[last]:
                tiles[last] = jnp.minimum(tiles[last], acc)
        p = jnp.concatenate(tiles, axis=1) if nt > 1 else tiles[0]
        ls.append(jnp.sum(acc, axis=1, keepdims=True))
        p_main.append(p[:, :r0 + SUB])
        for c in range(1, b + 1):
            p_ext[c - 1].append(p[:, r0 + c * SUB:r0 + (c + 1) * SUB])
    pm = jnp.concatenate(p_main, axis=0).astype(BF16)
    pe = [(jnp.concatenate(e, axis=0) if len(e) > 1 else e[0]).astype(BF16) for e in p_ext]
    return pm, pe, ls


def _pv(p, v, i):
    pm, pe, ls = p
    r0 = i * TQ
    nb = TQ // SUB
    o = jnp.dot(pm, v[0:r0 + SUB, :], preferred_element_type=F32)
    os_ = [o[b * SUB:(b + 1) * SUB] for b in range(nb)]
    for c in range(1, nb):
        oe = jnp.dot(pe[c - 1], v[r0 + c * SUB:r0 + (c + 1) * SUB, :], preferred_element_type=F32)
        for b in range(c, nb):
            os_[b] = os_[b] + oe[(b - c) * SUB:(b - c + 1) * SUB]
    return jnp.concatenate([os_[b] * _recip(ls[b]) for b in range(nb)], axis=0)


def _attn_pair(q_s, k_s, v_s, order, actions):
    sc, ctx = {}, {}

    def pair_ctx(i):
        return jnp.concatenate([ctx[(0, i)], ctx[(1, i)]], axis=1).astype(BF16)

    for tok in order.split():
        if tok[0] == 'S':
            h, i = int(tok[1]), int(tok[2])
            sc[(h, i)] = _qk(q_s.at[h], k_s.at[h], i)
        elif tok[0] == 'P':
            h, i = int(tok[1]), int(tok[2])
            ctx[(h, i)] = _pv(_softmax(sc.pop((h, i)), i), v_s.at[h], i)
        else:
            actions[tok[0]](int(tok[1:]), pair_ctx)


def _kernel(x_hbm, c_hbm, wq_hbm, wk_hbm, wv_hbm, wo_hbm, wr_ref, wg_hbm, wu_hbm, wd_hbm,
            out_hbm,
            io_v, c_v, xn_s, acc_s, h_s, ctx_s, q_s, k_s, v_s,
            wq_b, wk_b, wv_b, wo_b, wg_v, wu_v, wd_v,
            xsem, csem, wsem, osem_w, fsem, osem,
            *, S, M, D, NP, FF):
    U32 = jnp.uint32
    scale = (D ** -0.5) * math.log2(math.e)

    def xcopy(b):
        rows = pl.ds(pl.multiple_of(b * XB, XB), XB)
        return pltpu.make_async_copy(x_hbm.at[0, rows, :], io_v.at[rows, :], xsem.at[b])

    def ccopy(b):
        rows = pl.ds(pl.multiple_of(b * XB, XB), XB)
        return pltpu.make_async_copy(c_hbm.at[0, rows, :], c_v.at[rows, :], csem.at[b])

    def wcopies(jj, sl):
        return [
            pltpu.make_async_copy(wk_hbm.bitcast(U32).at[:, jj, :], wk_b.at[sl], wsem.at[0, sl]),
            pltpu.make_async_copy(wv_hbm.bitcast(U32).at[:, jj, :], wv_b.at[sl], wsem.at[1, sl]),
            pltpu.make_async_copy(wq_hbm.bitcast(U32).at[:, jj, :], wq_b.at[sl], wsem.at[2, sl]),
        ]

    def wocopy(jj, sl):
        return pltpu.make_async_copy(wo_hbm.at[pl.ds(2 * jj, 2)], wo_b.at[sl], osem_w.at[sl])

    def fcopy(t):
        if t == 0:
            return pltpu.make_async_copy(wg_hbm, wg_v, fsem.at[0])
        if t == 1:
            return pltpu.make_async_copy(wu_hbm, wu_v, fsem.at[1])
        return pltpu.make_async_copy(wd_hbm, wd_v.at[:, 0:M], fsem.at[2])

    def ocopy(b):
        rows = pl.ds(sum(EBLOCKS[:b]), EBLOCKS[b])
        return pltpu.make_async_copy(io_v.at[rows, :], out_hbm.at[0, rows, :], osem.at[b])

    def project(xn, c, sl, rows):
        kp = jnp.dot(c, _unpack_pair(wk_b[sl]), preferred_element_type=F32).astype(BF16)
        k_s[0, rows, :] = kp[:, :D]
        k_s[1, rows, :] = kp[:, D:]
        vp = jnp.dot(c, _unpack_pair(wv_b[sl]), preferred_element_type=F32).astype(BF16)
        v_s[0, rows, :] = vp[:, :D]
        v_s[1, rows, :] = vp[:, D:]
        qp = (jnp.dot(xn, _unpack_pair(wq_b[sl]), preferred_element_type=F32) * scale).astype(BF16)
        q_s[0, rows, :] = qp[:, :D]
        q_s[1, rows, :] = qp[:, D:]

    NXB = S // XB
    for cp in wcopies(0, 0):
        cp.start()
    ccopy(0).start()
    xcopy(0).start()
    for cp in wcopies(0, 0):
        cp.wait()
    for b in range(1, AHEAD):
        ccopy(b).start()
        xcopy(b).start()

    def first(b, carry):
        ccopy(b).wait()
        xcopy(b).wait()

        @pl.when(b + AHEAD < NXB)
        def _():
            ccopy(b + AHEAD).start()
            xcopy(b + AHEAD).start()

        @pl.when(b + AHEAD == NXB)
        def _():
            wocopy(0, 0).start()
            for cp in wcopies(1, 1):
                cp.start()

        rows = pl.ds(pl.multiple_of(b * XB, XB), XB)
        xf = io_v[rows, :].astype(F32)
        mu = jnp.mean(xf, axis=1, keepdims=True)
        xc = xf - mu
        var = jnp.mean(xc * xc, axis=1, keepdims=True)
        xn = (xc * lax.rsqrt(var + 1e-5)).astype(BF16)
        xn_s[rows, :] = xn
        acc_s[rows, :] = xf
        project(xn, c_v[rows, :], 0, rows)
        return carry
    lax.fori_loop(0, S // XB, first, 0)

    def step(j, carry):
        slot = j % 2
        wocopy(j, slot).wait()
        for cp in wcopies(j + 1, 1 - slot):
            cp.wait()
        wocopy(j + 1, 1 - slot).start()

        @pl.when(j + 2 < NP)
        def _():
            for cp in wcopies(j + 2, slot):
                cp.start()

        for t in range(3):
            @pl.when(j == 2 * t + 1)
            def _():
                fcopy(t).start()

        wo = wo_b[slot].reshape(2 * D, M)

        def oproj(ii, pair_ctx):
            acc_s[ii * TQ:(ii + 1) * TQ, :] += jnp.dot(pair_ctx(ii), wo, preferred_element_type=F32)

        _attn_pair(q_s, k_s, v_s, ORDER_MAIN, {'O': oproj})
        project(xn_s[...], c_v[...], 1 - slot, slice(None))
        return carry
    lax.fori_loop(0, NP - 1, step, 0)

    last = (NP - 1) % 2
    wocopy(NP - 1, last).wait()
    eps = jnp.asarray(1e-5, BF16).astype(F32)

    def last_head(h, carry):
        sc = {}
        for tok in ORDER_LAST.split():
            i = int(tok[1])
            if tok[0] == 'S':
                sc[i] = _qk(q_s.at[h], k_s.at[h], i)
            else:
                ctx_s[h, i * TQ:(i + 1) * TQ, :] = _pv(_softmax(sc.pop(i), i), v_s.at[h], i).astype(BF16)
        return carry
    lax.fori_loop(0, 2, last_head, 0)

    NCH = 4
    CW = M // NCH
    wr16 = [jnp.broadcast_to(wr_ref[:, t * CW:(t + 1) * CW].astype(F32), (16, CW)).astype(BF16) for t in range(NCH)]

    def oproj_part(r0, n, t):
        rows = slice(r0, r0 + n)
        cols = slice(t * CW, (t + 1) * CW)
        return (acc_s[rows, cols]
                + jnp.dot(ctx_s[0, rows, :], wo_b[last, 0, :, cols], preferred_element_type=F32)
                + jnp.dot(ctx_s[1, rows, :], wo_b[last, 1, :, cols], preferred_element_type=F32))

    def ln2(r0, n, h32):
        rows = slice(r0, r0 + n)
        hb = h32.astype(BF16)
        h_s[rows, :] = hb
        hf = hb.astype(F32)
        mu = jnp.mean(hf, axis=1, keepdims=True)
        mub = _rb(mu)
        d = hf - mub
        dm = mu - mub
        var = jnp.maximum(jnp.mean(d * d, axis=1, keepdims=True) - dm * dm, 0.0)
        ve = _rb(_rb(var) + eps)
        den = _rb(ve * lax.rsqrt(ve))
        ln = d * _recip(den)
        xn_s[rows, :] = ln.astype(BF16)
        io_v[rows, :] = (hf + ln).astype(BF16)

    def router_part(r0, n, t):
        cols = slice(t * CW, (t + 1) * CW)
        return lax.dot_general(wr16[t], xn_s[r0:r0 + n, cols], NT, preferred_element_type=F32)

    blocks = []
    r0 = 0
    for n in EBLOCKS:
        blocks.append((r0, n))
        r0 += n
    assert r0 == S
    rparts = []
    for k in range(len(blocks) + RLAG):
        hp, rp = [], None
        for t in range(NCH):
            if k < len(blocks):
                hp.append(oproj_part(*blocks[k], t))
            if k >= RLAG:
                part = router_part(*blocks[k - RLAG], t)
                rp = part if rp is None else rp + part
        if 1 <= k <= len(blocks):
            ocopy(k - 1).start()
        if k < len(blocks):
            ln2(*blocks[k], jnp.concatenate(hp, axis=1))
        if k >= RLAG:
            rparts.append(rp[0:8, :])
    rrow = _rb(jnp.concatenate(rparts, axis=1))

    r = rrow
    idx = lax.broadcasted_iota(jnp.int32, r.shape, 1).astype(F32)
    m1 = jnp.max(r, keepdims=True)
    f1 = jnp.min(jnp.where(r == m1, idx, float(S)), keepdims=True)
    r2 = jnp.where(idx == f1, -jnp.inf, r)
    m2 = jnp.max(r2, keepdims=True)
    f2 = jnp.min(jnp.where(r2 == m2, idx, float(S)), keepdims=True)
    i1 = jnp.clip(f1[0, 0].astype(jnp.int32), 0, S - 1)
    i2 = jnp.clip(f2[0, 0].astype(jnp.int32), 0, S - 1)
    g1 = pl.multiple_of((i1 // 16) * 16, 16)
    g2 = pl.multiple_of((i2 // 16) * 16, 16)

    rid = lax.broadcasted_iota(jnp.int32, (16, M), 0)

    def pick(g, i):
        blk = xn_s[pl.ds(g, 16), :].astype(F32)
        return jnp.sum(jnp.where(rid == i - g, blk, 0.0), axis=0, keepdims=True)

    xs = jnp.where(rid == 0, pick(g1, i1), pick(g2, i2))
    xsb = xs.astype(BF16)
    for t in range(3):
        fcopy(t).wait()
    FH = FF // NF

    def ffn(o, y):
        nch = FH // FC
        acts = []
        for t in range(nch + 1):
            if t < nch:
                cols = pl.ds(pl.multiple_of(o * FH + t * FC, 128), FC)
                a = _rb(jnp.dot(xsb, wg_v[:, cols], preferred_element_type=F32))
                u = _rb(jnp.dot(xsb, wu_v[:, cols], preferred_element_type=F32))
                g = _rb(a * _rb(jax.nn.sigmoid(a)))
                acts.append((g * u).astype(BF16))
            if t > 0:
                rws = pl.ds(pl.multiple_of(o * FH + (t - 1) * FC, 128), FC)
                y = y + jnp.dot(acts[t - 1], wd_v[rws, 0:M], preferred_element_type=F32)
        return y
    y = lax.fori_loop(0, NF, ffn, jnp.zeros((16, M), F32))
    rsel = jnp.where(rid == 0, m1, m2)
    y = _rb(_rb(y) * _rb(jax.nn.sigmoid(rsel)))
    upd = _rb(xs + y)

    for b in range(len(EBLOCKS)):
        ocopy(b).wait()
    for (ii, gg, rr) in ((i1, g1, 0), (i2, g2, 1)):
        new = h_s[pl.ds(gg, 16), :].astype(F32) + upd[rr:rr + 1, :]
        cur = io_v[pl.ds(gg, 16), :].astype(F32)
        io_v[pl.ds(gg, 16), :] = jnp.where(rid == ii - gg, new, cur).astype(BF16)

    def pcopy(g, k):
        return pltpu.make_async_copy(io_v.at[pl.ds(g, 16), :], out_hbm.at[0, pl.ds(g, 16), :], osem.at[k])

    pcopy(g1, 0).start()

    @pl.when(g2 != g1)
    def _():
        pcopy(g2, 1).start()
        pcopy(g2, 1).wait()
    pcopy(g1, 0).wait()


@jax.jit
def pallas_sequential_preLN__compressed_kv_cla__moe_arch_mod__prompt_kernel(
    A_x: jax.Array,
    A_c_kv: jax.Array,
    A_w_q: jax.Array,
    A_w_uk: jax.Array,
    A_w_uv: jax.Array,
    A_w_o: jax.Array,
    B_x: jax.Array,
    B_w_r: jax.Array,
    B_w_gate: jax.Array,
    B_w_up: jax.Array,
    B_w_down: jax.Array,
):
    _, S, M = A_x.shape
    C = A_c_kv.shape[2]
    H, D = A_w_q.shape[1], A_w_q.shape[2]
    FF = B_w_gate.shape[1]
    NP = H // 2
    any_spec = pl.BlockSpec(memory_space=pl.ANY)
    return pl.pallas_call(
        functools.partial(_kernel, S=S, M=M, D=D, NP=NP, FF=FF),
        in_specs=[
            any_spec, any_spec, any_spec, any_spec, any_spec, any_spec,
            pl.BlockSpec(memory_space=pltpu.VMEM),
            any_spec, any_spec, any_spec,
        ],
        out_specs=any_spec,
        out_shape=jax.ShapeDtypeStruct((1, S, M), BF16),
        scratch_shapes=[
            pltpu.VMEM((S, M), BF16),
            pltpu.VMEM((S, C), BF16),
            pltpu.VMEM((S, M), BF16),
            pltpu.VMEM((S, M), F32),
            pltpu.VMEM((S, M), BF16),
            pltpu.VMEM((2, S, D), BF16),
            pltpu.VMEM((2, S, D), BF16),
            pltpu.VMEM((2, S, D), BF16),
            pltpu.VMEM((2, S, D), BF16),
            pltpu.VMEM((2, M, D), jnp.uint32),
            pltpu.VMEM((2, C, D), jnp.uint32),
            pltpu.VMEM((2, C, D), jnp.uint32),
            pltpu.VMEM((2, 2, D, M), BF16),
            pltpu.VMEM((M, FF), BF16),
            pltpu.VMEM((M, FF), BF16),
            pltpu.VMEM((FF, M + 128), BF16),
            pltpu.SemaphoreType.DMA((S // XB,)),
            pltpu.SemaphoreType.DMA((S // XB,)),
            pltpu.SemaphoreType.DMA((3, 2)),
            pltpu.SemaphoreType.DMA((2,)),
            pltpu.SemaphoreType.DMA((3,)),
            pltpu.SemaphoreType.DMA((len(EBLOCKS),)),
        ],
        compiler_params=pltpu.CompilerParams(
            vmem_limit_bytes=110 * 1024 * 1024,
            disable_bounds_checks=bool(int(os.environ.get('NOBC', 0))),
        ),
    )(A_x, A_c_kv, A_w_q, A_w_uk, A_w_uv, A_w_o, B_w_r.reshape(1, M), B_w_gate, B_w_up, B_w_down)
```

```python
import functools
import math
import os

import jax
import jax.numpy as jnp
from jax import lax
import jax.experimental.pallas as pl
import jax.experimental.pallas.tpu as pltpu

F32 = jnp.float32
BF16 = jnp.bfloat16
NEG = -1e30
NT = (((1,), (1,)), ((), ()))
TQ = 512
SUB = 128
GRP = 4
SUMPACK = os.environ.get('SUMPACK', '')
ORDER_MAIN = os.environ.get("ORDER_MAIN", "S03 S13 P03 S02 P13 S12 P02 S01 P12 S11 O3 P01 S00 P11 S10 O2 P00 P10 O1 O0 K03 V03 Q03")
ORDER_LAST = os.environ.get("ORDER_LAST", "S2 S3 P2 S1 P3 S0 P1 P0")
XB = 256
AHEAD = int(os.environ.get('AHEAD', 2))
EBLOCKS = tuple(int(t) for t in os.environ.get('EBLOCKS', '128,128,128,128,128,128,128,128,128,128,128,128,128,128,128,128').split(','))
DEND = int(os.environ.get('DEND', 0))
LNMODE = int(os.environ.get('LNMODE', 1))
RPOS = os.environ.get('RPOS', '02')
RG = len(RPOS)
PONLY = int(os.environ.get('PONLY', 0))
RLAG = int(os.environ.get('RLAG', 2))
FC = 256
NF = 2


def _rb(v):
    return v.astype(BF16).astype(F32)


def _recip(l):
    r = pl.reciprocal(l, approx=True)
    return r * (2.0 - l * r)


def _unpack_pair(w32):
    lo = pltpu.bitcast(w32 << 16, F32)
    hi = pltpu.bitcast(w32 & jnp.uint32(0xFFFF0000), F32)
    return jnp.concatenate([lo, hi], axis=1).astype(BF16)


def _qk(q, k, i):
    r0 = i * TQ
    nb = TQ // SUB
    qb = q[r0:r0 + TQ, :]
    s_main = lax.dot_general(qb, k[0:r0 + SUB, :], NT, preferred_element_type=F32)
    s_ext = [lax.dot_general(qb[c * SUB:, :], k[r0 + c * SUB:r0 + (c + 1) * SUB, :], NT,
                             preferred_element_type=F32) for c in range(1, nb)]
    return s_main, s_ext


def _softmax(s, i):
    s_main, s_ext = s
    r0 = i * TQ
    nb = TQ // SUB
    row = lax.broadcasted_iota(jnp.int32, (SUB, SUB), 0)
    col = lax.broadcasted_iota(jnp.int32, (SUB, SUB), 1)
    tri = col <= row
    p_main, p_ext, ls = [], [[] for _ in range(1, nb)], []
    for b in range(nb):
        sm = s_main[b * SUB:(b + 1) * SUB, :]
        if b == 0:
            d = jnp.where(tri, sm[:, r0:], NEG)
            sm = jnp.concatenate([sm[:, :r0], d], axis=1) if r0 > 0 else d
        parts = [sm]
        for c in range(1, b + 1):
            e = s_ext[c - 1][(b - c) * SUB:(b - c + 1) * SUB, :]
            if c == b:
                e = jnp.where(tri, e, NEG)
            parts.append(e)
        sb = jnp.concatenate(parts, axis=1) if len(parts) > 1 else parts[0]
        m = jnp.max(sb, axis=1, keepdims=True)
        p = jnp.exp2(sb - m)
        if i == 0 and SUMPACK:
            tb = [p[:, t * SUB:(t + 1) * SUB].astype(BF16) for t in range(b + 1)]
            acc = tb[0].astype(F32)
            for t in tb[1:]:
                acc = acc + t.astype(F32)
            ls.append(jnp.sum(acc, axis=1, keepdims=True))
            p_main.append(tb[0])
            for c in range(1, b + 1):
                p_ext[c - 1].append(tb[c])
            continue
        else:
            nt = p.shape[1] // SUB
            tiles = [p[:, t * SUB:(t + 1) * SUB] for t in range(nt)]
            acc = None
            for t0 in range(0, nt, GRP):
                grp = tiles[t0:t0 + GRP]
                tot = grp[0]
                for g in grp[1:]:
                    tot = tot + g
                acc = tot if acc is None else acc + tot
                last = t0 + len(grp) - 1
                if acc is not tiles[last]:
                    tiles[last] = jnp.minimum(tiles[last], acc)
            p = jnp.concatenate(tiles, axis=1) if nt > 1 else tiles[0]
            ls.append(jnp.sum(acc, axis=1, keepdims=True))
        p_main.append(p[:, :r0 + SUB])
        for c in range(1, b + 1):
            p_ext[c - 1].append(p[:, r0 + c * SUB:r0 + (c + 1) * SUB])
    pm = jnp.concatenate(p_main, axis=0).astype(BF16)
    pe = [(jnp.concatenate(e, axis=0) if len(e) > 1 else e[0]).astype(BF16) for e in p_ext]
    return pm, pe, ls


def _pv(p, v, i):
    pm, pe, ls = p
    r0 = i * TQ
    nb = TQ // SUB
    o = jnp.dot(pm, v[0:r0 + SUB, :], preferred_element_type=F32)
    os_ = [o[b * SUB:(b + 1) * SUB] for b in range(nb)]
    for c in range(1, nb):
        oe = jnp.dot(pe[c - 1], v[r0 + c * SUB:r0 + (c + 1) * SUB, :], preferred_element_type=F32)
        for b in range(c, nb):
            os_[b] = os_[b] + oe[(b - c) * SUB:(b - c + 1) * SUB]
    return jnp.concatenate([os_[b] * _recip(ls[b]) for b in range(nb)], axis=0)


def _attn_pair(q_s, k_s, v_s, order, actions):
    sc, ctx = {}, {}

    def pair_ctx(i):
        return jnp.concatenate([ctx[(0, i)], ctx[(1, i)]], axis=1).astype(BF16)

    for tok in order.split():
        if tok[0] == 'S':
            h, i = int(tok[1]), int(tok[2])
            sc[(h, i)] = _qk(q_s.at[h], k_s.at[h], i)
        elif tok[0] == 'P':
            h, i = int(tok[1]), int(tok[2])
            ctx[(h, i)] = _pv(_softmax(sc.pop((h, i)), i), v_s.at[h], i)
        else:
            actions[tok[0]](int(tok[1:]), pair_ctx)


def _kernel(x_hbm, c_hbm, wq_hbm, wk_hbm, wv_hbm, wo_hbm, wr_hbm, wg_hbm, wu_hbm, wd_hbm,
            out_hbm,
            io_v, c_v, xn_s, acc_s, h_s, ctx_s, q_s, k_s, v_s,
            wq_b, wk_b, wv_b, wo_b, wr_ref, wg_v, wu_v, wd_v,
            xsem, csem, wsem, osem_w, fsem, osem,
            *, S, M, D, NP, FF):
    U32 = jnp.uint32
    scale = (D ** -0.5) * math.log2(math.e)

    def xcopy(b):
        rows = pl.ds(pl.multiple_of(b * XB, XB), XB)
        return pltpu.make_async_copy(x_hbm.at[0, rows, :], io_v.at[rows, :], xsem.at[b])

    def ccopy(b):
        rows = pl.ds(pl.multiple_of(b * XB, XB), XB)
        return pltpu.make_async_copy(c_hbm.at[0, rows, :], c_v.at[rows, :], csem.at[b])

    def wcopies(jj, sl):
        return [
            pltpu.make_async_copy(wk_hbm.bitcast(U32).at[:, jj, :], wk_b.at[sl], wsem.at[0, sl]),
            pltpu.make_async_copy(wv_hbm.bitcast(U32).at[:, jj, :], wv_b.at[sl], wsem.at[1, sl]),
            pltpu.make_async_copy(wq_hbm.bitcast(U32).at[:, jj, :], wq_b.at[sl], wsem.at[2, sl]),
        ]

    def wocopy(jj, sl):
        return pltpu.make_async_copy(wo_hbm.at[pl.ds(2 * jj, 2)], wo_b.at[sl], osem_w.at[sl])

    def fcopy(t):
        if t == 0:
            return pltpu.make_async_copy(wg_hbm, wg_v, fsem.at[0])
        if t == 1:
            return pltpu.make_async_copy(wu_hbm, wu_v, fsem.at[1])
        if t == 2:
            return pltpu.make_async_copy(wd_hbm, wd_v.at[:, 0:M], fsem.at[2])
        return pltpu.make_async_copy(wr_hbm, wr_ref, fsem.at[3])

    def ocopy(b):
        rows = pl.ds(sum(EBLOCKS[:b]), EBLOCKS[b])
        return pltpu.make_async_copy(io_v.at[rows, :], out_hbm.at[0, rows, :], osem.at[b])

    def project(dst, lhs, w32, rows, mult=None):
        y = jnp.dot(lhs, _unpack_pair(w32), preferred_element_type=F32)
        if mult is not None:
            y = y * mult
        y = y.astype(BF16)
        dst[0, rows, :] = y[:, :D]
        dst[1, rows, :] = y[:, D:]

    NXB = S // XB
    for cp in wcopies(0, 0):
        cp.start()
    ccopy(0).start()
    xcopy(0).start()
    for cp in wcopies(0, 0):
        cp.wait()
    for b in range(1, AHEAD):
        ccopy(b).start()
        xcopy(b).start()

    def first(b, carry):
        ccopy(b).wait()
        xcopy(b).wait()

        @pl.when(b + AHEAD < NXB)
        def _():
            ccopy(b + AHEAD).start()
            xcopy(b + AHEAD).start()

        @pl.when(b + AHEAD == NXB)
        def _():
            wocopy(0, 0).start()
            fcopy(3).start()
            for cp in wcopies(1, 1):
                cp.start()

        rows = pl.ds(pl.multiple_of(b * XB, XB), XB)
        xf = io_v[rows, :].astype(F32)
        mu = jnp.mean(xf, axis=1, keepdims=True)
        xc = xf - mu
        var = jnp.mean(xc * xc, axis=1, keepdims=True)
        xn = (xc * lax.rsqrt(var + 1e-5)).astype(BF16)
        xn_s[rows, :] = xn
        acc_s[rows, :] = xf
        c = c_v[rows, :]
        project(k_s, c, wk_b[0], rows)
        project(v_s, c, wv_b[0], rows)
        project(q_s, xn, wq_b[0], rows, scale)
        return carry
    lax.fori_loop(0, S // XB, first, 0)

    def step(j, carry):
        slot = j % 2
        wocopy(j, slot).wait()
        for cp in wcopies(j + 1, 1 - slot):
            cp.wait()
        wocopy(j + 1, 1 - slot).start()

        @pl.when(j + 2 < NP)
        def _():
            for cp in wcopies(j + 2, slot):
                cp.start()

        for t in range(3):
            @pl.when(j == 2 * t + 1)
            def _():
                fcopy(t).start()

        wo = wo_b[slot].reshape(2 * D, M)

        def oproj(ii, pair_ctx):
            acc_s[ii * TQ:(ii + 1) * TQ, :] += jnp.dot(pair_ctx(ii), wo, preferred_element_type=F32)

        def rows_of(code):
            return slice((code // 10) * TQ, (code % 10 + 1) * TQ)

        _attn_pair(q_s, k_s, v_s, ORDER_MAIN, {
            'O': oproj,
            'K': lambda code, _: project(k_s, c_v[rows_of(code), :], wk_b[1 - slot], rows_of(code)),
            'V': lambda code, _: project(v_s, c_v[rows_of(code), :], wv_b[1 - slot], rows_of(code)),
            'Q': lambda code, _: project(q_s, xn_s[rows_of(code), :], wq_b[1 - slot], rows_of(code), scale),
        })
        return carry
    lax.fori_loop(0, NP - 1, step, 0)

    last = (NP - 1) % 2
    wocopy(NP - 1, last).wait()
    fcopy(3).wait()
    if PONLY:
        return
    eps = jnp.asarray(1e-5, BF16).astype(F32)

    def last_head(h, carry):
        sc = {}
        for tok in ORDER_LAST.split():
            i = int(tok[1])
            if tok[0] == 'S':
                sc[i] = _qk(q_s.at[h], k_s.at[h], i)
            else:
                ctx_s[h, i * TQ:(i + 1) * TQ, :] = _pv(_softmax(sc.pop(i), i), v_s.at[h], i).astype(BF16)
        return carry
    lax.fori_loop(0, 2, last_head, 0)

    NCH = 4
    CW = M // NCH
    RW = M // RG
    wr16 = [jnp.broadcast_to(wr_ref[t * RW:(t + 1) * RW].astype(F32).reshape(1, RW), (16, RW)).astype(BF16)
            for t in range(RG)]

    def oproj_part(r0, n, t):
        rows = slice(r0, r0 + n)
        cols = slice(t * CW, (t + 1) * CW)
        return (acc_s[rows, cols]
                + jnp.dot(ctx_s[0, rows, :], wo_b[last, 0, :, cols], preferred_element_type=F32)
                + jnp.dot(ctx_s[1, rows, :], wo_b[last, 1, :, cols], preferred_element_type=F32))

    def ln2(r0, n, h32):
        rows = slice(r0, r0 + n)
        if LNMODE == 0:
            hb = h32.astype(BF16)
            h_s[rows, :] = hb
            hf = hb.astype(F32)
            get = lambda: hf
        elif LNMODE == 1:
            hf = h32
            acc_s[rows, :] = hf
            get = lambda: acc_s[rows, :]
        else:
            hb = h32.astype(BF16)
            h_s[rows, :] = hb
            hf = hb.astype(F32)
            get = lambda: h_s[rows, :].astype(F32)
        mu = jnp.mean(hf, axis=1, keepdims=True)
        mub = _rb(mu)
        d = get() - mub
        dm = mu - mub
        var = jnp.maximum(jnp.mean(d * d, axis=1, keepdims=True) - dm * dm, 0.0)
        ve = _rb(_rb(var) + eps)
        den = _rb(ve * lax.rsqrt(ve))
        h3 = get()
        ln = (d if LNMODE == 0 else h3 - mub) * _recip(den)
        xn_s[rows, :] = ln.astype(BF16)
        io_v[rows, :] = (h3 + ln).astype(BF16)

    def router_part(r0, n, t):
        cols = slice(t * RW, (t + 1) * RW)
        return lax.dot_general(wr16[t], xn_s[r0:r0 + n, cols], NT, preferred_element_type=F32)

    blocks = []
    r0 = 0
    for n in EBLOCKS:
        blocks.append((r0, n))
        r0 += n
    assert r0 == S
    rparts = []
    for k in range(len(blocks) + RLAG):
        hp, rp = [], None
        for t in range(NCH):
            if k < len(blocks):
                hp.append(oproj_part(*blocks[k], t))
            if k >= RLAG and str(t) in RPOS:
                part = router_part(*blocks[k - RLAG], RPOS.index(str(t)))
                rp = part if rp is None else rp + part
        if 1 <= k <= len(blocks) and not DEND:
            ocopy(k - 1).start()
        if k < len(blocks):
            ln2(*blocks[k], jnp.concatenate(hp, axis=1))
        if k >= RLAG:
            rparts.append(rp[0:8, :])
    if DEND:
        for k in range(len(blocks)):
            ocopy(k).start()
    rrow = _rb(jnp.concatenate(rparts, axis=1))

    I32 = jnp.int32
    b16 = lax.shift_right_logical(pltpu.bitcast(rrow, I32), 16)
    rank = jnp.where(b16 >= 0x8000, 0x10000 - b16, 0x8000 + b16)
    lane = lax.broadcasted_iota(I32, rrow.shape, 1)
    key = pltpu.bitcast(rank * S + (S - 1 - lane) + 0x20000000, F32)
    k1 = jnp.max(key, axis=1, keepdims=True)
    k2 = jnp.max(jnp.where(key == k1, 0.0, key), axis=1, keepdims=True)
    i1 = (S - 1) - (pltpu.bitcast(k1, I32)[0, 0] & (S - 1))
    i2 = (S - 1) - (pltpu.bitcast(k2, I32)[0, 0] & (S - 1))
    m1 = jnp.max(jnp.where(key == k1, rrow, -jnp.inf), axis=1, keepdims=True)[0:1, :]
    m2 = jnp.max(jnp.where(key == k2, rrow, -jnp.inf), axis=1, keepdims=True)[0:1, :]
    g1 = pl.multiple_of((i1 // 16) * 16, 16)
    g2 = pl.multiple_of((i2 // 16) * 16, 16)

    rid = lax.broadcasted_iota(jnp.int32, (16, M), 0)

    def pick(g, i):
        blk = xn_s[pl.ds(g, 16), :].astype(F32)
        return jnp.sum(jnp.where(rid == i - g, blk, 0.0), axis=0, keepdims=True)

    xs = jnp.where(rid == 0, pick(g1, i1), pick(g2, i2))
    xsb = xs.astype(BF16)
    for t in range(3):
        fcopy(t).wait()
    FH = FF // NF

    def ffn(o, y):
        nch = FH // FC
        acts = []
        for t in range(nch + 1):
            if t < nch:
                cols = pl.ds(pl.multiple_of(o * FH + t * FC, 128), FC)
                a = _rb(jnp.dot(xsb, wg_v[:, cols], preferred_element_type=F32))
                u = _rb(jnp.dot(xsb, wu_v[:, cols], preferred_element_type=F32))
                g = _rb(a * _rb(jax.nn.sigmoid(a)))
                acts.append((g * u).astype(BF16))
            if t > 0:
                rws = pl.ds(pl.multiple_of(o * FH + (t - 1) * FC, 128), FC)
                y = y + jnp.dot(acts[t - 1], wd_v[rws, 0:M], preferred_element_type=F32)
        return y
    y = lax.fori_loop(0, NF, ffn, jnp.zeros((16, M), F32))
    rsel = jnp.where(rid == 0, m1, m2)
    y = _rb(_rb(y) * _rb(jax.nn.sigmoid(rsel)))
    upd = _rb(xs + y)

    for b in range(len(EBLOCKS)):
        ocopy(b).wait()
    for (ii, gg, rr) in ((i1, g1, 0), (i2, g2, 1)):
        hrow = _rb(acc_s[pl.ds(gg, 16), :]) if LNMODE == 1 else h_s[pl.ds(gg, 16), :].astype(F32)
        new = hrow + upd[rr:rr + 1, :]
        cur = io_v[pl.ds(gg, 16), :].astype(F32)
        io_v[pl.ds(gg, 16), :] = jnp.where(rid == ii - gg, new, cur).astype(BF16)

    def pcopy(g, k):
        return pltpu.make_async_copy(io_v.at[pl.ds(g, 16), :], out_hbm.at[0, pl.ds(g, 16), :], osem.at[k])

    pcopy(g1, 0).start()

    @pl.when(g2 != g1)
    def _():
        pcopy(g2, 1).start()
        pcopy(g2, 1).wait()
    pcopy(g1, 0).wait()


@jax.jit
def pallas_sequential_preLN__compressed_kv_cla__moe_arch_mod__prompt_kernel(
    A_x: jax.Array,
    A_c_kv: jax.Array,
    A_w_q: jax.Array,
    A_w_uk: jax.Array,
    A_w_uv: jax.Array,
    A_w_o: jax.Array,
    B_x: jax.Array,
    B_w_r: jax.Array,
    B_w_gate: jax.Array,
    B_w_up: jax.Array,
    B_w_down: jax.Array,
):
    _, S, M = A_x.shape
    C = A_c_kv.shape[2]
    H, D = A_w_q.shape[1], A_w_q.shape[2]
    FF = B_w_gate.shape[1]
    NP = H // 2
    any_spec = pl.BlockSpec(memory_space=pl.ANY)
    return pl.pallas_call(
        functools.partial(_kernel, S=S, M=M, D=D, NP=NP, FF=FF),
        in_specs=[
            any_spec, any_spec, any_spec, any_spec, any_spec, any_spec,
            any_spec, any_spec, any_spec, any_spec,
        ],
        out_specs=any_spec,
        out_shape=jax.ShapeDtypeStruct((1, S, M), BF16),
        scratch_shapes=[
            pltpu.VMEM((S, M), BF16),
            pltpu.VMEM((S, C), BF16),
            pltpu.VMEM((S, M), BF16),
            pltpu.VMEM((S, M), F32),
            pltpu.VMEM((S, M), BF16),
            pltpu.VMEM((2, S, D), BF16),
            pltpu.VMEM((2, S, D), BF16),
            pltpu.VMEM((2, S, D), BF16),
            pltpu.VMEM((2, S, D), BF16),
            pltpu.VMEM((2, M, D), jnp.uint32),
            pltpu.VMEM((2, C, D), jnp.uint32),
            pltpu.VMEM((2, C, D), jnp.uint32),
            pltpu.VMEM((2, 2, D, M), BF16),
            pltpu.VMEM((M,), BF16),
            pltpu.VMEM((M, FF), BF16),
            pltpu.VMEM((M, FF), BF16),
            pltpu.VMEM((FF, M + 128), BF16),
            pltpu.SemaphoreType.DMA((S // XB,)),
            pltpu.SemaphoreType.DMA((S // XB,)),
            pltpu.SemaphoreType.DMA((3, 2)),
            pltpu.SemaphoreType.DMA((2,)),
            pltpu.SemaphoreType.DMA((4,)),
            pltpu.SemaphoreType.DMA((len(EBLOCKS),)),
        ],
        compiler_params=pltpu.CompilerParams(
            vmem_limit_bytes=110 * 1024 * 1024,
            disable_bounds_checks=bool(int(os.environ.get('NOBC', 0))),
        ),
    )(A_x, A_c_kv, A_w_q, A_w_uk, A_w_uv, A_w_o, B_w_r, B_w_gate, B_w_up, B_w_down)
```

```python
import functools
import math
import os

import jax
import jax.numpy as jnp
from jax import lax
import jax.experimental.pallas as pl
import jax.experimental.pallas.tpu as pltpu

F32 = jnp.float32
BF16 = jnp.bfloat16
U32 = jnp.uint32
NEG = -1e30
NT = (((1,), (1,)), ((), ()))
TQ = 512
SUB = 128
GRP = 4
ORDER_MAIN = os.environ.get("ORDER_MAIN", "S03 S13 P03 S02 P13 S12 P02 S01 P12 S11 O3 P01 S00 P11 S10 O2 P00 P10 O1 O0 K03 V03 Q03")
ORDER_LAST = os.environ.get("ORDER_LAST", "S2 S3 P2 S1 P3 S0 P1 P0")
XB = 256
AHEAD = int(os.environ.get('AHEAD', 2))
EBLOCKS = tuple(int(t) for t in os.environ.get('EBLOCKS', '128,128,128,128,128,128,128,128,128,128,128,128,128,128,128,128').split(','))
DCUTS = tuple(int(t) for t in os.environ.get('DCUTS', ','.join(str(i) for i in range(1, 17))).split(','))
RPOS = os.environ.get('RPOS', '02')
RG = len(RPOS)
PONLY = int(os.environ.get('PONLY', 0))
NEWTON = int(os.environ.get('NEWTON', 1))
RLAG = int(os.environ.get('RLAG', 2))
FC = int(os.environ.get('FC', 256))
NF = int(os.environ.get('NF', 2))


def _rb(v):
    return v.astype(BF16).astype(F32)


def _recip(l):
    return pl.reciprocal(l, approx=True)


def _unpack_pair(w32):
    lo = pltpu.bitcast(w32 << 16, F32)
    hi = pltpu.bitcast(w32 & jnp.uint32(0xFFFF0000), F32)
    return jnp.concatenate([lo, hi], axis=1).astype(BF16)


class _Packed:
    def __init__(self, ref):
        self.ref = ref

    @staticmethod
    def half(rows):
        if isinstance(rows, slice):
            return slice(rows.start // 2, rows.stop // 2)
        start, size, align = rows
        return pl.ds(pl.multiple_of(start // 2, align // 2), size // 2)

    def __getitem__(self, idx):
        rows, cols = idx
        return pltpu.bitcast(self.ref[self.half(rows), cols], BF16)

    def __setitem__(self, idx, val):
        rows, cols = idx
        self.ref[self.half(rows), cols] = pltpu.bitcast(val.astype(BF16), U32)


def _qk(q, k, i):
    r0 = i * TQ
    nb = TQ // SUB
    qb = q[r0:r0 + TQ, :]
    s_main = lax.dot_general(qb, k[0:r0 + SUB, :], NT, preferred_element_type=F32)
    s_ext = [lax.dot_general(qb[c * SUB:, :], k[r0 + c * SUB:r0 + (c + 1) * SUB, :], NT,
                             preferred_element_type=F32) for c in range(1, nb)]
    return s_main, s_ext


def _softmax(s, i):
    s_main, s_ext = s
    r0 = i * TQ
    nb = TQ // SUB
    row = lax.broadcasted_iota(jnp.int32, (SUB, SUB), 0)
    col = lax.broadcasted_iota(jnp.int32, (SUB, SUB), 1)
    tri = col <= row
    p_main, p_ext, ls = [], [[] for _ in range(1, nb)], []
    for b in range(nb):
        sm = s_main[b * SUB:(b + 1) * SUB, :]
        if b == 0:
            d = jnp.where(tri, sm[:, r0:], NEG)
            sm = jnp.concatenate([sm[:, :r0], d], axis=1) if r0 > 0 else d
        parts = [sm]
        for c in range(1, b + 1):
            e = s_ext[c - 1][(b - c) * SUB:(b - c + 1) * SUB, :]
            if c == b:
                e = jnp.where(tri, e, NEG)
            parts.append(e)
        sb = jnp.concatenate(parts, axis=1) if len(parts) > 1 else parts[0]
        m = jnp.max(sb, axis=1, keepdims=True)
        p = jnp.exp2(sb - m)
        nt = p.shape[1] // SUB
        tiles = [p[:, t * SUB:(t + 1) * SUB] for t in range(nt)]
        acc = None
        for t0 in range(0, nt, GRP):
            grp = tiles[t0:t0 + GRP]
            tot = grp[0]
            for g in grp[1:]:
                tot = tot + g
            acc = tot if acc is None else acc + tot
            last = t0 + len(grp) - 1
            if acc is not tiles[last]:
                tiles[last] = jnp.minimum(tiles[last], acc)
        p = jnp.concatenate(tiles, axis=1) if nt > 1 else tiles[0]
        ls.append(jnp.sum(acc, axis=1, keepdims=True))
        p_main.append(p[:, :r0 + SUB])
        for c in range(1, b + 1):
            p_ext[c - 1].append(p[:, r0 + c * SUB:r0 + (c + 1) * SUB])
    pm = jnp.concatenate(p_main, axis=0).astype(BF16)
    pe = [(jnp.concatenate(e, axis=0) if len(e) > 1 else e[0]).astype(BF16) for e in p_ext]
    return pm, pe, ls


def _pv(p, v, i):
    pm, pe, ls = p
    r0 = i * TQ
    nb = TQ // SUB
    o = jnp.dot(pm, v[0:r0 + SUB, :], preferred_element_type=F32)
    os_ = [o[b * SUB:(b + 1) * SUB] for b in range(nb)]
    for c in range(1, nb):
        oe = jnp.dot(pe[c - 1], v[r0 + c * SUB:r0 + (c + 1) * SUB, :], preferred_element_type=F32)
        for b in range(c, nb):
            os_[b] = os_[b] + oe[(b - c) * SUB:(b - c + 1) * SUB]
    return jnp.concatenate([os_[b] * _recip(ls[b]) for b in range(nb)], axis=0)


def _attn_pair(q_s, k_s, v_s, order, actions):
    sc, ctx = {}, {}

    def pair_ctx(i):
        return jnp.concatenate([ctx[(0, i)], ctx[(1, i)]], axis=1).astype(BF16)

    for tok in order.split():
        if tok[0] == 'S':
            h, i = int(tok[1]), int(tok[2])
            sc[(h, i)] = _qk(_Packed(q_s.at[h]), _Packed(k_s.at[h]), i)
        elif tok[0] == 'P':
            h, i = int(tok[1]), int(tok[2])
            ctx[(h, i)] = _pv(_softmax(sc.pop((h, i)), i), _Packed(v_s.at[h]), i)
        else:
            actions[tok[0]](int(tok[1:]), pair_ctx)


def _kernel(x_hbm, c_hbm, wq_hbm, wk_hbm, wv_hbm, wo_hbm, wr_hbm, wg_hbm, wu_hbm, wd_hbm,
            out_hbm,
            io_v, c_v, xn_s, acc_s, ctx_s, q_s, k_s, v_s,
            wq_b, wk_b, wv_b, wo_v, wr_ref, wg_v, wu_v, wd_v,
            xsem, csem, wsem, osem_w, fsem, osem,
            *, S, M, D, NP, FF):
    ALL = slice(None)
    xn_p, c_p = _Packed(xn_s), _Packed(c_v)
    scale = (D ** -0.5) * math.log2(math.e)

    def xcopy(b):
        rows = pl.ds(pl.multiple_of(b * XB, XB), XB)
        return pltpu.make_async_copy(x_hbm.at[0, rows, :], io_v.at[rows, :], xsem.at[b])

    def ccopy(b):
        rows = pl.ds(pl.multiple_of(b * (XB // 2), XB // 2), XB // 2)
        return pltpu.make_async_copy(c_hbm.bitcast(U32).at[0, rows, :], c_v.at[rows, :], csem.at[b])

    def wcopies(jj, sl):
        return [
            pltpu.make_async_copy(wk_hbm.bitcast(U32).at[:, jj, :], wk_b.at[sl], wsem.at[0, sl]),
            pltpu.make_async_copy(wv_hbm.bitcast(U32).at[:, jj, :], wv_b.at[sl], wsem.at[1, sl]),
            pltpu.make_async_copy(wq_hbm.bitcast(U32).at[:, jj, :], wq_b.at[sl], wsem.at[2, sl]),
        ]

    def wocopy(t):
        heads = pl.ds(0, 2) if t == 0 else pl.ds(2, 2 * NP - 2)
        return pltpu.make_async_copy(wo_hbm.bitcast(U32).at[heads], wo_v.at[heads], osem_w.at[t])

    def fcopy(t):
        if t == 0:
            return pltpu.make_async_copy(wg_hbm, wg_v, fsem.at[0])
        if t == 1:
            return pltpu.make_async_copy(wu_hbm, wu_v, fsem.at[1])
        if t == 2:
            return pltpu.make_async_copy(wd_hbm, wd_v.at[:, 0:M], fsem.at[2])
        return pltpu.make_async_copy(wr_hbm, wr_ref, fsem.at[3])

    def ocopy(g):
        r0 = sum(EBLOCKS[:DCUTS[g - 1]]) if g > 0 else 0
        rows = pl.ds(r0, sum(EBLOCKS[:DCUTS[g]]) - r0)
        return pltpu.make_async_copy(io_v.at[rows, :], out_hbm.at[0, rows, :], osem.at[g])

    def project(dst, lhs, w32, rows, mult=None):
        y = jnp.dot(lhs, _unpack_pair(w32), preferred_element_type=F32)
        if mult is not None:
            y = y * mult
        _Packed(dst.at[0])[rows, ALL] = y[:, :D]
        _Packed(dst.at[1])[rows, ALL] = y[:, D:]

    NXB = S // XB
    for cp in wcopies(0, 0):
        cp.start()
    ccopy(0).start()
    xcopy(0).start()
    for cp in wcopies(0, 0):
        cp.wait()
    for b in range(1, AHEAD):
        ccopy(b).start()
        xcopy(b).start()
    wocopy(0).start()

    def first(b, carry):
        ccopy(b).wait()
        xcopy(b).wait()

        @pl.when(b + AHEAD < NXB)
        def _():
            ccopy(b + AHEAD).start()
            xcopy(b + AHEAD).start()

        @pl.when(b + AHEAD == NXB)
        def _():
            fcopy(3).start()
            for cp in wcopies(1, 1):
                cp.start()

        rows = pl.ds(pl.multiple_of(b * XB, XB), XB)
        xf = io_v[rows, :].astype(F32)
        mu = jnp.mean(xf, axis=1, keepdims=True)
        xc = xf - mu
        var = jnp.mean(xc * xc, axis=1, keepdims=True)
        xn = (xc * lax.rsqrt(var + 1e-5)).astype(BF16)
        prow = (b * XB, XB, XB)
        xn_p[prow, ALL] = xn
        acc_s[rows, :] = xf
        c = c_p[prow, ALL]
        project(k_s, c, wk_b[0], prow)
        project(v_s, c, wv_b[0], prow)
        project(q_s, xn, wq_b[0], prow, scale)
        return carry
    lax.fori_loop(0, S // XB, first, 0)
    wocopy(1).start()
    wocopy(0).wait()

    def step(j, carry):
        slot = j % 2

        @pl.when(j == 1)
        def _():
            wocopy(1).wait()

        for cp in wcopies(j + 1, 1 - slot):
            cp.wait()

        @pl.when(j + 2 < NP)
        def _():
            for cp in wcopies(j + 2, slot):
                cp.start()

        for t in range(3):
            @pl.when(j == 2 * t + 1)
            def _():
                fcopy(t).start()

        wo = pltpu.bitcast(wo_v[pl.ds(2 * j, 2)].reshape(D, M), BF16)

        def oproj(ii, pair_ctx):
            acc_s[ii * TQ:(ii + 1) * TQ, :] += jnp.dot(pair_ctx(ii), wo, preferred_element_type=F32)

        def rows_of(code):
            return slice((code // 10) * TQ, (code % 10 + 1) * TQ)

        _attn_pair(q_s, k_s, v_s, ORDER_MAIN, {
            'O': oproj,
            'K': lambda code, _: project(k_s, c_p[rows_of(code), ALL], wk_b[1 - slot], rows_of(code)),
            'V': lambda code, _: project(v_s, c_p[rows_of(code), ALL], wv_b[1 - slot], rows_of(code)),
            'Q': lambda code, _: project(q_s, xn_p[rows_of(code), ALL], wq_b[1 - slot], rows_of(code), scale),
        })
        return carry
    lax.fori_loop(0, NP - 1, step, 0)

    fcopy(3).wait()
    if PONLY:
        return
    eps = jnp.asarray(1e-5, BF16).astype(F32)

    def last_head(h, carry):
        sc = {}
        for tok in ORDER_LAST.split():
            i = int(tok[1])
            if tok[0] == 'S':
                sc[i] = _qk(_Packed(q_s.at[h]), _Packed(k_s.at[h]), i)
            else:
                _Packed(ctx_s.at[h])[slice(i * TQ, (i + 1) * TQ), ALL] = _pv(
                    _softmax(sc.pop(i), i), _Packed(v_s.at[h]), i)
        return carry
    lax.fori_loop(0, 2, last_head, 0)

    NCH = 4
    CW = M // NCH
    RW = M // RG
    wr16 = [jnp.broadcast_to(wr_ref[t * RW:(t + 1) * RW].astype(F32).reshape(1, RW), (16, RW)).astype(BF16)
            for t in range(RG)]

    def oproj_part(r0, n, t):
        rows = slice(r0, r0 + n)
        cols = slice(t * CW, (t + 1) * CW)
        return (acc_s[rows, cols]
                + jnp.dot(_Packed(ctx_s.at[0])[rows, ALL], pltpu.bitcast(wo_v[2 * NP - 2, :, cols], BF16),
                           preferred_element_type=F32)
                + jnp.dot(_Packed(ctx_s.at[1])[rows, ALL], pltpu.bitcast(wo_v[2 * NP - 1, :, cols], BF16),
                           preferred_element_type=F32))

    def ln2(r0, n, h):
        rows = slice(r0, r0 + n)
        acc_s[rows, :] = h
        mu = jnp.mean(h, axis=1, keepdims=True)
        mub = _rb(mu)
        d = acc_s[rows, :] - mub
        dm = mu - mub
        var = jnp.maximum(jnp.mean(d * d, axis=1, keepdims=True) - dm * dm, 0.0)
        ve = _rb(_rb(var) + eps)
        den = _rb(ve * lax.rsqrt(ve))
        h = acc_s[rows, :]
        inv = _recip(den)
        if NEWTON:
            inv = inv * (2.0 - den * inv)
        ln = (h - mub) * inv
        xn_p[rows, ALL] = ln
        io_v[rows, :] = (h + ln).astype(BF16)

    def router_part(r0, n, t):
        cols = slice(t * RW, (t + 1) * RW)
        return lax.dot_general(wr16[t], xn_p[slice(r0, r0 + n), cols], NT, preferred_element_type=F32)

    blocks = []
    r0 = 0
    for n in EBLOCKS:
        blocks.append((r0, n))
        r0 += n
    assert r0 == S
    rparts = []
    for k in range(len(blocks) + RLAG):
        hp, rp = [], None
        for t in range(NCH):
            if k < len(blocks):
                hp.append(oproj_part(*blocks[k], t))
            if k >= RLAG and str(t) in RPOS:
                part = router_part(*blocks[k - RLAG], RPOS.index(str(t)))
                rp = part if rp is None else rp + part
        if k in DCUTS:
            ocopy(DCUTS.index(k)).start()
        if k < len(blocks):
            ln2(*blocks[k], jnp.concatenate(hp, axis=1))
        if k >= RLAG:
            rparts.append(rp[0:8, :])
    rrow = _rb(jnp.concatenate(rparts, axis=1))

    I32 = jnp.int32
    b16 = lax.shift_right_logical(pltpu.bitcast(rrow, I32), 16)
    rank = jnp.where(b16 >= 0x8000, 0x10000 - b16, 0x8000 + b16)
    lane = lax.broadcasted_iota(I32, rrow.shape, 1)
    key = pltpu.bitcast(rank * S + (S - 1 - lane) + 0x20000000, F32)
    k1 = jnp.max(key, axis=1, keepdims=True)
    k2 = jnp.max(jnp.where(key == k1, 0.0, key), axis=1, keepdims=True)
    i1 = (S - 1) - (pltpu.bitcast(k1, I32)[0, 0] & (S - 1))
    i2 = (S - 1) - (pltpu.bitcast(k2, I32)[0, 0] & (S - 1))
    m1 = jnp.max(jnp.where(key == k1, rrow, -jnp.inf), axis=1, keepdims=True)[0:1, :]
    m2 = jnp.max(jnp.where(key == k2, rrow, -jnp.inf), axis=1, keepdims=True)[0:1, :]
    g1 = pl.multiple_of((i1 // 16) * 16, 16)
    g2 = pl.multiple_of((i2 // 16) * 16, 16)

    rid = lax.broadcasted_iota(jnp.int32, (16, M), 0)

    def pick(g, i):
        blk = xn_p[(g, 16, 16), ALL].astype(F32)
        return jnp.sum(jnp.where(rid == i - g, blk, 0.0), axis=0, keepdims=True)

    xs = jnp.where(rid == 0, pick(g1, i1), pick(g2, i2))
    xsb = xs.astype(BF16)
    for t in range(3):
        fcopy(t).wait()
    FH = FF // NF

    def ffn(o, y):
        nch = FH // FC
        acts = []
        for t in range(nch + 1):
            if t < nch:
                cols = pl.ds(pl.multiple_of(o * FH + t * FC, 128), FC)
                a = _rb(jnp.dot(xsb, wg_v[:, cols], preferred_element_type=F32))
                u = _rb(jnp.dot(xsb, wu_v[:, cols], preferred_element_type=F32))
                g = _rb(a * _rb(jax.nn.sigmoid(a)))
                acts.append((g * u).astype(BF16))
            if t > 0:
                rws = pl.ds(pl.multiple_of(o * FH + (t - 1) * FC, 128), FC)
                y = y + jnp.dot(acts[t - 1], wd_v[rws, 0:M], preferred_element_type=F32)
        return y
    y = lax.fori_loop(0, NF, ffn, jnp.zeros((16, M), F32))
    rsel = jnp.where(rid == 0, m1, m2)
    y = _rb(_rb(y) * _rb(jax.nn.sigmoid(rsel)))
    upd = _rb(xs + y)

    for b in range(len(DCUTS)):
        ocopy(b).wait()
    for (ii, gg, rr) in ((i1, g1, 0), (i2, g2, 1)):
        new = _rb(acc_s[pl.ds(gg, 16), :]) + upd[rr:rr + 1, :]
        cur = io_v[pl.ds(gg, 16), :].astype(F32)
        io_v[pl.ds(gg, 16), :] = jnp.where(rid == ii - gg, new, cur).astype(BF16)

    def pcopy(g, k):
        return pltpu.make_async_copy(io_v.at[pl.ds(g, 16), :], out_hbm.at[0, pl.ds(g, 16), :], osem.at[k])

    pcopy(g1, 0).start()

    @pl.when(g2 != g1)
    def _():
        pcopy(g2, 1).start()
        pcopy(g2, 1).wait()
    pcopy(g1, 0).wait()


@jax.jit
def pallas_sequential_preLN__compressed_kv_cla__moe_arch_mod__prompt_kernel(
    A_x: jax.Array,
    A_c_kv: jax.Array,
    A_w_q: jax.Array,
    A_w_uk: jax.Array,
    A_w_uv: jax.Array,
    A_w_o: jax.Array,
    B_x: jax.Array,
    B_w_r: jax.Array,
    B_w_gate: jax.Array,
    B_w_up: jax.Array,
    B_w_down: jax.Array,
):
    _, S, M = A_x.shape
    C = A_c_kv.shape[2]
    H, D = A_w_q.shape[1], A_w_q.shape[2]
    FF = B_w_gate.shape[1]
    NP = H // 2
    any_spec = pl.BlockSpec(memory_space=pl.ANY)
    return pl.pallas_call(
        functools.partial(_kernel, S=S, M=M, D=D, NP=NP, FF=FF),
        in_specs=[
            any_spec, any_spec, any_spec, any_spec, any_spec, any_spec,
            any_spec, any_spec, any_spec, any_spec,
        ],
        out_specs=any_spec,
        out_shape=jax.ShapeDtypeStruct((1, S, M), BF16),
        scratch_shapes=[
            pltpu.VMEM((S, M), BF16),
            pltpu.VMEM((S // 2, C), U32),
            pltpu.VMEM((S // 2, M), U32),
            pltpu.VMEM((S, M), F32),
            pltpu.VMEM((2, S // 2, D), U32),
            pltpu.VMEM((2, S // 2, D), U32),
            pltpu.VMEM((2, S // 2, D), U32),
            pltpu.VMEM((2, S // 2, D), U32),
            pltpu.VMEM((2, M, D), U32),
            pltpu.VMEM((2, C, D), U32),
            pltpu.VMEM((2, C, D), U32),
            pltpu.VMEM((H, D // 2, M), U32),
            pltpu.VMEM((M,), BF16),
            pltpu.VMEM((M, FF), BF16),
            pltpu.VMEM((M, FF), BF16),
            pltpu.VMEM((FF, M + 128), BF16),
            pltpu.SemaphoreType.DMA((S // XB,)),
            pltpu.SemaphoreType.DMA((S // XB,)),
            pltpu.SemaphoreType.DMA((3, 2)),
            pltpu.SemaphoreType.DMA((2,)),
            pltpu.SemaphoreType.DMA((4,)),
            pltpu.SemaphoreType.DMA((max(len(DCUTS), 2),)),
        ],
        compiler_params=pltpu.CompilerParams(
            vmem_limit_bytes=110 * 1024 * 1024,
            disable_bounds_checks=bool(int(os.environ.get('NOBC', 0))),
        ),
    )(A_x, A_c_kv, A_w_q, A_w_uk, A_w_uv, A_w_o, B_w_r, B_w_gate, B_w_up, B_w_down)
```

```python
import functools
import math
import os

import jax
import jax.numpy as jnp
from jax import lax
import jax.experimental.pallas as pl
import jax.experimental.pallas.tpu as pltpu

F32 = jnp.float32
BF16 = jnp.bfloat16
U32 = jnp.uint32
NEG = -1e30
NT = (((1,), (1,)), ((), ()))
TQ = 512
SUB = 128
GRP = 4
ORDER_MAIN = os.environ.get("ORDER_MAIN", "S03 S13 P03 S02 P13 S12 P02 S01 P12 S11 O3 P01 S00 P11 S10 O2 P00 P10 O1 O0 K03 V03 Q03")
ORDER_LAST = os.environ.get("ORDER_LAST", "S2 S3 P2 S1 P3 S0 P1 P0")
XB = 256
AHEAD = int(os.environ.get('AHEAD', 2))
EBLOCKS = tuple(int(t) for t in os.environ.get('EBLOCKS', '128,128,128,128,128,128,128,128,128,128,128,128,128,128,128,128').split(','))
DCUTS = tuple(int(t) for t in os.environ.get('DCUTS', ','.join(str(i) for i in range(1, 17))).split(','))
RPOS = os.environ.get('RPOS', '02')
RG = len(RPOS)
PONLY = int(os.environ.get('PONLY', 0))
NEWTON = int(os.environ.get('NEWTON', 1))
RLAG = int(os.environ.get('RLAG', 2))
FC = int(os.environ.get('FC', 256))
NF = int(os.environ.get('NF', 2))


def _rb(v):
    return v.astype(BF16).astype(F32)


def _recip(l):
    return pl.reciprocal(l, approx=True)


def _unpack_pair(w32):
    lo = pltpu.bitcast(w32 << 16, F32)
    hi = pltpu.bitcast(w32 & jnp.uint32(0xFFFF0000), F32)
    return jnp.concatenate([lo, hi], axis=1).astype(BF16)


class _Packed:
    def __init__(self, ref):
        self.ref = ref

    @staticmethod
    def half(rows):
        if isinstance(rows, slice):
            return slice(rows.start // 2, rows.stop // 2)
        start, size, align = rows
        return pl.ds(pl.multiple_of(start // 2, align // 2), size // 2)

    def __getitem__(self, idx):
        rows, cols = idx
        return pltpu.bitcast(self.ref[self.half(rows), cols], BF16)

    def __setitem__(self, idx, val):
        rows, cols = idx
        self.ref[self.half(rows), cols] = pltpu.bitcast(val.astype(BF16), U32)


def _qk(q, k, i):
    r0 = i * TQ
    nb = TQ // SUB
    qb = q[r0:r0 + TQ, :]
    s_main = lax.dot_general(qb, k[0:r0 + SUB, :], NT, preferred_element_type=F32)
    s_ext = [lax.dot_general(qb[c * SUB:, :], k[r0 + c * SUB:r0 + (c + 1) * SUB, :], NT,
                             preferred_element_type=F32) for c in range(1, nb)]
    return s_main, s_ext


def _softmax(s, i):
    s_main, s_ext = s
    r0 = i * TQ
    nb = TQ // SUB
    row = lax.broadcasted_iota(jnp.int32, (SUB, SUB), 0)
    col = lax.broadcasted_iota(jnp.int32, (SUB, SUB), 1)
    tri = col <= row
    p_main, p_ext, ls = [], [[] for _ in range(1, nb)], []
    for b in range(nb):
        sm = s_main[b * SUB:(b + 1) * SUB, :]
        if b == 0:
            d = jnp.where(tri, sm[:, r0:], NEG)
            sm = jnp.concatenate([sm[:, :r0], d], axis=1) if r0 > 0 else d
        parts = [sm]
        for c in range(1, b + 1):
            e = s_ext[c - 1][(b - c) * SUB:(b - c + 1) * SUB, :]
            if c == b:
                e = jnp.where(tri, e, NEG)
            parts.append(e)
        sb = jnp.concatenate(parts, axis=1) if len(parts) > 1 else parts[0]
        m = jnp.max(sb, axis=1, keepdims=True)
        p = jnp.exp2(sb - m)
        nt = p.shape[1] // SUB
        tiles = [p[:, t * SUB:(t + 1) * SUB] for t in range(nt)]
        acc = None
        for t0 in range(0, nt, GRP):
            grp = tiles[t0:t0 + GRP]
            tot = grp[0]
            for g in grp[1:]:
                tot = tot + g
            acc = tot if acc is None else acc + tot
            last = t0 + len(grp) - 1
            if acc is not tiles[last]:
                tiles[last] = jnp.minimum(tiles[last], acc)
        p = jnp.concatenate(tiles, axis=1) if nt > 1 else tiles[0]
        ls.append(jnp.sum(acc, axis=1, keepdims=True))
        p_main.append(p[:, :r0 + SUB])
        for c in range(1, b + 1):
            p_ext[c - 1].append(p[:, r0 + c * SUB:r0 + (c + 1) * SUB])
    pm = jnp.concatenate(p_main, axis=0).astype(BF16)
    pe = [(jnp.concatenate(e, axis=0) if len(e) > 1 else e[0]).astype(BF16) for e in p_ext]
    return pm, pe, ls


def _pv(p, v, i):
    pm, pe, ls = p
    r0 = i * TQ
    nb = TQ // SUB
    o = jnp.dot(pm, v[0:r0 + SUB, :], preferred_element_type=F32)
    os_ = [o[b * SUB:(b + 1) * SUB] for b in range(nb)]
    for c in range(1, nb):
        oe = jnp.dot(pe[c - 1], v[r0 + c * SUB:r0 + (c + 1) * SUB, :], preferred_element_type=F32)
        for b in range(c, nb):
            os_[b] = os_[b] + oe[(b - c) * SUB:(b - c + 1) * SUB]
    return jnp.concatenate([os_[b] * _recip(ls[b]) for b in range(nb)], axis=0)


def _attn_pair(q_s, k_s, v_s, order, actions):
    sc, ctx = {}, {}

    def pair_ctx(i):
        return jnp.concatenate([ctx[(0, i)], ctx[(1, i)]], axis=1).astype(BF16)

    for tok in order.split():
        if tok[0] == 'S':
            h, i = int(tok[1]), int(tok[2])
            sc[(h, i)] = _qk(_Packed(q_s.at[h]), _Packed(k_s.at[h]), i)
        elif tok[0] == 'P':
            h, i = int(tok[1]), int(tok[2])
            ctx[(h, i)] = _pv(_softmax(sc.pop((h, i)), i), _Packed(v_s.at[h]), i)
        else:
            actions[tok[0]](int(tok[1:]), pair_ctx)


def _kernel(x_hbm, c_hbm, wq_hbm, wk_hbm, wv_hbm, wo_hbm, wr_hbm, wg_hbm, wu_hbm, wd_hbm,
            out_hbm,
            io_v, c_v, xn_s, acc_s, ctx_s, q_s, k_s, v_s,
            wq_b, wk_b, wv_b, wo_v, wr_ref, wg_v, wu_v, wd_v,
            xsem, csem, wsem, osem_w, fsem, osem,
            *, S, M, D, NP, FF):
    ALL = slice(None)
    xn_p, c_p = _Packed(xn_s), _Packed(c_v)
    scale = (D ** -0.5) * math.log2(math.e)

    def xcopy(b):
        rows = pl.ds(pl.multiple_of(b * XB, XB), XB)
        return pltpu.make_async_copy(x_hbm.at[0, rows, :], io_v.at[rows, :], xsem.at[b])

    def ccopy(b):
        rows = pl.ds(pl.multiple_of(b * (XB // 2), XB // 2), XB // 2)
        return pltpu.make_async_copy(c_hbm.bitcast(U32).at[0, rows, :], c_v.at[rows, :], csem.at[b])

    def wcopies(jj, sl):
        return [
            pltpu.make_async_copy(wk_hbm.bitcast(U32).at[:, jj, :], wk_b.at[sl], wsem.at[0, sl]),
            pltpu.make_async_copy(wv_hbm.bitcast(U32).at[:, jj, :], wv_b.at[sl], wsem.at[1, sl]),
            pltpu.make_async_copy(wq_hbm.bitcast(U32).at[:, jj, :], wq_b.at[sl], wsem.at[2, sl]),
        ]

    def wocopy(t):
        heads = pl.ds(0, 2) if t == 0 else pl.ds(2, 2 * NP - 2)
        return pltpu.make_async_copy(wo_hbm.bitcast(U32).at[heads], wo_v.at[heads], osem_w.at[t])

    def fcopy(t):
        if t == 0:
            return pltpu.make_async_copy(wg_hbm, wg_v, fsem.at[0])
        if t == 1:
            return pltpu.make_async_copy(wu_hbm, wu_v, fsem.at[1])
        if t == 2:
            return pltpu.make_async_copy(wd_hbm, wd_v.at[:, 0:M], fsem.at[2])
        return pltpu.make_async_copy(wr_hbm, wr_ref, fsem.at[3])

    def ocopy(g):
        r0 = sum(EBLOCKS[:DCUTS[g - 1]]) if g > 0 else 0
        rows = pl.ds(r0, sum(EBLOCKS[:DCUTS[g]]) - r0)
        return pltpu.make_async_copy(io_v.at[rows, :], out_hbm.at[0, rows, :], osem.at[g])

    def project(dst, lhs, w32, rows, mult=None):
        y = jnp.dot(lhs, _unpack_pair(w32), preferred_element_type=F32)
        if mult is not None:
            y = y * mult
        _Packed(dst.at[0])[rows, ALL] = y[:, :D]
        _Packed(dst.at[1])[rows, ALL] = y[:, D:]

    NXB = S // XB
    for cp in wcopies(0, 0):
        cp.start()
    ccopy(0).start()
    xcopy(0).start()
    for cp in wcopies(0, 0):
        cp.wait()
    for b in range(1, AHEAD):
        ccopy(b).start()
        xcopy(b).start()

    def first(b, carry):
        ccopy(b).wait()
        xcopy(b).wait()

        @pl.when(b + AHEAD < NXB)
        def _():
            ccopy(b + AHEAD).start()
            xcopy(b + AHEAD).start()

        @pl.when(b + AHEAD == NXB)
        def _():
            wocopy(0).start()
            fcopy(3).start()
            for cp in wcopies(1, 1):
                cp.start()

        rows = pl.ds(pl.multiple_of(b * XB, XB), XB)
        xf = io_v[rows, :].astype(F32)
        mu = jnp.mean(xf, axis=1, keepdims=True)
        xc = xf - mu
        var = jnp.mean(xc * xc, axis=1, keepdims=True)
        xn = (xc * lax.rsqrt(var + 1e-5)).astype(BF16)
        prow = (b * XB, XB, XB)
        xn_p[prow, ALL] = xn
        acc_s[rows, :] = xf
        c = c_p[prow, ALL]
        project(k_s, c, wk_b[0], prow)
        project(v_s, c, wv_b[0], prow)
        project(q_s, xn, wq_b[0], prow, scale)
        return carry
    lax.fori_loop(0, S // XB, first, 0)
    for cp in wcopies(2, 0):
        cp.start()
    wocopy(1).start()
    for t in range(3):
        fcopy(t).start()
    wocopy(0).wait()

    def step(j, carry):
        slot = j % 2

        @pl.when(j == 1)
        def _():
            wocopy(1).wait()

        for cp in wcopies(j + 1, 1 - slot):
            cp.wait()

        @pl.when(jnp.logical_and(j >= 1, j + 2 < NP))
        def _():
            for cp in wcopies(j + 2, slot):
                cp.start()

        wo = pltpu.bitcast(wo_v[pl.ds(2 * j, 2)].reshape(D, M), BF16)

        def oproj(ii, pair_ctx):
            acc_s[ii * TQ:(ii + 1) * TQ, :] += jnp.dot(pair_ctx(ii), wo, preferred_element_type=F32)

        def rows_of(code):
            return slice((code // 10) * TQ, (code % 10 + 1) * TQ)

        _attn_pair(q_s, k_s, v_s, ORDER_MAIN, {
            'O': oproj,
            'K': lambda code, _: project(k_s, c_p[rows_of(code), ALL], wk_b[1 - slot], rows_of(code)),
            'V': lambda code, _: project(v_s, c_p[rows_of(code), ALL], wv_b[1 - slot], rows_of(code)),
            'Q': lambda code, _: project(q_s, xn_p[rows_of(code), ALL], wq_b[1 - slot], rows_of(code), scale),
        })
        return carry
    lax.fori_loop(0, NP - 1, step, 0)

    fcopy(3).wait()
    if PONLY:
        return
    eps = jnp.asarray(1e-5, BF16).astype(F32)

    def last_head(h, carry):
        sc = {}
        for tok in ORDER_LAST.split():
            i = int(tok[1])
            if tok[0] == 'S':
                sc[i] = _qk(_Packed(q_s.at[h]), _Packed(k_s.at[h]), i)
            else:
                _Packed(ctx_s.at[h])[slice(i * TQ, (i + 1) * TQ), ALL] = _pv(
                    _softmax(sc.pop(i), i), _Packed(v_s.at[h]), i)
        return carry
    lax.fori_loop(0, 2, last_head, 0)

    NCH = 4
    CW = M // NCH
    RW = M // RG
    wr16 = [jnp.broadcast_to(wr_ref[t * RW:(t + 1) * RW].astype(F32).reshape(1, RW), (16, RW)).astype(BF16)
            for t in range(RG)]

    def oproj_part(r0, n, t):
        rows = slice(r0, r0 + n)
        cols = slice(t * CW, (t + 1) * CW)
        return (acc_s[rows, cols]
                + jnp.dot(_Packed(ctx_s.at[0])[rows, ALL], pltpu.bitcast(wo_v[2 * NP - 2, :, cols], BF16),
                           preferred_element_type=F32)
                + jnp.dot(_Packed(ctx_s.at[1])[rows, ALL], pltpu.bitcast(wo_v[2 * NP - 1, :, cols], BF16),
                           preferred_element_type=F32))

    def ln2(r0, n, h):
        rows = slice(r0, r0 + n)
        acc_s[rows, :] = h
        mu = jnp.mean(h, axis=1, keepdims=True)
        mub = _rb(mu)
        d = acc_s[rows, :] - mub
        dm = mu - mub
        var = jnp.maximum(jnp.mean(d * d, axis=1, keepdims=True) - dm * dm, 0.0)
        ve = _rb(_rb(var) + eps)
        den = _rb(ve * lax.rsqrt(ve))
        h = acc_s[rows, :]
        inv = _recip(den)
        if NEWTON:
            inv = inv * (2.0 - den * inv)
        ln = (h - mub) * inv
        xn_p[rows, ALL] = ln
        io_v[rows, :] = (h + ln).astype(BF16)

    def router_part(r0, n, t):
        cols = slice(t * RW, (t + 1) * RW)
        return lax.dot_general(wr16[t], xn_p[slice(r0, r0 + n), cols], NT, preferred_element_type=F32)

    blocks = []
    r0 = 0
    for n in EBLOCKS:
        blocks.append((r0, n))
        r0 += n
    assert r0 == S
    rparts = []
    for k in range(len(blocks) + RLAG):
        hp, rp = [], None
        for t in range(NCH):
            if k < len(blocks):
                hp.append(oproj_part(*blocks[k], t))
            if k >= RLAG and str(t) in RPOS:
                part = router_part(*blocks[k - RLAG], RPOS.index(str(t)))
                rp = part if rp is None else rp + part
        if k in DCUTS:
            ocopy(DCUTS.index(k)).start()
        if k < len(blocks):
            ln2(*blocks[k], jnp.concatenate(hp, axis=1))
        if k >= RLAG:
            rparts.append(rp[0:8, :])
    rrow = _rb(jnp.concatenate(rparts, axis=1))

    I32 = jnp.int32
    b16 = lax.shift_right_logical(pltpu.bitcast(rrow, I32), 16)
    rank = jnp.where(b16 >= 0x8000, 0x10000 - b16, 0x8000 + b16)
    lane = lax.broadcasted_iota(I32, rrow.shape, 1)
    key = pltpu.bitcast(rank * S + (S - 1 - lane) + 0x20000000, F32)
    k1 = jnp.max(key, axis=1, keepdims=True)
    k2 = jnp.max(jnp.where(key == k1, 0.0, key), axis=1, keepdims=True)
    i1 = (S - 1) - (pltpu.bitcast(k1, I32)[0, 0] & (S - 1))
    i2 = (S - 1) - (pltpu.bitcast(k2, I32)[0, 0] & (S - 1))
    m1 = jnp.max(jnp.where(key == k1, rrow, -jnp.inf), axis=1, keepdims=True)[0:1, :]
    m2 = jnp.max(jnp.where(key == k2, rrow, -jnp.inf), axis=1, keepdims=True)[0:1, :]
    g1 = pl.multiple_of((i1 // 16) * 16, 16)
    g2 = pl.multiple_of((i2 // 16) * 16, 16)

    rid = lax.broadcasted_iota(jnp.int32, (16, M), 0)

    def pick(g, i):
        blk = xn_p[(g, 16, 16), ALL].astype(F32)
        return jnp.sum(jnp.where(rid == i - g, blk, 0.0), axis=0, keepdims=True)

    xs = jnp.where(rid == 0, pick(g1, i1), pick(g2, i2))
    xsb = xs.astype(BF16)
    for t in range(3):
        fcopy(t).wait()
    FH = FF // NF

    def ffn(o, y):
        nch = FH // FC
        acts = []
        for t in range(nch + 1):
            if t < nch:
                cols = pl.ds(pl.multiple_of(o * FH + t * FC, 128), FC)
                a = _rb(jnp.dot(xsb, wg_v[:, cols], preferred_element_type=F32))
                u = _rb(jnp.dot(xsb, wu_v[:, cols], preferred_element_type=F32))
                g = _rb(a * _rb(jax.nn.sigmoid(a)))
                acts.append((g * u).astype(BF16))
            if t > 0:
                rws = pl.ds(pl.multiple_of(o * FH + (t - 1) * FC, 128), FC)
                y = y + jnp.dot(acts[t - 1], wd_v[rws, 0:M], preferred_element_type=F32)
        return y
    y = lax.fori_loop(0, NF, ffn, jnp.zeros((16, M), F32))
    rsel = jnp.where(rid == 0, m1, m2)
    y = _rb(_rb(y) * _rb(jax.nn.sigmoid(rsel)))
    upd = _rb(xs + y)

    for b in range(len(DCUTS)):
        ocopy(b).wait()
    for (ii, gg, rr) in ((i1, g1, 0), (i2, g2, 1)):
        new = _rb(acc_s[pl.ds(gg, 16), :]) + upd[rr:rr + 1, :]
        cur = io_v[pl.ds(gg, 16), :].astype(F32)
        io_v[pl.ds(gg, 16), :] = jnp.where(rid == ii - gg, new, cur).astype(BF16)

    def pcopy(g, k):
        return pltpu.make_async_copy(io_v.at[pl.ds(g, 16), :], out_hbm.at[0, pl.ds(g, 16), :], osem.at[k])

    pcopy(g1, 0).start()

    @pl.when(g2 != g1)
    def _():
        pcopy(g2, 1).start()
        pcopy(g2, 1).wait()
    pcopy(g1, 0).wait()


@jax.jit
def pallas_sequential_preLN__compressed_kv_cla__moe_arch_mod__prompt_kernel(
    A_x: jax.Array,
    A_c_kv: jax.Array,
    A_w_q: jax.Array,
    A_w_uk: jax.Array,
    A_w_uv: jax.Array,
    A_w_o: jax.Array,
    B_x: jax.Array,
    B_w_r: jax.Array,
    B_w_gate: jax.Array,
    B_w_up: jax.Array,
    B_w_down: jax.Array,
):
    _, S, M = A_x.shape
    C = A_c_kv.shape[2]
    H, D = A_w_q.shape[1], A_w_q.shape[2]
    FF = B_w_gate.shape[1]
    NP = H // 2
    any_spec = pl.BlockSpec(memory_space=pl.ANY)
    return pl.pallas_call(
        functools.partial(_kernel, S=S, M=M, D=D, NP=NP, FF=FF),
        in_specs=[
            any_spec, any_spec, any_spec, any_spec, any_spec, any_spec,
            any_spec, any_spec, any_spec, any_spec,
        ],
        out_specs=any_spec,
        out_shape=jax.ShapeDtypeStruct((1, S, M), BF16),
        scratch_shapes=[
            pltpu.VMEM((S, M), BF16),
            pltpu.VMEM((S // 2, C), U32),
            pltpu.VMEM((S // 2, M), U32),
            pltpu.VMEM((S, M), F32),
            pltpu.VMEM((2, S // 2, D), U32),
            pltpu.VMEM((2, S // 2, D), U32),
            pltpu.VMEM((2, S // 2, D), U32),
            pltpu.VMEM((2, S // 2, D), U32),
            pltpu.VMEM((2, M, D), U32),
            pltpu.VMEM((2, C, D), U32),
            pltpu.VMEM((2, C, D), U32),
            pltpu.VMEM((H, D // 2, M), U32),
            pltpu.VMEM((M,), BF16),
            pltpu.VMEM((M, FF), BF16),
            pltpu.VMEM((M, FF), BF16),
            pltpu.VMEM((FF, M + 128), BF16),
            pltpu.SemaphoreType.DMA((S // XB,)),
            pltpu.SemaphoreType.DMA((S // XB,)),
            pltpu.SemaphoreType.DMA((3, 2)),
            pltpu.SemaphoreType.DMA((2,)),
            pltpu.SemaphoreType.DMA((4,)),
            pltpu.SemaphoreType.DMA((max(len(DCUTS), 2),)),
        ],
        compiler_params=pltpu.CompilerParams(
            vmem_limit_bytes=110 * 1024 * 1024,
            disable_bounds_checks=bool(int(os.environ.get('NOBC', 1))),
        ),
    )(A_x, A_c_kv, A_w_q, A_w_uk, A_w_uv, A_w_o, B_w_r, B_w_gate, B_w_up, B_w_down)
```

```python
import functools
import math
import os

import jax
import jax.numpy as jnp
from jax import lax
import jax.experimental.pallas as pl
import jax.experimental.pallas.tpu as pltpu

F32 = jnp.float32
BF16 = jnp.bfloat16
U32 = jnp.uint32
NEG = -1e30
NT = (((1,), (1,)), ((), ()))
TQ = 512
SUB = 128
GRP = 4
ORDER_MAIN = os.environ.get("ORDER_MAIN", "S03 S13 P03 K33 S02 P13 S12 P02 S01 P12 S11 Q23 S00 P01 P11 S10 K02 P00 P10 O3 Q01 O2 O1 O0 V03")
ORDER_LAST = os.environ.get("ORDER_LAST", "S2 S3 P2 S1 P3 S0 P1 P0")
XB = 256
EBLOCKS = tuple(int(t) for t in os.environ.get('EBLOCKS', '128,128,128,128,128,128,128,128,128,128,128,128,128,128,128,128').split(','))
DCUTS = tuple(int(t) for t in os.environ.get('DCUTS', '2,4,6,8,10,12,14,16').split(','))
RPOS = os.environ.get('RPOS', '01')
RG = len(RPOS)
PONLY = int(os.environ.get('PONLY', 0))
RLAG = int(os.environ.get('RLAG', 2))
FC = int(os.environ.get('FC', 512))
NF = int(os.environ.get('NF', 1))


def _rb(v):
    return v.astype(BF16).astype(F32)


def _recip(l):
    return pl.reciprocal(l, approx=True)


def _unpack_pair(w32):
    lo = pltpu.bitcast(w32 << 16, F32)
    hi = pltpu.bitcast(w32 & jnp.uint32(0xFFFF0000), F32)
    return jnp.concatenate([lo, hi], axis=1).astype(BF16)


class _Packed:
    def __init__(self, ref):
        self.ref = ref

    @staticmethod
    def half(rows):
        if isinstance(rows, slice):
            return slice(rows.start // 2, rows.stop // 2)
        start, size, align = rows
        return pl.ds(pl.multiple_of(start // 2, align // 2), size // 2)

    def __getitem__(self, idx):
        rows, cols = idx
        return pltpu.bitcast(self.ref[self.half(rows), cols], BF16)

    def __setitem__(self, idx, val):
        rows, cols = idx
        self.ref[self.half(rows), cols] = pltpu.bitcast(val.astype(BF16), U32)


def _qk(q, k, i):
    r0 = i * TQ
    nb = TQ // SUB
    qb = q[r0:r0 + TQ, :]
    s_main = lax.dot_general(qb, k[0:r0 + SUB, :], NT, preferred_element_type=F32)
    s_ext = [lax.dot_general(qb[c * SUB:, :], k[r0 + c * SUB:r0 + (c + 1) * SUB, :], NT,
                             preferred_element_type=F32) for c in range(1, nb)]
    return s_main, s_ext


def _softmax(s, i):
    s_main, s_ext = s
    r0 = i * TQ
    nb = TQ // SUB
    row = lax.broadcasted_iota(jnp.int32, (SUB, SUB), 0)
    col = lax.broadcasted_iota(jnp.int32, (SUB, SUB), 1)
    tri = col <= row
    p_main, p_ext, ls = [], [[] for _ in range(1, nb)], []
    for b in range(nb):
        sm = s_main[b * SUB:(b + 1) * SUB, :]
        if b == 0:
            d = jnp.where(tri, sm[:, r0:], NEG)
            sm = jnp.concatenate([sm[:, :r0], d], axis=1) if r0 > 0 else d
        parts = [sm]
        for c in range(1, b + 1):
            e = s_ext[c - 1][(b - c) * SUB:(b - c + 1) * SUB, :]
            if c == b:
                e = jnp.where(tri, e, NEG)
            parts.append(e)
        sb = jnp.concatenate(parts, axis=1) if len(parts) > 1 else parts[0]
        m = jnp.max(sb, axis=1, keepdims=True)
        p = jnp.exp2(sb - m)
        nt = p.shape[1] // SUB
        tiles = [p[:, t * SUB:(t + 1) * SUB] for t in range(nt)]
        acc = None
        for t0 in range(0, nt, GRP):
            grp = tiles[t0:t0 + GRP]
            tot = grp[0]
            for g in grp[1:]:
                tot = tot + g
            acc = tot if acc is None else acc + tot
            last = t0 + len(grp) - 1
            if acc is not tiles[last]:
                tiles[last] = jnp.minimum(tiles[last], acc)
        p = jnp.concatenate(tiles, axis=1) if nt > 1 else tiles[0]
        ls.append(jnp.sum(acc, axis=1, keepdims=True))
        p_main.append(p[:, :r0 + SUB])
        for c in range(1, b + 1):
            p_ext[c - 1].append(p[:, r0 + c * SUB:r0 + (c + 1) * SUB])
    pm = jnp.concatenate(p_main, axis=0).astype(BF16)
    pe = [(jnp.concatenate(e, axis=0) if len(e) > 1 else e[0]).astype(BF16) for e in p_ext]
    return pm, pe, ls


def _pv(p, v, i):
    pm, pe, ls = p
    r0 = i * TQ
    nb = TQ // SUB
    o = jnp.dot(pm, v[0:r0 + SUB, :], preferred_element_type=F32)
    os_ = [o[b * SUB:(b + 1) * SUB] for b in range(nb)]
    for c in range(1, nb):
        oe = jnp.dot(pe[c - 1], v[r0 + c * SUB:r0 + (c + 1) * SUB, :], preferred_element_type=F32)
        for b in range(c, nb):
            os_[b] = os_[b] + oe[(b - c) * SUB:(b - c + 1) * SUB]
    return jnp.concatenate([os_[b] * _recip(ls[b]) for b in range(nb)], axis=0)


def _attn_pair(q_s, k_s, v_s, order, actions):
    sc, ctx = {}, {}

    def pair_ctx(i):
        return jnp.concatenate([ctx[(0, i)], ctx[(1, i)]], axis=1).astype(BF16)

    for tok in order.split():
        if tok[0] == 'S':
            h, i = int(tok[1]), int(tok[2])
            sc[(h, i)] = _qk(_Packed(q_s.at[h]), _Packed(k_s.at[h]), i)
        elif tok[0] == 'P':
            h, i = int(tok[1]), int(tok[2])
            ctx[(h, i)] = _pv(_softmax(sc.pop((h, i)), i), _Packed(v_s.at[h]), i)
        else:
            actions[tok[0]](int(tok[1:]), pair_ctx)


def _kernel(x_hbm, c_hbm, wq_hbm, wk_hbm, wv_hbm, wo_hbm, wr_hbm, wg_hbm, wu_hbm, wd_hbm,
            out_hbm,
            io_v, c_v, xn_s, acc_s, mux_s, ctx_s, q_s, k_s, v_s,
            wq_b, wk_b, wv_b, wo_v, wr_ref, wg_v, wu_v, wd_v,
            xsem, csem, wsem, osem_w, fsem, osem,
            *, S, M, D, NP, FF):
    ALL = slice(None)
    xn_p, c_p = _Packed(xn_s), _Packed(c_v)
    scale = (D ** -0.5) * math.log2(math.e)

    def xcopy(b):
        rows = pl.ds(pl.multiple_of(b * XB, XB), XB)
        return pltpu.make_async_copy(x_hbm.at[0, rows, :], io_v.at[rows, :], xsem.at[b])

    def ccopy(b):
        rows = pl.ds(pl.multiple_of(b * (XB // 2), XB // 2), XB // 2)
        return pltpu.make_async_copy(c_hbm.bitcast(U32).at[0, rows, :], c_v.at[rows, :], csem.at[b])

    def wcopies(jj, sl):
        return [
            pltpu.make_async_copy(wk_hbm.bitcast(U32).at[:, jj, :], wk_b.at[sl], wsem.at[0, sl]),
            pltpu.make_async_copy(wv_hbm.bitcast(U32).at[:, jj, :], wv_b.at[sl], wsem.at[1, sl]),
            pltpu.make_async_copy(wq_hbm.bitcast(U32).at[:, jj, :], wq_b.at[sl], wsem.at[2, sl]),
        ]

    def wocopy(t):
        heads = pl.ds(0, 2) if t == 0 else pl.ds(2, 2 * NP - 2)
        return pltpu.make_async_copy(wo_hbm.bitcast(U32).at[heads], wo_v.at[heads], osem_w.at[t])

    def fcopy(t):
        if t == 0:
            return pltpu.make_async_copy(wg_hbm, wg_v, fsem.at[0])
        if t == 1:
            return pltpu.make_async_copy(wu_hbm, wu_v, fsem.at[1])
        if t == 2:
            return pltpu.make_async_copy(wd_hbm, wd_v.at[:, 0:M], fsem.at[2])
        return pltpu.make_async_copy(wr_hbm, wr_ref, fsem.at[3])

    def ocopy(g):
        r0 = sum(EBLOCKS[:DCUTS[g - 1]]) if g > 0 else 0
        rows = pl.ds(r0, sum(EBLOCKS[:DCUTS[g]]) - r0)
        return pltpu.make_async_copy(io_v.at[rows, :], out_hbm.at[0, rows, :], osem.at[g])

    def project(dst, lhs, w32, rows, mult=None):
        y = jnp.dot(lhs, _unpack_pair(w32), preferred_element_type=F32)
        if mult is not None:
            y = y * mult
        _Packed(dst.at[0])[rows, ALL] = y[:, :D]
        _Packed(dst.at[1])[rows, ALL] = y[:, D:]

    NXB = S // XB
    for cp in wcopies(0, 0):
        cp.start()
    for b in range(NXB):
        ccopy(b).start()
        xcopy(b).start()
    wocopy(0).start()
    fcopy(3).start()
    for cp in wcopies(1, 1):
        cp.start()
    for cp in wcopies(0, 0):
        cp.wait()

    def first(b, carry):
        ccopy(b).wait()
        xcopy(b).wait()
        rows = pl.ds(pl.multiple_of(b * XB, XB), XB)
        xf = io_v[rows, :].astype(F32)
        mu = jnp.mean(xf, axis=1, keepdims=True)
        xc = xf - mu
        var = jnp.mean(xc * xc, axis=1, keepdims=True)
        xn = (xc * lax.rsqrt(var + 1e-5)).astype(BF16)
        prow = (b * XB, XB, XB)
        xn_p[prow, ALL] = xn
        acc_s[rows, :] = xc
        mux_s[rows, :] = jnp.broadcast_to(mu, (XB, 128))
        c = c_p[prow, ALL]
        project(k_s, c, wk_b[0], prow)
        project(v_s, c, wv_b[0], prow)
        project(q_s, xn, wq_b[0], prow, scale)
        return carry
    lax.fori_loop(0, S // XB, first, 0)
    for cp in wcopies(2, 0):
        cp.start()
    wocopy(1).start()
    for t in range(3):
        fcopy(t).start()
    wocopy(0).wait()

    def step(j, carry):
        slot = j % 2

        @pl.when(j == 1)
        def _():
            wocopy(1).wait()

        for cp in wcopies(j + 1, 1 - slot):
            cp.wait()

        @pl.when(jnp.logical_and(j >= 1, j + 2 < NP))
        def _():
            for cp in wcopies(j + 2, slot):
                cp.start()

        wo = pltpu.bitcast(wo_v[pl.ds(2 * j, 2)].reshape(D, M), BF16)

        def oproj(ii, pair_ctx):
            acc_s[ii * TQ:(ii + 1) * TQ, :] += jnp.dot(pair_ctx(ii), wo, preferred_element_type=F32)

        def rows_of(code):
            return slice((code // 10) * TQ, (code % 10 + 1) * TQ)

        _attn_pair(q_s, k_s, v_s, ORDER_MAIN, {
            'O': oproj,
            'K': lambda code, _: project(k_s, c_p[rows_of(code), ALL], wk_b[1 - slot], rows_of(code)),
            'V': lambda code, _: project(v_s, c_p[rows_of(code), ALL], wv_b[1 - slot], rows_of(code)),
            'Q': lambda code, _: project(q_s, xn_p[rows_of(code), ALL], wq_b[1 - slot], rows_of(code), scale),
        })
        return carry
    lax.fori_loop(0, NP - 1, step, 0)

    fcopy(3).wait()
    if PONLY:
        return
    eps = jnp.asarray(1e-5, BF16).astype(F32)

    def last_head(h, carry):
        sc = {}
        for tok in ORDER_LAST.split():
            i = int(tok[1])
            if tok[0] == 'S':
                sc[i] = _qk(_Packed(q_s.at[h]), _Packed(k_s.at[h]), i)
            else:
                _Packed(ctx_s.at[h])[slice(i * TQ, (i + 1) * TQ), ALL] = _pv(
                    _softmax(sc.pop(i), i), _Packed(v_s.at[h]), i)
        return carry
    lax.fori_loop(0, 2, last_head, 0)

    NCH = 4
    CW = M // NCH
    RW = M // RG
    wr16 = [jnp.broadcast_to(wr_ref[t * RW:(t + 1) * RW].astype(F32).reshape(1, RW), (16, RW)).astype(BF16)
            for t in range(RG)]

    def oproj_part(r0, n, t):
        rows = slice(r0, r0 + n)
        cols = slice(t * CW, (t + 1) * CW)
        return (acc_s[rows, cols]
                + jnp.dot(_Packed(ctx_s.at[0])[rows, ALL], pltpu.bitcast(wo_v[2 * NP - 2, :, cols], BF16),
                           preferred_element_type=F32)
                + jnp.dot(_Packed(ctx_s.at[1])[rows, ALL], pltpu.bitcast(wo_v[2 * NP - 1, :, cols], BF16),
                           preferred_element_type=F32))

    def ln2(r0, n, a):
        rows = slice(r0, r0 + n)
        acc_s[rows, :] = a
        s1 = jnp.mean(a, axis=1, keepdims=True)
        var = jnp.maximum(jnp.mean(a * a, axis=1, keepdims=True) - s1 * s1, 0.0)
        ve = _rb(_rb(var) + eps)
        den = _rb(ve * lax.rsqrt(ve))
        inv = _recip(den)
        inv = inv * (2.0 - den * inv)
        mux = mux_s[rows, :]
        c1 = (_rb(mux + s1) - mux) * inv
        c2 = mux - c1
        a = acc_s[rows, :]
        t = a * inv
        xn_p[rows, ALL] = t - jnp.concatenate([c1] * (M // 128), axis=1)
        io_v[rows, :] = ((a + t) + jnp.concatenate([c2] * (M // 128), axis=1)).astype(BF16)

    def router_part(r0, n, t):
        cols = slice(t * RW, (t + 1) * RW)
        return lax.dot_general(wr16[t], xn_p[slice(r0, r0 + n), cols], NT, preferred_element_type=F32)

    blocks = []
    r0 = 0
    for n in EBLOCKS:
        blocks.append((r0, n))
        r0 += n
    assert r0 == S
    rparts = []
    for k in range(len(blocks) + RLAG):
        hp, rp = [], None
        for t in range(NCH):
            if k < len(blocks):
                hp.append(oproj_part(*blocks[k], t))
            if k >= RLAG and str(t) in RPOS:
                part = router_part(*blocks[k - RLAG], RPOS.index(str(t)))[0:8, :]
                rp = part if rp is None else rp + part
        if k in DCUTS:
            ocopy(DCUTS.index(k)).start()
        if k < len(blocks):
            ln2(*blocks[k], jnp.concatenate(hp, axis=1))
        if k >= RLAG:
            rparts.append(rp)
    rrow = _rb(jnp.concatenate(rparts, axis=1))

    I32 = jnp.int32
    b16 = lax.shift_right_logical(pltpu.bitcast(rrow, I32), 16)
    rank = jnp.where(b16 >= 0x8000, 0x10000 - b16, 0x8000 + b16)
    lane = lax.broadcasted_iota(I32, rrow.shape, 1)
    key = pltpu.bitcast(rank * S + (S - 1 - lane) + 0x20000000, F32)
    k1 = jnp.max(key, axis=1, keepdims=True)
    k2 = jnp.max(jnp.where(key == k1, 0.0, key), axis=1, keepdims=True)
    i1 = (S - 1) - (pltpu.bitcast(k1, I32)[0, 0] & (S - 1))
    i2 = (S - 1) - (pltpu.bitcast(k2, I32)[0, 0] & (S - 1))
    m1 = jnp.max(jnp.where(key == k1, rrow, -jnp.inf), axis=1, keepdims=True)[0:1, :]
    m2 = jnp.max(jnp.where(key == k2, rrow, -jnp.inf), axis=1, keepdims=True)[0:1, :]
    g1 = pl.multiple_of((i1 // 16) * 16, 16)
    g2 = pl.multiple_of((i2 // 16) * 16, 16)

    rid = lax.broadcasted_iota(jnp.int32, (16, M), 0)

    def pick(g, i):
        blk = xn_p[(g, 16, 16), ALL].astype(F32)
        return jnp.sum(jnp.where(rid == i - g, blk, 0.0), axis=0, keepdims=True)

    xs = jnp.where(rid == 0, pick(g1, i1), pick(g2, i2))
    xsb = xs.astype(BF16)
    for t in range(3):
        fcopy(t).wait()
    FH = FF // NF

    def ffn(o, y):
        nch = FH // FC
        acts = []
        for t in range(nch + 1):
            if t < nch:
                cols = pl.ds(pl.multiple_of(o * FH + t * FC, 128), FC)
                a = _rb(jnp.dot(xsb, wg_v[:, cols], preferred_element_type=F32))
                u = _rb(jnp.dot(xsb, wu_v[:, cols], preferred_element_type=F32))
                g = _rb(a * _rb(jax.nn.sigmoid(a)))
                acts.append((g * u).astype(BF16))
            if t > 0:
                rws = pl.ds(pl.multiple_of(o * FH + (t - 1) * FC, 128), FC)
                y = y + jnp.dot(acts[t - 1], wd_v[rws, 0:M], preferred_element_type=F32)
        return y
    y = lax.fori_loop(0, NF, ffn, jnp.zeros((16, M), F32))
    rsel = jnp.where(rid == 0, m1, m2)
    y = _rb(_rb(y) * _rb(jax.nn.sigmoid(rsel)))
    upd = _rb(xs + y)

    for b in range(len(DCUTS)):
        ocopy(b).wait()
    for (ii, gg, rr) in ((i1, g1, 0), (i2, g2, 1)):
        hrow = acc_s[pl.ds(gg, 16), :] + jnp.concatenate([mux_s[pl.ds(gg, 16), :]] * (M // 128), axis=1)
        new = _rb(hrow) + upd[rr:rr + 1, :]
        cur = io_v[pl.ds(gg, 16), :].astype(F32)
        io_v[pl.ds(gg, 16), :] = jnp.where(rid == ii - gg, new, cur).astype(BF16)

    def pcopy(g, k):
        return pltpu.make_async_copy(io_v.at[pl.ds(g, 16), :], out_hbm.at[0, pl.ds(g, 16), :], osem.at[k])

    pcopy(g1, 0).start()

    @pl.when(g2 != g1)
    def _():
        pcopy(g2, 1).start()
        pcopy(g2, 1).wait()
    pcopy(g1, 0).wait()


@jax.jit
def pallas_sequential_preLN__compressed_kv_cla__moe_arch_mod__prompt_kernel(
    A_x: jax.Array,
    A_c_kv: jax.Array,
    A_w_q: jax.Array,
    A_w_uk: jax.Array,
    A_w_uv: jax.Array,
    A_w_o: jax.Array,
    B_x: jax.Array,
    B_w_r: jax.Array,
    B_w_gate: jax.Array,
    B_w_up: jax.Array,
    B_w_down: jax.Array,
):
    _, S, M = A_x.shape
    C = A_c_kv.shape[2]
    H, D = A_w_q.shape[1], A_w_q.shape[2]
    FF = B_w_gate.shape[1]
    NP = H // 2
    any_spec = pl.BlockSpec(memory_space=pl.ANY)
    return pl.pallas_call(
        functools.partial(_kernel, S=S, M=M, D=D, NP=NP, FF=FF),
        in_specs=[
            any_spec, any_spec, any_spec, any_spec, any_spec, any_spec,
            any_spec, any_spec, any_spec, any_spec,
        ],
        out_specs=any_spec,
        out_shape=jax.ShapeDtypeStruct((1, S, M), BF16),
        scratch_shapes=[
            pltpu.VMEM((S, M), BF16),
            pltpu.VMEM((S // 2, C), U32),
            pltpu.VMEM((S // 2, M), U32),
            pltpu.VMEM((S, M), F32),
            pltpu.VMEM((S, 128), F32),
            pltpu.VMEM((2, S // 2, D), U32),
            pltpu.VMEM((2, S // 2, D), U32),
            pltpu.VMEM((2, S // 2, D), U32),
            pltpu.VMEM((2, S // 2, D), U32),
            pltpu.VMEM((2, M, D), U32),
            pltpu.VMEM((2, C, D), U32),
            pltpu.VMEM((2, C, D), U32),
            pltpu.VMEM((H, D // 2, M), U32),
            pltpu.VMEM((M,), BF16),
            pltpu.VMEM((M, FF), BF16),
            pltpu.VMEM((M, FF), BF16),
            pltpu.VMEM((FF, M + 128), BF16),
            pltpu.SemaphoreType.DMA((S // XB,)),
            pltpu.SemaphoreType.DMA((S // XB,)),
            pltpu.SemaphoreType.DMA((3, 2)),
            pltpu.SemaphoreType.DMA((2,)),
            pltpu.SemaphoreType.DMA((4,)),
            pltpu.SemaphoreType.DMA((max(len(DCUTS), 2),)),
        ],
        compiler_params=pltpu.CompilerParams(
            vmem_limit_bytes=110 * 1024 * 1024,
            disable_bounds_checks=True,
            disable_semaphore_checks=True,
        ),
    )(A_x, A_c_kv, A_w_q, A_w_uk, A_w_uv, A_w_o, B_w_r, B_w_gate, B_w_up, B_w_down)
```

```python
import functools
import math

import jax
import jax.numpy as jnp
from jax import lax
import jax.experimental.pallas as pl
import jax.experimental.pallas.tpu as pltpu

F32 = jnp.float32
BF16 = jnp.bfloat16
U32 = jnp.uint32
NEG = -1e30
NT = (((1,), (1,)), ((), ()))
TQ = 512
SUB = 128
GRP = 4
XB = 256
EB = 128
OB = 512
NCH = 4
RG = 2
RLAG = 2
FC = 512

ORDER_MAIN = ("S03 S13 P03 K33 S02 P13 S12 P02 S01 P12 S11 Q23 S00 P01 P11 S10 K02 P00 P10 "
              "O3 Q01 O2 O1 O0 V03")
ORDER_LAST = "S2 S3 P2 S1 P3 S0 P1 P0"


def _rb(v):
    return v.astype(BF16).astype(F32)


def _recip(l):
    return pl.reciprocal(l, approx=True)


def _unpack_pair(w32):
    lo = pltpu.bitcast(w32 << 16, F32)
    hi = pltpu.bitcast(w32 & jnp.uint32(0xFFFF0000), F32)
    return jnp.concatenate([lo, hi], axis=1).astype(BF16)


class _Packed:
    def __init__(self, ref):
        self.ref = ref

    @staticmethod
    def half(rows):
        if isinstance(rows, slice):
            return slice(rows.start // 2, rows.stop // 2)
        start, size, align = rows
        return pl.ds(pl.multiple_of(start // 2, align // 2), size // 2)

    def __getitem__(self, idx):
        rows, cols = idx
        return pltpu.bitcast(self.ref[self.half(rows), cols], BF16)

    def __setitem__(self, idx, val):
        rows, cols = idx
        self.ref[self.half(rows), cols] = pltpu.bitcast(val.astype(BF16), U32)


def _qk(q, k, i):
    r0 = i * TQ
    nb = TQ // SUB
    qb = q[r0:r0 + TQ, :]
    s_main = lax.dot_general(qb, k[0:r0 + SUB, :], NT, preferred_element_type=F32)
    s_ext = [lax.dot_general(qb[c * SUB:, :], k[r0 + c * SUB:r0 + (c + 1) * SUB, :], NT,
                             preferred_element_type=F32) for c in range(1, nb)]
    return s_main, s_ext


def _softmax(s, i):
    s_main, s_ext = s
    r0 = i * TQ
    nb = TQ // SUB
    row = lax.broadcasted_iota(jnp.int32, (SUB, SUB), 0)
    col = lax.broadcasted_iota(jnp.int32, (SUB, SUB), 1)
    tri = col <= row
    p_main, p_ext, ls = [], [[] for _ in range(1, nb)], []
    for b in range(nb):
        sm = s_main[b * SUB:(b + 1) * SUB, :]
        if b == 0:
            d = jnp.where(tri, sm[:, r0:], NEG)
            sm = jnp.concatenate([sm[:, :r0], d], axis=1) if r0 > 0 else d
        parts = [sm]
        for c in range(1, b + 1):
            e = s_ext[c - 1][(b - c) * SUB:(b - c + 1) * SUB, :]
            if c == b:
                e = jnp.where(tri, e, NEG)
            parts.append(e)
        sb = jnp.concatenate(parts, axis=1) if len(parts) > 1 else parts[0]
        m = jnp.max(sb, axis=1, keepdims=True)
        p = jnp.exp2(sb - m)
        nt = p.shape[1] // SUB
        tiles = [p[:, t * SUB:(t + 1) * SUB] for t in range(nt)]
        acc = None
        for t0 in range(0, nt, GRP):
            grp = tiles[t0:t0 + GRP]
            tot = grp[0]
            for g in grp[1:]:
                tot = tot + g
            acc = tot if acc is None else acc + tot
            last = t0 + len(grp) - 1
            if acc is not tiles[last]:
                tiles[last] = jnp.minimum(tiles[last], acc)
        p = jnp.concatenate(tiles, axis=1) if nt > 1 else tiles[0]
        ls.append(jnp.sum(acc, axis=1, keepdims=True))
        p_main.append(p[:, :r0 + SUB])
        for c in range(1, b + 1):
            p_ext[c - 1].append(p[:, r0 + c * SUB:r0 + (c + 1) * SUB])
    pm = jnp.concatenate(p_main, axis=0).astype(BF16)
    pe = [(jnp.concatenate(e, axis=0) if len(e) > 1 else e[0]).astype(BF16) for e in p_ext]
    return pm, pe, ls


def _pv(p, v, i):
    pm, pe, ls = p
    r0 = i * TQ
    nb = TQ // SUB
    o = jnp.dot(pm, v[0:r0 + SUB, :], preferred_element_type=F32)
    os_ = [o[b * SUB:(b + 1) * SUB] for b in range(nb)]
    for c in range(1, nb):
        oe = jnp.dot(pe[c - 1], v[r0 + c * SUB:r0 + (c + 1) * SUB, :], preferred_element_type=F32)
        for b in range(c, nb):
            os_[b] = os_[b] + oe[(b - c) * SUB:(b - c + 1) * SUB]
    return jnp.concatenate([os_[b] * _recip(ls[b]) for b in range(nb)], axis=0)


def _attn_pair(q_s, k_s, v_s, order, actions):
    sc, ctx = {}, {}

    def pair_ctx(i):
        return jnp.concatenate([ctx[(0, i)], ctx[(1, i)]], axis=1).astype(BF16)

    for tok in order.split():
        if tok[0] == 'S':
            h, i = int(tok[1]), int(tok[2])
            sc[(h, i)] = _qk(_Packed(q_s.at[h]), _Packed(k_s.at[h]), i)
        elif tok[0] == 'P':
            h, i = int(tok[1]), int(tok[2])
            ctx[(h, i)] = _pv(_softmax(sc.pop((h, i)), i), _Packed(v_s.at[h]), i)
        else:
            actions[tok[0]](int(tok[1:]), pair_ctx)


def _kernel(x_hbm, c_hbm, wq_hbm, wk_hbm, wv_hbm, wo_hbm, wr_hbm, wg_hbm, wu_hbm, wd_hbm,
            out_hbm,
            io_v, pt_v, c_v, xn_s, acc_s, mux_s, ctx_s, q_s, k_s, v_s,
            wq_b, wk_b, wv_b, wo_v, wr_ref, wg_v, wu_v, wd_v,
            xsem, csem, wsem, osem_w, fsem, osem,
            *, S, M, D, NP, FF):
    ALL = slice(None)
    xn_p, c_p = _Packed(xn_s), _Packed(c_v)
    scale = (D ** -0.5) * math.log2(math.e)

    def xcopy(b):
        rows = pl.ds(pl.multiple_of(b * XB, XB), XB)
        return pltpu.make_async_copy(x_hbm.at[0, rows, :], io_v.at[rows, :], xsem.at[b])

    def ccopy(b):
        rows = pl.ds(pl.multiple_of(b * (XB // 2), XB // 2), XB // 2)
        return pltpu.make_async_copy(c_hbm.bitcast(U32).at[0, rows, :], c_v.at[rows, :], csem.at[b])

    def wcopies(jj, sl):
        return [
            pltpu.make_async_copy(wk_hbm.bitcast(U32).at[:, jj, :], wk_b.at[sl], wsem.at[0, sl]),
            pltpu.make_async_copy(wv_hbm.bitcast(U32).at[:, jj, :], wv_b.at[sl], wsem.at[1, sl]),
            pltpu.make_async_copy(wq_hbm.bitcast(U32).at[:, jj, :], wq_b.at[sl], wsem.at[2, sl]),
        ]

    def wocopy(t):
        heads = pl.ds(0, 2) if t == 0 else pl.ds(2, 2 * NP - 2)
        return pltpu.make_async_copy(wo_hbm.bitcast(U32).at[heads], wo_v.at[heads], osem_w.at[t])

    def fcopy(t):
        if t == 0:
            return pltpu.make_async_copy(wg_hbm, wg_v, fsem.at[0])
        if t == 1:
            return pltpu.make_async_copy(wu_hbm, wu_v, fsem.at[1])
        if t == 2:
            return pltpu.make_async_copy(wd_hbm, wd_v.at[:, 0:M], fsem.at[2])
        return pltpu.make_async_copy(wr_hbm, wr_ref, fsem.at[3])

    def ocopy(g):
        rows = pl.ds(g * OB, OB)
        return pltpu.make_async_copy(io_v.at[rows, :], out_hbm.at[0, rows, :], osem.at[g])

    def project(dst, lhs, w32, rows, mult=None):
        y = jnp.dot(lhs, _unpack_pair(w32), preferred_element_type=F32)
        if mult is not None:
            y = y * mult
        _Packed(dst.at[0])[rows, ALL] = y[:, :D]
        _Packed(dst.at[1])[rows, ALL] = y[:, D:]

    NXB = S // XB
    for cp in wcopies(0, 0):
        cp.start()
    for b in range(NXB):
        ccopy(b).start()
        xcopy(b).start()
    wocopy(0).start()
    fcopy(3).start()
    for cp in wcopies(1, 1):
        cp.start()
    for cp in wcopies(0, 0):
        cp.wait()

    def first(b, carry):
        ccopy(b).wait()
        xcopy(b).wait()
        rows = pl.ds(pl.multiple_of(b * XB, XB), XB)
        xf = io_v[rows, :].astype(F32)
        mu = jnp.mean(xf, axis=1, keepdims=True)
        xc = xf - mu
        var = jnp.mean(xc * xc, axis=1, keepdims=True)
        xn = (xc * lax.rsqrt(var + 1e-5)).astype(BF16)
        prow = (b * XB, XB, XB)
        xn_p[prow, ALL] = xn
        acc_s[rows, :] = xc
        mux_s[rows, :] = jnp.broadcast_to(mu, (XB, 128))
        c = c_p[prow, ALL]
        project(k_s, c, wk_b[0], prow)
        project(v_s, c, wv_b[0], prow)
        project(q_s, xn, wq_b[0], prow, scale)
        return carry
    lax.fori_loop(0, S // XB, first, 0)
    for cp in wcopies(2, 0):
        cp.start()
    wocopy(1).start()
    for t in range(3):
        fcopy(t).start()
    wocopy(0).wait()

    def step(j, carry):
        slot = j % 2

        @pl.when(j == 1)
        def _():
            wocopy(1).wait()

        for cp in wcopies(j + 1, 1 - slot):
            cp.wait()

        @pl.when(jnp.logical_and(j >= 1, j + 2 < NP))
        def _():
            for cp in wcopies(j + 2, slot):
                cp.start()

        wo = pltpu.bitcast(wo_v[pl.ds(2 * j, 2)].reshape(D, M), BF16)

        def oproj(ii, pair_ctx):
            acc_s[ii * TQ:(ii + 1) * TQ, :] += jnp.dot(pair_ctx(ii), wo, preferred_element_type=F32)

        def rows_of(code):
            return slice((code // 10) * TQ, (code % 10 + 1) * TQ)

        _attn_pair(q_s, k_s, v_s, ORDER_MAIN, {
            'O': oproj,
            'K': lambda code, _: project(k_s, c_p[rows_of(code), ALL], wk_b[1 - slot], rows_of(code)),
            'V': lambda code, _: project(v_s, c_p[rows_of(code), ALL], wv_b[1 - slot], rows_of(code)),
            'Q': lambda code, _: project(q_s, xn_p[rows_of(code), ALL], wq_b[1 - slot], rows_of(code), scale),
        })
        return carry
    lax.fori_loop(0, NP - 1, step, 0)

    for t in range(4):
        fcopy(t).wait()
    eps = jnp.asarray(1e-5, BF16).astype(F32)

    def last_head(h, carry):
        sc = {}
        for tok in ORDER_LAST.split():
            i = int(tok[1])
            if tok[0] == 'S':
                sc[i] = _qk(_Packed(q_s.at[h]), _Packed(k_s.at[h]), i)
            else:
                _Packed(ctx_s.at[h])[slice(i * TQ, (i + 1) * TQ), ALL] = _pv(
                    _softmax(sc.pop(i), i), _Packed(v_s.at[h]), i)
        return carry
    lax.fori_loop(0, 2, last_head, 0)

    CW = M // NCH
    RW = M // RG
    wr16 = [jnp.broadcast_to(wr_ref[t * RW:(t + 1) * RW].astype(F32).reshape(1, RW), (16, RW)).astype(BF16)
            for t in range(RG)]

    def oproj_part(r0, t):
        rows = slice(r0, r0 + EB)
        cols = slice(t * CW, (t + 1) * CW)
        return (acc_s[rows, cols]
                + jnp.dot(_Packed(ctx_s.at[0])[rows, ALL], pltpu.bitcast(wo_v[2 * NP - 2, :, cols], BF16),
                           preferred_element_type=F32)
                + jnp.dot(_Packed(ctx_s.at[1])[rows, ALL], pltpu.bitcast(wo_v[2 * NP - 1, :, cols], BF16),
                           preferred_element_type=F32))

    def ln2(r0, a):
        rows = slice(r0, r0 + EB)
        acc_s[rows, :] = a
        s1 = jnp.mean(a, axis=1, keepdims=True)
        var = jnp.maximum(jnp.mean(a * a, axis=1, keepdims=True) - s1 * s1, 0.0)
        ve = _rb(_rb(var) + eps)
        den = _rb(ve * lax.rsqrt(ve))
        inv = _recip(den)
        inv = inv * (2.0 - den * inv)
        mux = mux_s[rows, :]
        c1 = (_rb(mux + s1) - mux) * inv
        c2 = mux - c1
        a = acc_s[rows, :]
        t = a * inv
        xn_p[rows, ALL] = t - jnp.concatenate([c1] * (M // 128), axis=1)
        io_v[rows, :] = ((a + t) + jnp.concatenate([c2] * (M // 128), axis=1)).astype(BF16)

    def router_part(r0, t):
        cols = slice(t * RW, (t + 1) * RW)
        return lax.dot_general(wr16[t], xn_p[slice(r0, r0 + EB), cols], NT, preferred_element_type=F32)

    neb = S // EB
    rparts = []
    for k in range(neb + RLAG):
        hp, rp = [], None
        for t in range(NCH):
            if k < neb:
                hp.append(oproj_part(k * EB, t))
            if k >= RLAG and t < RG:
                part = router_part((k - RLAG) * EB, t)[0:8, :]
                rp = part if rp is None else rp + part
        if k > 0 and k <= neb and (k * EB) % OB == 0:
            ocopy(k * EB // OB - 1).start()
        if k < neb:
            ln2(k * EB, jnp.concatenate(hp, axis=1))
        if k >= RLAG:
            rparts.append(rp)
    rrow = _rb(jnp.concatenate(rparts, axis=1))

    I32 = jnp.int32
    b16 = lax.shift_right_logical(pltpu.bitcast(rrow, I32), 16)
    rank = jnp.where(b16 >= 0x8000, 0x10000 - b16, 0x8000 + b16)
    lane = lax.broadcasted_iota(I32, rrow.shape, 1)
    key = pltpu.bitcast(rank * S + (S - 1 - lane) + 0x20000000, F32)
    k1 = jnp.max(key, axis=1, keepdims=True)
    k2 = jnp.max(jnp.where(key == k1, 0.0, key), axis=1, keepdims=True)
    i1 = (S - 1) - (pltpu.bitcast(k1, I32)[0, 0] & (S - 1))
    i2 = (S - 1) - (pltpu.bitcast(k2, I32)[0, 0] & (S - 1))
    m1 = jnp.max(jnp.where(key == k1, rrow, -jnp.inf), axis=1, keepdims=True)[0:1, :]
    m2 = jnp.max(jnp.where(key == k2, rrow, -jnp.inf), axis=1, keepdims=True)[0:1, :]
    g1 = pl.multiple_of((i1 // 16) * 16, 16)
    g2 = pl.multiple_of((i2 // 16) * 16, 16)

    rid = lax.broadcasted_iota(jnp.int32, (16, M), 0)

    def pick(g, i):
        blk = xn_p[(g, 16, 16), ALL].astype(F32)
        return jnp.sum(jnp.where(rid == i - g, blk, 0.0), axis=0, keepdims=True)

    xs = jnp.where(rid == 0, pick(g1, i1), pick(g2, i2))
    xsb = xs.astype(BF16)
    ocopy(0).wait()
    nch = FF // FC
    acts, y = [], None
    for t in range(nch + 1):
        if t < nch:
            cols = slice(t * FC, (t + 1) * FC)
            a = _rb(jnp.dot(xsb, wg_v[:, cols], preferred_element_type=F32))
            u = _rb(jnp.dot(xsb, wu_v[:, cols], preferred_element_type=F32))
            g = _rb(a * _rb(jax.nn.sigmoid(a)))
            acts.append((g * u).astype(BF16))
        if t > 0:
            yt = jnp.dot(acts[t - 1], wd_v[(t - 1) * FC:t * FC, 0:M], preferred_element_type=F32)
            y = yt if y is None else y + yt
    rsel = jnp.where(rid == 0, m1, m2)
    y = _rb(_rb(y) * _rb(jax.nn.sigmoid(rsel)))
    upd = _rb(xs + y)

    for k, gg in enumerate((g1, g2)):
        rows = pl.ds(gg, 16)
        hb = _rb(acc_s[rows, :] + jnp.concatenate([mux_s[rows, :]] * (M // 128), axis=1))
        val = jnp.where(rid == i1 - gg, hb + upd[0:1, :],
                        jnp.where(rid == i2 - gg, hb + upd[1:2, :], io_v[rows, :].astype(F32)))
        pt_v[k] = val.astype(BF16)

    def pcopy(g, k):
        return pltpu.make_async_copy(pt_v.at[k], out_hbm.at[0, pl.ds(g, 16), :], osem.at[k])

    for b in range(1, S // OB):
        ocopy(b).wait()
    pcopy(g1, 0).start()

    @pl.when(g2 != g1)
    def _():
        pcopy(g2, 1).start()
        pcopy(g2, 1).wait()
    pcopy(g1, 0).wait()


@jax.jit
def pallas_sequential_preLN__compressed_kv_cla__moe_arch_mod__prompt_kernel(
    A_x: jax.Array,
    A_c_kv: jax.Array,
    A_w_q: jax.Array,
    A_w_uk: jax.Array,
    A_w_uv: jax.Array,
    A_w_o: jax.Array,
    B_x: jax.Array,
    B_w_r: jax.Array,
    B_w_gate: jax.Array,
    B_w_up: jax.Array,
    B_w_down: jax.Array,
):
    _, S, M = A_x.shape
    C = A_c_kv.shape[2]
    H, D = A_w_q.shape[1], A_w_q.shape[2]
    FF = B_w_gate.shape[1]
    NP = H // 2
    any_spec = pl.BlockSpec(memory_space=pl.ANY)
    return pl.pallas_call(
        functools.partial(_kernel, S=S, M=M, D=D, NP=NP, FF=FF),
        in_specs=[
            any_spec, any_spec, any_spec, any_spec, any_spec, any_spec,
            any_spec, any_spec, any_spec, any_spec,
        ],
        out_specs=any_spec,
        out_shape=jax.ShapeDtypeStruct((1, S, M), BF16),
        scratch_shapes=[
            pltpu.VMEM((S, M), BF16),
            pltpu.VMEM((2, 16, M), BF16),
            pltpu.VMEM((S // 2, C), U32),
            pltpu.VMEM((S // 2, M), U32),
            pltpu.VMEM((S, M), F32),
            pltpu.VMEM((S, 128), F32),
            pltpu.VMEM((2, S // 2, D), U32),
            pltpu.VMEM((2, S // 2, D), U32),
            pltpu.VMEM((2, S // 2, D), U32),
            pltpu.VMEM((2, S // 2, D), U32),
            pltpu.VMEM((2, M, D), U32),
            pltpu.VMEM((2, C, D), U32),
            pltpu.VMEM((2, C, D), U32),
            pltpu.VMEM((H, D // 2, M), U32),
            pltpu.VMEM((M,), BF16),
            pltpu.VMEM((M, FF), BF16),
            pltpu.VMEM((M, FF), BF16),
            pltpu.VMEM((FF, M + 128), BF16),
            pltpu.SemaphoreType.DMA((S // XB,)),
            pltpu.SemaphoreType.DMA((S // XB,)),
            pltpu.SemaphoreType.DMA((3, 2)),
            pltpu.SemaphoreType.DMA((2,)),
            pltpu.SemaphoreType.DMA((4,)),
            pltpu.SemaphoreType.DMA((S // OB,)),
        ],
        compiler_params=pltpu.CompilerParams(
            vmem_limit_bytes=110 * 1024 * 1024,
            disable_bounds_checks=True,
            disable_semaphore_checks=True,
        ),
    )(A_x, A_c_kv, A_w_q, A_w_uk, A_w_uv, A_w_o, B_w_r, B_w_gate, B_w_up, B_w_down)
```

```python
import functools
import math

import jax
import jax.numpy as jnp
from jax import lax
import jax.experimental.pallas as pl
import jax.experimental.pallas.tpu as pltpu

F32 = jnp.float32
BF16 = jnp.bfloat16
U32 = jnp.uint32
NEG = -1e30
NT = (((1,), (1,)), ((), ()))
TQ = 512
SUB = 128
GRP = 4
XB = 256
EB = 128
OB = 512
NCH = 4
RG = 2
RLAG = 2
FC = 512

ORDER_MAIN = ("S03 S13 P03 K33 S02 P13 S12 P02 S01 P12 S11 Q23 S00 P01 P11 S10 K02 P00 P10 "
              "O3 Q01 O2 O1 O0 V03")
ORDER_LAST = "S2 S3 P2 S1 P3 S0 P1 P0"


def _rb(v):
    return v.astype(BF16).astype(F32)


def _recip(l):
    return pl.reciprocal(l, approx=True)


def _unpack_pair(w32):
    lo = pltpu.bitcast(w32 << 16, F32)
    hi = pltpu.bitcast(w32 & jnp.uint32(0xFFFF0000), F32)
    return jnp.concatenate([lo, hi], axis=1).astype(BF16)


class _Packed:
    def __init__(self, ref):
        self.ref = ref

    @staticmethod
    def half(rows):
        if isinstance(rows, slice):
            return slice(rows.start // 2, rows.stop // 2)
        start, size, align = rows
        return pl.ds(pl.multiple_of(start // 2, align // 2), size // 2)

    def __getitem__(self, idx):
        rows, cols = idx
        return pltpu.bitcast(self.ref[self.half(rows), cols], BF16)

    def __setitem__(self, idx, val):
        rows, cols = idx
        self.ref[self.half(rows), cols] = pltpu.bitcast(val.astype(BF16), U32)


def _qk(q, k, i):
    r0 = i * TQ
    nb = TQ // SUB
    qb = q[r0:r0 + TQ, :]
    s_main = lax.dot_general(qb, k[0:r0 + SUB, :], NT, preferred_element_type=F32)
    s_ext = [lax.dot_general(qb[c * SUB:, :], k[r0 + c * SUB:r0 + (c + 1) * SUB, :], NT,
                             preferred_element_type=F32) for c in range(1, nb)]
    return s_main, s_ext


def _softmax(s, i):
    s_main, s_ext = s
    r0 = i * TQ
    nb = TQ // SUB
    row = lax.broadcasted_iota(jnp.int32, (SUB, SUB), 0)
    col = lax.broadcasted_iota(jnp.int32, (SUB, SUB), 1)
    tri = col <= row
    p_main, p_ext, ls = [], [[] for _ in range(1, nb)], []
    for b in range(nb):
        sm = s_main[b * SUB:(b + 1) * SUB, :]
        if b == 0:
            d = jnp.where(tri, sm[:, r0:], NEG)
            sm = jnp.concatenate([sm[:, :r0], d], axis=1) if r0 > 0 else d
        parts = [sm]
        for c in range(1, b + 1):
            e = s_ext[c - 1][(b - c) * SUB:(b - c + 1) * SUB, :]
            if c == b:
                e = jnp.where(tri, e, NEG)
            parts.append(e)
        sb = jnp.concatenate(parts, axis=1) if len(parts) > 1 else parts[0]
        m = jnp.max(sb, axis=1, keepdims=True)
        p = jnp.exp2(sb - m)
        nt = p.shape[1] // SUB
        tiles = [p[:, t * SUB:(t + 1) * SUB] for t in range(nt)]
        acc = None
        for t0 in range(0, nt, GRP):
            grp = tiles[t0:t0 + GRP]
            tot = grp[0]
            for g in grp[1:]:
                tot = tot + g
            acc = tot if acc is None else acc + tot
            last = t0 + len(grp) - 1
            if acc is not tiles[last]:
                tiles[last] = jnp.minimum(tiles[last], acc)
        p = jnp.concatenate(tiles, axis=1) if nt > 1 else tiles[0]
        ls.append(jnp.sum(acc, axis=1, keepdims=True))
        p_main.append(p[:, :r0 + SUB])
        for c in range(1, b + 1):
            p_ext[c - 1].append(p[:, r0 + c * SUB:r0 + (c + 1) * SUB])
    pm = jnp.concatenate(p_main, axis=0).astype(BF16)
    pe = [(jnp.concatenate(e, axis=0) if len(e) > 1 else e[0]).astype(BF16) for e in p_ext]
    return pm, pe, ls


def _pv(p, v, i):
    pm, pe, ls = p
    r0 = i * TQ
    nb = TQ // SUB
    o = jnp.dot(pm, v[0:r0 + SUB, :], preferred_element_type=F32)
    os_ = [o[b * SUB:(b + 1) * SUB] for b in range(nb)]
    for c in range(1, nb):
        oe = jnp.dot(pe[c - 1], v[r0 + c * SUB:r0 + (c + 1) * SUB, :], preferred_element_type=F32)
        for b in range(c, nb):
            os_[b] = os_[b] + oe[(b - c) * SUB:(b - c + 1) * SUB]
    return jnp.concatenate([os_[b] * _recip(ls[b]) for b in range(nb)], axis=0)


def _attn_pair(q_s, k_s, v_s, order, actions):
    sc, ctx = {}, {}

    def pair_ctx(i):
        return jnp.concatenate([ctx[(0, i)], ctx[(1, i)]], axis=1).astype(BF16)

    for tok in order.split():
        if tok[0] == 'S':
            h, i = int(tok[1]), int(tok[2])
            sc[(h, i)] = _qk(_Packed(q_s.at[h]), _Packed(k_s.at[h]), i)
        elif tok[0] == 'P':
            h, i = int(tok[1]), int(tok[2])
            ctx[(h, i)] = _pv(_softmax(sc.pop((h, i)), i), _Packed(v_s.at[h]), i)
        else:
            actions[tok[0]](int(tok[1:]), pair_ctx)


def _kernel(x_hbm, c_hbm, wq_hbm, wk_hbm, wv_hbm, wo_hbm, wr_hbm, wg_hbm, wu_hbm, wd_hbm,
            out_hbm,
            io_v, pt_v, c_v, xn_s, acc_s, mux_s, ctx_s, q_s, k_s, v_s,
            w_b, wo_v, wr_ref, wg_v, wu_v, wd_v,
            xsem, csem, wsem, osem_w, fsem, osem,
            *, S, M, C, D, NP, FF):
    ALL = slice(None)
    xn_p, c_p = _Packed(xn_s), _Packed(c_v)
    scale = (D ** -0.5) * math.log2(math.e)

    def xcopy(b):
        rows = pl.ds(pl.multiple_of(b * XB, XB), XB)
        return pltpu.make_async_copy(x_hbm.at[0, rows, :], io_v.at[rows, :], xsem.at[b])

    def ccopy(b):
        rows = pl.ds(pl.multiple_of(b * (XB // 2), XB // 2), XB // 2)
        return pltpu.make_async_copy(c_hbm.bitcast(U32).at[0, rows, :], c_v.at[rows, :], csem.at[b])

    KR, VR, QR = slice(0, C), slice(C, 2 * C), slice(2 * C, 2 * C + M)

    def wstart(jj, sl):
        for src, rows in ((wk_hbm, KR), (wv_hbm, VR), (wq_hbm, QR)):
            pltpu.make_async_copy(src.bitcast(U32).at[:, jj, :], w_b.at[sl, rows, :], wsem.at[sl]).start()

    def wwait(sl):
        pltpu.make_async_copy(w_b.at[sl], w_b.at[sl], wsem.at[sl]).wait()

    def wocopy(t):
        heads = pl.ds(0, 2) if t == 0 else pl.ds(2, 2 * NP - 2)
        return pltpu.make_async_copy(wo_hbm.bitcast(U32).at[heads], wo_v.at[heads], osem_w.at[t])

    def fcopy(t):
        if t == 0:
            return pltpu.make_async_copy(wg_hbm, wg_v, fsem.at[0])
        if t == 1:
            return pltpu.make_async_copy(wu_hbm, wu_v, fsem.at[1])
        if t == 2:
            return pltpu.make_async_copy(wd_hbm, wd_v.at[:, 0:M], fsem.at[2])
        return pltpu.make_async_copy(wr_hbm, wr_ref, fsem.at[3])

    def ocopy(g):
        rows = pl.ds(g * OB, OB)
        return pltpu.make_async_copy(io_v.at[rows, :], out_hbm.at[0, rows, :], osem.at[g])

    def project(dst, lhs, w32, rows, mult=None):
        y = jnp.dot(lhs, _unpack_pair(w32), preferred_element_type=F32)
        if mult is not None:
            y = y * mult
        _Packed(dst.at[0])[rows, ALL] = y[:, :D]
        _Packed(dst.at[1])[rows, ALL] = y[:, D:]

    NXB = S // XB
    wstart(0, 0)
    for b in range(NXB):
        ccopy(b).start()
        xcopy(b).start()
    wocopy(0).start()
    fcopy(3).start()
    wstart(1, 1)
    wwait(0)

    def first(b, carry):
        ccopy(b).wait()
        xcopy(b).wait()
        rows = pl.ds(pl.multiple_of(b * XB, XB), XB)
        xf = io_v[rows, :].astype(F32)
        mu = jnp.mean(xf, axis=1, keepdims=True)
        xc = xf - mu
        var = jnp.mean(xc * xc, axis=1, keepdims=True)
        xn = (xc * lax.rsqrt(var + 1e-5)).astype(BF16)
        prow = (b * XB, XB, XB)
        xn_p[prow, ALL] = xn
        acc_s[rows, :] = xc
        mux_s[rows, :] = jnp.broadcast_to(mu, (XB, 128))
        c = c_p[prow, ALL]
        project(k_s, c, w_b[0, KR, :], prow)
        project(v_s, c, w_b[0, VR, :], prow)
        project(q_s, xn, w_b[0, QR, :], prow, scale)
        return carry
    lax.fori_loop(0, S // XB, first, 0)
    wstart(2, 0)
    wocopy(1).start()
    for t in range(3):
        fcopy(t).start()
    wocopy(0).wait()

    def step(j, carry):
        slot = j & 1

        @pl.when(j == 1)
        def _():
            wocopy(1).wait()

        wwait(1 - slot)

        @pl.when(jnp.logical_and(j >= 1, j + 2 < NP))
        def _():
            wstart(j + 2, slot)

        wo = pltpu.bitcast(wo_v[pl.ds(2 * j, 2)].reshape(D, M), BF16)

        def oproj(ii, pair_ctx):
            acc_s[ii * TQ:(ii + 1) * TQ, :] += jnp.dot(pair_ctx(ii), wo, preferred_element_type=F32)

        def rows_of(code):
            return slice((code // 10) * TQ, (code % 10 + 1) * TQ)

        _attn_pair(q_s, k_s, v_s, ORDER_MAIN, {
            'O': oproj,
            'K': lambda code, _: project(k_s, c_p[rows_of(code), ALL], w_b[1 - slot, KR, :], rows_of(code)),
            'V': lambda code, _: project(v_s, c_p[rows_of(code), ALL], w_b[1 - slot, VR, :], rows_of(code)),
            'Q': lambda code, _: project(q_s, xn_p[rows_of(code), ALL], w_b[1 - slot, QR, :], rows_of(code), scale),
        })
        return carry
    lax.fori_loop(0, NP - 1, step, 0)

    for t in range(4):
        fcopy(t).wait()
    eps = jnp.asarray(1e-5, BF16).astype(F32)

    def last_head(h, carry):
        sc = {}
        for tok in ORDER_LAST.split():
            i = int(tok[1])
            if tok[0] == 'S':
                sc[i] = _qk(_Packed(q_s.at[h]), _Packed(k_s.at[h]), i)
            else:
                _Packed(ctx_s.at[h])[slice(i * TQ, (i + 1) * TQ), ALL] = _pv(
                    _softmax(sc.pop(i), i), _Packed(v_s.at[h]), i)
        return carry
    lax.fori_loop(0, 2, last_head, 0)

    CW = M // NCH
    RW = M // RG
    wr16 = [jnp.broadcast_to(wr_ref[t * RW:(t + 1) * RW].astype(F32).reshape(1, RW), (16, RW)).astype(BF16)
            for t in range(RG)]

    def oproj_part(r0, t):
        rows = slice(r0, r0 + EB)
        cols = slice(t * CW, (t + 1) * CW)
        return (acc_s[rows, cols]
                + jnp.dot(_Packed(ctx_s.at[0])[rows, ALL], pltpu.bitcast(wo_v[2 * NP - 2, :, cols], BF16),
                           preferred_element_type=F32)
                + jnp.dot(_Packed(ctx_s.at[1])[rows, ALL], pltpu.bitcast(wo_v[2 * NP - 1, :, cols], BF16),
                           preferred_element_type=F32))

    def ln2(r0, a):
        rows = slice(r0, r0 + EB)
        acc_s[rows, :] = a
        s1 = jnp.mean(a, axis=1, keepdims=True)
        var = jnp.maximum(jnp.mean(a * a, axis=1, keepdims=True) - s1 * s1, 0.0)
        ve = _rb(_rb(var) + eps)
        den = _rb(ve * lax.rsqrt(ve))
        inv = _recip(den)
        inv = inv * (2.0 - den * inv)
        mux = mux_s[rows, :]
        c1 = (_rb(mux + s1) - mux) * inv
        c2 = mux - c1
        a = acc_s[rows, :]
        t = a * inv
        xn_p[rows, ALL] = t - jnp.concatenate([c1] * (M // 128), axis=1)
        io_v[rows, :] = ((a + t) + jnp.concatenate([c2] * (M // 128), axis=1)).astype(BF16)

    def router_part(r0, t):
        cols = slice(t * RW, (t + 1) * RW)
        return lax.dot_general(wr16[t], xn_p[slice(r0, r0 + EB), cols], NT, preferred_element_type=F32)

    neb = S // EB
    rparts = []
    for k in range(neb + RLAG):
        hp, rp = [], None
        for t in range(NCH):
            if k < neb:
                hp.append(oproj_part(k * EB, t))
            if k >= RLAG and t < RG:
                part = router_part((k - RLAG) * EB, t)[0:8, :]
                rp = part if rp is None else rp + part
        if k > 0 and k <= neb and (k * EB) % OB == 0:
            ocopy(k * EB // OB - 1).start()
        if k < neb:
            ln2(k * EB, jnp.concatenate(hp, axis=1))
        if k >= RLAG:
            rparts.append(rp)
    rrow = _rb(jnp.concatenate(rparts, axis=1))

    I32 = jnp.int32
    b16 = lax.shift_right_logical(pltpu.bitcast(rrow, I32), 16)
    rank = jnp.where(b16 >= 0x8000, 0x10000 - b16, 0x8000 + b16)
    lane = lax.broadcasted_iota(I32, rrow.shape, 1)
    key = pltpu.bitcast(rank * S + (S - 1 - lane) + 0x20000000, F32)
    k1 = jnp.max(key, axis=1, keepdims=True)
    k2 = jnp.max(jnp.where(key == k1, 0.0, key), axis=1, keepdims=True)
    i1 = (S - 1) - (pltpu.bitcast(k1, I32)[0, 0] & (S - 1))
    i2 = (S - 1) - (pltpu.bitcast(k2, I32)[0, 0] & (S - 1))
    m1 = jnp.max(jnp.where(key == k1, rrow, -jnp.inf), axis=1, keepdims=True)[0:1, :]
    m2 = jnp.max(jnp.where(key == k2, rrow, -jnp.inf), axis=1, keepdims=True)[0:1, :]
    g1 = pl.multiple_of((i1 // 16) * 16, 16)
    g2 = pl.multiple_of((i2 // 16) * 16, 16)

    rid = lax.broadcasted_iota(jnp.int32, (16, M), 0)

    def pick(g, i):
        blk = xn_p[(g, 16, 16), ALL].astype(F32)
        return jnp.sum(jnp.where(rid == i - g, blk, 0.0), axis=0, keepdims=True)

    xs = jnp.where(rid == 0, pick(g1, i1), pick(g2, i2))
    xsb = xs.astype(BF16)
    ocopy(0).wait()
    nch = FF // FC
    acts, y = [], None
    for t in range(nch + 1):
        if t < nch:
            cols = slice(t * FC, (t + 1) * FC)
            a = _rb(jnp.dot(xsb, wg_v[:, cols], preferred_element_type=F32))
            u = _rb(jnp.dot(xsb, wu_v[:, cols], preferred_element_type=F32))
            g = _rb(a * _rb(jax.nn.sigmoid(a)))
            acts.append((g * u).astype(BF16))
        if t > 0:
            yt = jnp.dot(acts[t - 1], wd_v[(t - 1) * FC:t * FC, 0:M], preferred_element_type=F32)
            y = yt if y is None else y + yt
    rsel = jnp.where(rid == 0, m1, m2)
    y = _rb(_rb(y) * _rb(jax.nn.sigmoid(rsel)))
    upd = _rb(xs + y)

    for k, gg in enumerate((g1, g2)):
        rows = pl.ds(gg, 16)
        hb = _rb(acc_s[rows, :] + jnp.concatenate([mux_s[rows, :]] * (M // 128), axis=1))
        val = jnp.where(rid == i1 - gg, hb + upd[0:1, :],
                        jnp.where(rid == i2 - gg, hb + upd[1:2, :], io_v[rows, :].astype(F32)))
        pt_v[k] = val.astype(BF16)

    def pcopy(g, k):
        return pltpu.make_async_copy(pt_v.at[k], out_hbm.at[0, pl.ds(g, 16), :], osem.at[k])

    for b in range(1, S // OB):
        ocopy(b).wait()
    pcopy(g1, 0).start()

    @pl.when(g2 != g1)
    def _():
        pcopy(g2, 1).start()
        pcopy(g2, 1).wait()
    pcopy(g1, 0).wait()


@jax.jit
def pallas_sequential_preLN__compressed_kv_cla__moe_arch_mod__prompt_kernel(
    A_x: jax.Array,
    A_c_kv: jax.Array,
    A_w_q: jax.Array,
    A_w_uk: jax.Array,
    A_w_uv: jax.Array,
    A_w_o: jax.Array,
    B_x: jax.Array,
    B_w_r: jax.Array,
    B_w_gate: jax.Array,
    B_w_up: jax.Array,
    B_w_down: jax.Array,
):
    _, S, M = A_x.shape
    C = A_c_kv.shape[2]
    H, D = A_w_q.shape[1], A_w_q.shape[2]
    FF = B_w_gate.shape[1]
    NP = H // 2
    any_spec = pl.BlockSpec(memory_space=pl.ANY)
    return pl.pallas_call(
        functools.partial(_kernel, S=S, M=M, C=C, D=D, NP=NP, FF=FF),
        in_specs=[
            any_spec, any_spec, any_spec, any_spec, any_spec, any_spec,
            any_spec, any_spec, any_spec, any_spec,
        ],
        out_specs=any_spec,
        out_shape=jax.ShapeDtypeStruct((1, S, M), BF16),
        scratch_shapes=[
            pltpu.VMEM((S, M), BF16),
            pltpu.VMEM((2, 16, M), BF16),
            pltpu.VMEM((S // 2, C), U32),
            pltpu.VMEM((S // 2, M), U32),
            pltpu.VMEM((S, M), F32),
            pltpu.VMEM((S, 128), F32),
            pltpu.VMEM((2, S // 2, D), U32),
            pltpu.VMEM((2, S // 2, D), U32),
            pltpu.VMEM((2, S // 2, D), U32),
            pltpu.VMEM((2, S // 2, D), U32),
            pltpu.VMEM((2, 2 * C + M, D), U32),
            pltpu.VMEM((H, D // 2, M), U32),
            pltpu.VMEM((M,), BF16),
            pltpu.VMEM((M, FF), BF16),
            pltpu.VMEM((M, FF), BF16),
            pltpu.VMEM((FF, M + 128), BF16),
            pltpu.SemaphoreType.DMA((S // XB,)),
            pltpu.SemaphoreType.DMA((S // XB,)),
            pltpu.SemaphoreType.DMA((2,)),
            pltpu.SemaphoreType.DMA((2,)),
            pltpu.SemaphoreType.DMA((4,)),
            pltpu.SemaphoreType.DMA((S // OB,)),
        ],
        compiler_params=pltpu.CompilerParams(
            vmem_limit_bytes=110 * 1024 * 1024,
            disable_bounds_checks=True,
            disable_semaphore_checks=True,
        ),
    )(A_x, A_c_kv, A_w_q, A_w_uk, A_w_uv, A_w_o, B_w_r, B_w_gate, B_w_up, B_w_down)
```

```python
import functools
import math

import jax
import jax.numpy as jnp
from jax import lax
import jax.experimental.pallas as pl
import jax.experimental.pallas.tpu as pltpu

F32 = jnp.float32
BF16 = jnp.bfloat16
U32 = jnp.uint32
NEG = -1e30
NT = (((1,), (1,)), ((), ()))
TQ = 512
SUB = 128
GRP = 4
XB = 256
EB = 128
OB = 512
NCH = 4
RG = 2
RLAG = 2
FC = 512

ORDER_MAIN = ("S03 S13 P03 K33 S02 P13 S12 P02 S01 P12 S11 Q23 S00 P01 P11 S10 K02 P00 P10 "
              "O3 Q01 O2 O1 O0 V03")
ORDER_LAST = "S2 S3 P2 S1 P3 S0 P1 P0"


def _rb(v):
    return v.astype(BF16).astype(F32)


def _recip(l):
    return pl.reciprocal(l, approx=True)


def _unpack_pair(w32):
    lo = pltpu.bitcast(w32 << 16, F32)
    hi = pltpu.bitcast(w32 & jnp.uint32(0xFFFF0000), F32)
    return jnp.concatenate([lo, hi], axis=1).astype(BF16)


class _Packed:
    def __init__(self, ref):
        self.ref = ref

    @staticmethod
    def half(rows):
        if isinstance(rows, slice):
            return slice(rows.start // 2, rows.stop // 2)
        start, size, align = rows
        return pl.ds(pl.multiple_of(start // 2, align // 2), size // 2)

    def __getitem__(self, idx):
        rows, cols = idx
        return pltpu.bitcast(self.ref[self.half(rows), cols], BF16)

    def __setitem__(self, idx, val):
        rows, cols = idx
        self.ref[self.half(rows), cols] = pltpu.bitcast(val.astype(BF16), U32)


def _qk(q, k, i):
    r0 = i * TQ
    nb = TQ // SUB
    qb = q[r0:r0 + TQ, :]
    s_main = lax.dot_general(qb, k[0:r0 + SUB, :], NT, preferred_element_type=F32)
    s_ext = [lax.dot_general(qb[c * SUB:, :], k[r0 + c * SUB:r0 + (c + 1) * SUB, :], NT,
                             preferred_element_type=F32) for c in range(1, nb)]
    return s_main, s_ext


def _softmax(s, i):
    s_main, s_ext = s
    r0 = i * TQ
    nb = TQ // SUB
    row = lax.broadcasted_iota(jnp.int32, (SUB, SUB), 0)
    col = lax.broadcasted_iota(jnp.int32, (SUB, SUB), 1)
    tri = col <= row
    p_main, p_ext, ls = [], [[] for _ in range(1, nb)], []
    for b in range(nb):
        sm = s_main[b * SUB:(b + 1) * SUB, :]
        if b == 0:
            d = jnp.where(tri, sm[:, r0:], NEG)
            sm = jnp.concatenate([sm[:, :r0], d], axis=1) if r0 > 0 else d
        parts = [sm]
        for c in range(1, b + 1):
            e = s_ext[c - 1][(b - c) * SUB:(b - c + 1) * SUB, :]
            if c == b:
                e = jnp.where(tri, e, NEG)
            parts.append(e)
        sb = jnp.concatenate(parts, axis=1) if len(parts) > 1 else parts[0]
        m = jnp.max(sb, axis=1, keepdims=True)
        p = jnp.exp2(sb - m)
        nt = p.shape[1] // SUB
        tiles = [p[:, t * SUB:(t + 1) * SUB] for t in range(nt)]
        acc = None
        for t0 in range(0, nt, GRP):
            grp = tiles[t0:t0 + GRP]
            tot = grp[0]
            for g in grp[1:]:
                tot = tot + g
            acc = tot if acc is None else acc + tot
            last = t0 + len(grp) - 1
            if acc is not tiles[last]:
                tiles[last] = jnp.minimum(tiles[last], acc)
        p = jnp.concatenate(tiles, axis=1) if nt > 1 else tiles[0]
        ls.append(jnp.sum(acc, axis=1, keepdims=True))
        p_main.append(p[:, :r0 + SUB])
        for c in range(1, b + 1):
            p_ext[c - 1].append(p[:, r0 + c * SUB:r0 + (c + 1) * SUB])
    pm = jnp.concatenate(p_main, axis=0).astype(BF16)
    pe = [(jnp.concatenate(e, axis=0) if len(e) > 1 else e[0]).astype(BF16) for e in p_ext]
    return pm, pe, ls


def _pv(p, v, i):
    pm, pe, ls = p
    r0 = i * TQ
    nb = TQ // SUB
    o = jnp.dot(pm, v[0:r0 + SUB, :], preferred_element_type=F32)
    os_ = [o[b * SUB:(b + 1) * SUB] for b in range(nb)]
    for c in range(1, nb):
        oe = jnp.dot(pe[c - 1], v[r0 + c * SUB:r0 + (c + 1) * SUB, :], preferred_element_type=F32)
        for b in range(c, nb):
            os_[b] = os_[b] + oe[(b - c) * SUB:(b - c + 1) * SUB]
    return jnp.concatenate([os_[b] * _recip(ls[b]) for b in range(nb)], axis=0)


def _attn_pair(q_s, k_s, v_s, order, actions):
    sc, ctx = {}, {}

    def pair_ctx(i):
        return jnp.concatenate([ctx[(0, i)], ctx[(1, i)]], axis=1).astype(BF16)

    for tok in order.split():
        if tok[0] == 'S':
            h, i = int(tok[1]), int(tok[2])
            sc[(h, i)] = _qk(_Packed(q_s.at[h]), _Packed(k_s.at[h]), i)
        elif tok[0] == 'P':
            h, i = int(tok[1]), int(tok[2])
            ctx[(h, i)] = _pv(_softmax(sc.pop((h, i)), i), _Packed(v_s.at[h]), i)
        else:
            actions[tok[0]](int(tok[1:]), pair_ctx)


def _kernel(x_hbm, c_hbm, wq_hbm, wk_hbm, wv_hbm, wo_hbm, wr_hbm, wg_hbm, wu_hbm, wd_hbm,
            out_hbm,
            io_v, pt_v, c_v, xn_s, acc_s, mux_s, ctx_s, q_s, k_s, v_s,
            w_b, wo_v, wr_ref, wg_v, wu_v, wd_v,
            xsem, csem, wsem, osem_w, fsem, osem,
            *, S, M, C, D, NP, FF):
    ALL = slice(None)
    xn_p, c_p = _Packed(xn_s), _Packed(c_v)
    scale = (D ** -0.5) * math.log2(math.e)

    def xcopy(b):
        rows = pl.ds(pl.multiple_of(b * XB, XB), XB)
        return pltpu.make_async_copy(x_hbm.at[0, rows, :], io_v.at[rows, :], xsem.at[b])

    def ccopy(b):
        rows = pl.ds(pl.multiple_of(b * (XB // 2), XB // 2), XB // 2)
        return pltpu.make_async_copy(c_hbm.bitcast(U32).at[0, rows, :], c_v.at[rows, :], csem.at[b])

    KR, VR, QR = slice(0, C), slice(C, 2 * C), slice(2 * C, 2 * C + M)

    def wstart(jj, sl):
        for src, rows in ((wk_hbm, KR), (wv_hbm, VR), (wq_hbm, QR)):
            pltpu.make_async_copy(src.bitcast(U32).at[:, jj, :], w_b.at[sl, rows, :], wsem.at[sl]).start()

    def wwait(sl):
        pltpu.make_async_copy(w_b.at[sl], w_b.at[sl], wsem.at[sl]).wait()

    def wocopy(t):
        heads = pl.ds(0, 2) if t == 0 else pl.ds(2, 2 * NP - 2)
        return pltpu.make_async_copy(wo_hbm.bitcast(U32).at[heads], wo_v.at[heads], osem_w.at[t])

    def fcopy(t):
        if t == 0:
            return pltpu.make_async_copy(wg_hbm, wg_v, fsem.at[0])
        if t == 1:
            return pltpu.make_async_copy(wu_hbm, wu_v, fsem.at[1])
        if t == 2:
            return pltpu.make_async_copy(wd_hbm, wd_v.at[:, 0:M], fsem.at[2])
        return pltpu.make_async_copy(wr_hbm, wr_ref, fsem.at[3])

    def ocopy(g):
        rows = pl.ds(g * OB, OB)
        return pltpu.make_async_copy(io_v.at[rows, :], out_hbm.at[0, rows, :], osem.at[g])

    def project(dst, lhs, w32, rows, mult=None):
        y = jnp.dot(lhs, _unpack_pair(w32), preferred_element_type=F32)
        if mult is not None:
            y = y * mult
        _Packed(dst.at[0])[rows, ALL] = y[:, :D]
        _Packed(dst.at[1])[rows, ALL] = y[:, D:]

    NXB = S // XB
    wstart(0, 0)
    for b in range(NXB):
        ccopy(b).start()
        xcopy(b).start()
    wocopy(0).start()
    fcopy(3).start()
    wstart(1, 1)
    wwait(0)

    def first(b, carry):
        ccopy(b).wait()
        xcopy(b).wait()
        rows = pl.ds(pl.multiple_of(b * XB, XB), XB)
        xf = io_v[rows, :].astype(F32)
        mu = jnp.mean(xf, axis=1, keepdims=True)
        xc = xf - mu
        var = jnp.mean(xc * xc, axis=1, keepdims=True)
        xn = (xc * lax.rsqrt(var + 1e-5)).astype(BF16)
        prow = (b * XB, XB, XB)
        xn_p[prow, ALL] = xn
        acc_s[rows, :] = xc
        mux_s[rows, :] = jnp.broadcast_to(mu, (XB, 128))
        c = c_p[prow, ALL]
        project(k_s, c, w_b[0, KR, :], prow)
        project(v_s, c, w_b[0, VR, :], prow)
        project(q_s, xn, w_b[0, QR, :], prow, scale)
        return carry
    lax.fori_loop(0, S // XB, first, 0)
    wstart(2, 0)
    wocopy(1).start()
    for t in range(3):
        fcopy(t).start()
    wocopy(0).wait()

    def step(j, carry):
        slot = j & 1

        @pl.when(j == 1)
        def _():
            wocopy(1).wait()

        wwait(1 - slot)

        @pl.when(jnp.logical_and(j >= 1, j + 2 < NP))
        def _():
            wstart(j + 2, slot)

        wo = pltpu.bitcast(wo_v[pl.ds(2 * j, 2)].reshape(D, M), BF16)

        def oproj(ii, pair_ctx):
            acc_s[ii * TQ:(ii + 1) * TQ, :] += jnp.dot(pair_ctx(ii), wo, preferred_element_type=F32)

        def rows_of(code):
            return slice((code // 10) * TQ, (code % 10 + 1) * TQ)

        _attn_pair(q_s, k_s, v_s, ORDER_MAIN, {
            'O': oproj,
            'K': lambda code, _: project(k_s, c_p[rows_of(code), ALL], w_b[1 - slot, KR, :], rows_of(code)),
            'V': lambda code, _: project(v_s, c_p[rows_of(code), ALL], w_b[1 - slot, VR, :], rows_of(code)),
            'Q': lambda code, _: project(q_s, xn_p[rows_of(code), ALL], w_b[1 - slot, QR, :], rows_of(code), scale),
        })
        return carry
    lax.fori_loop(0, NP - 1, step, 0)

    for t in range(4):
        fcopy(t).wait()
    eps = jnp.asarray(1e-5, BF16).astype(F32)

    def last_head(h, carry):
        sc = {}
        for tok in ORDER_LAST.split():
            i = int(tok[1])
            if tok[0] == 'S':
                sc[i] = _qk(_Packed(q_s.at[h]), _Packed(k_s.at[h]), i)
            else:
                _Packed(ctx_s.at[h])[slice(i * TQ, (i + 1) * TQ), ALL] = _pv(
                    _softmax(sc.pop(i), i), _Packed(v_s.at[h]), i)
        return carry
    lax.fori_loop(0, 2, last_head, 0)

    CW = M // NCH
    RW = M // RG
    wr16 = [jnp.broadcast_to(wr_ref[t * RW:(t + 1) * RW].astype(F32).reshape(1, RW), (16, RW)).astype(BF16)
            for t in range(RG)]

    def oproj_part(r0, t):
        rows = slice(r0, r0 + EB)
        cols = slice(t * CW, (t + 1) * CW)
        return (acc_s[rows, cols]
                + jnp.dot(_Packed(ctx_s.at[0])[rows, ALL], pltpu.bitcast(wo_v[2 * NP - 2, :, cols], BF16),
                           preferred_element_type=F32)
                + jnp.dot(_Packed(ctx_s.at[1])[rows, ALL], pltpu.bitcast(wo_v[2 * NP - 1, :, cols], BF16),
                           preferred_element_type=F32))

    def ln2(r0, a):
        rows = slice(r0, r0 + EB)
        acc_s[rows, :] = a
        s1 = jnp.mean(a, axis=1, keepdims=True)
        var = jnp.maximum(jnp.mean(a * a, axis=1, keepdims=True) - s1 * s1, 0.0)
        ve = _rb(_rb(var) + eps)
        den = _rb(ve * lax.rsqrt(ve))
        inv = _recip(den)
        inv = inv * (2.0 - den * inv)
        mux = mux_s[rows, :]
        c1 = (_rb(mux + s1) - mux) * inv
        c2 = mux - c1
        a = acc_s[rows, :]
        t = a * inv
        xn_p[rows, ALL] = t - jnp.concatenate([c1] * (M // 128), axis=1)
        io_v[rows, :] = ((a + t) + jnp.concatenate([c2] * (M // 128), axis=1)).astype(BF16)

    def router_part(r0, t):
        cols = slice(t * RW, (t + 1) * RW)
        return lax.dot_general(wr16[t], xn_p[slice(r0, r0 + EB), cols], NT, preferred_element_type=F32)

    neb = S // EB
    rparts = []
    for k in range(neb + RLAG):
        hp, rp = [], None
        for t in range(NCH):
            if k < neb:
                hp.append(oproj_part(k * EB, t))
            if k >= RLAG and t < RG:
                part = router_part((k - RLAG) * EB, t)[0:8, :]
                rp = part if rp is None else rp + part
        if k > 0 and k <= neb and (k * EB) % OB == 0:
            ocopy(k * EB // OB - 1).start()
        if k < neb:
            ln2(k * EB, jnp.concatenate(hp, axis=1))
        if k >= RLAG:
            rparts.append(rp)
    rrow = _rb(jnp.concatenate(rparts, axis=1))

    I32 = jnp.int32
    b16 = lax.shift_right_logical(pltpu.bitcast(rrow, I32), 16)
    rank = jnp.where(b16 >= 0x8000, 0x10000 - b16, 0x8000 + b16)
    lane = lax.broadcasted_iota(I32, rrow.shape, 1)
    key = pltpu.bitcast(rank * S + (S - 1 - lane) + 0x20000000, F32)
    k1 = jnp.max(key, axis=1, keepdims=True)
    k2 = jnp.max(jnp.where(key == k1, 0.0, key), axis=1, keepdims=True)
    i1 = (S - 1) - (pltpu.bitcast(k1, I32)[0, 0] & (S - 1))
    i2 = (S - 1) - (pltpu.bitcast(k2, I32)[0, 0] & (S - 1))
    m1 = jnp.max(jnp.where(key == k1, rrow, -jnp.inf), axis=1, keepdims=True)[0:1, :]
    m2 = jnp.max(jnp.where(key == k2, rrow, -jnp.inf), axis=1, keepdims=True)[0:1, :]
    g1 = pl.multiple_of((i1 // 16) * 16, 16)
    g2 = pl.multiple_of((i2 // 16) * 16, 16)

    rid = lax.broadcasted_iota(jnp.int32, (16, M), 0)

    def pick(g, i):
        blk = xn_p[(g, 16, 16), ALL].astype(F32)
        return jnp.sum(jnp.where(rid == i - g, blk, 0.0), axis=0, keepdims=True)

    xs = jnp.where(rid == 0, pick(g1, i1), pick(g2, i2))
    xsb = xs.astype(BF16)
    ocopy(0).wait()
    nch = FF // FC
    acts, y = [], None
    for t in range(nch + 1):
        if t < nch:
            cols = slice(t * FC, (t + 1) * FC)
            a = _rb(jnp.dot(xsb, wg_v[:, cols], preferred_element_type=F32))
            u = _rb(jnp.dot(xsb, wu_v[:, cols], preferred_element_type=F32))
            g = _rb(a * _rb(jax.nn.sigmoid(a)))
            acts.append((g * u).astype(BF16))
        if t > 0:
            yt = jnp.dot(acts[t - 1], wd_v[(t - 1) * FC:t * FC, 0:M], preferred_element_type=F32)
            y = yt if y is None else y + yt
    rsel = jnp.where(rid == 0, m1, m2)
    y = _rb(_rb(y) * _rb(jax.nn.sigmoid(rsel)))
    upd = _rb(xs + y)

    for k, gg in enumerate((g1, g2)):
        rows = pl.ds(gg, 16)
        hb = _rb(acc_s[rows, :] + jnp.concatenate([mux_s[rows, :]] * (M // 128), axis=1))
        val = jnp.where(rid == i1 - gg, hb + upd[0:1, :],
                        jnp.where(rid == i2 - gg, hb + upd[1:2, :], io_v[rows, :].astype(F32)))
        pt_v[k] = val.astype(BF16)

    def pcopy(g, k):
        return pltpu.make_async_copy(pt_v.at[k], out_hbm.at[0, pl.ds(g, 16), :], osem.at[k])

    for b in range(1, S // OB):
        ocopy(b).wait()
    pcopy(g1, 0).start()

    @pl.when(g2 != g1)
    def _():
        pcopy(g2, 1).start()
        pcopy(g2, 1).wait()
    pcopy(g1, 0).wait()


def _compiler_params():
    vmem = 110 * 1024 * 1024
    try:
        return pltpu.CompilerParams(vmem_limit_bytes=vmem, disable_bounds_checks=True,
                                    disable_semaphore_checks=True)
    except TypeError:
        return pltpu.CompilerParams(vmem_limit_bytes=vmem, disable_bounds_checks=True)


@jax.jit
def pallas_sequential_preLN__compressed_kv_cla__moe_arch_mod__prompt_kernel(
    A_x: jax.Array,
    A_c_kv: jax.Array,
    A_w_q: jax.Array,
    A_w_uk: jax.Array,
    A_w_uv: jax.Array,
    A_w_o: jax.Array,
    B_x: jax.Array,
    B_w_r: jax.Array,
    B_w_gate: jax.Array,
    B_w_up: jax.Array,
    B_w_down: jax.Array,
):
    _, S, M = A_x.shape
    C = A_c_kv.shape[2]
    H, D = A_w_q.shape[1], A_w_q.shape[2]
    FF = B_w_gate.shape[1]
    NP = H // 2
    any_spec = pl.BlockSpec(memory_space=pl.ANY)
    return pl.pallas_call(
        functools.partial(_kernel, S=S, M=M, C=C, D=D, NP=NP, FF=FF),
        in_specs=[
            any_spec, any_spec, any_spec, any_spec, any_spec, any_spec,
            any_spec, any_spec, any_spec, any_spec,
        ],
        out_specs=any_spec,
        out_shape=jax.ShapeDtypeStruct((1, S, M), BF16),
        scratch_shapes=[
            pltpu.VMEM((S, M), BF16),
            pltpu.VMEM((2, 16, M), BF16),
            pltpu.VMEM((S // 2, C), U32),
            pltpu.VMEM((S // 2, M), U32),
            pltpu.VMEM((S, M), F32),
            pltpu.VMEM((S, 128), F32),
            pltpu.VMEM((2, S // 2, D), U32),
            pltpu.VMEM((2, S // 2, D), U32),
            pltpu.VMEM((2, S // 2, D), U32),
            pltpu.VMEM((2, S // 2, D), U32),
            pltpu.VMEM((2, 2 * C + M, D), U32),
            pltpu.VMEM((H, D // 2, M), U32),
            pltpu.VMEM((M,), BF16),
            pltpu.VMEM((M, FF), BF16),
            pltpu.VMEM((M, FF), BF16),
            pltpu.VMEM((FF, M + 128), BF16),
            pltpu.SemaphoreType.DMA((S // XB,)),
            pltpu.SemaphoreType.DMA((S // XB,)),
            pltpu.SemaphoreType.DMA((2,)),
            pltpu.SemaphoreType.DMA((2,)),
            pltpu.SemaphoreType.DMA((4,)),
            pltpu.SemaphoreType.DMA((S // OB,)),
        ],
        compiler_params=_compiler_params(),
    )(A_x, A_c_kv, A_w_q, A_w_uk, A_w_uv, A_w_o, B_w_r, B_w_gate, B_w_up, B_w_down)
```

```python
import functools
import math

import jax
import jax.numpy as jnp
from jax import lax
import jax.experimental.pallas as pl
import jax.experimental.pallas.tpu as pltpu

F32 = jnp.float32
BF16 = jnp.bfloat16
U32 = jnp.uint32
NEG = -1e30
NT = (((1,), (1,)), ((), ()))
TQ = 512
SUB = 128
GRP = 4
XB = 256
EB = 128
OB = 512
NCH = 4
RG = 2
RLAG = 2
FC = 512

ORDER_MAIN = ("S03 S13 P03 K33 S02 P13 S12 P02 S01 P12 S11 Q23 S00 P01 P11 S10 K02 P00 P10 "
              "O3 Q01 O2 O1 O0 V03")
ORDER_LAST = "S2 S3 P2 S1 P3 S0 P1 P0"


def _rb(v):
    return v.astype(BF16).astype(F32)


def _recip(l):
    return pl.reciprocal(l, approx=True)


def _unpack_pair(w32):
    lo = pltpu.bitcast(w32 << 16, F32)
    hi = pltpu.bitcast(w32 & jnp.uint32(0xFFFF0000), F32)
    return jnp.concatenate([lo, hi], axis=1).astype(BF16)


class _Packed:
    def __init__(self, ref):
        self.ref = ref

    @staticmethod
    def half(rows):
        if isinstance(rows, slice):
            return slice(rows.start // 2, rows.stop // 2)
        blk, size = rows
        return pl.ds(pl.multiple_of(blk * (size // 2), size // 2), size // 2)

    def __getitem__(self, idx):
        rows, cols = idx
        return pltpu.bitcast(self.ref[self.half(rows), cols], BF16)

    def __setitem__(self, idx, val):
        rows, cols = idx
        self.ref[self.half(rows), cols] = pltpu.bitcast(val.astype(BF16), U32)


def _qk(q, k, i):
    r0 = i * TQ
    nb = TQ // SUB
    qb = q[r0:r0 + TQ, :]
    s_main = lax.dot_general(qb, k[0:r0 + SUB, :], NT, preferred_element_type=F32)
    s_ext = [lax.dot_general(qb[c * SUB:, :], k[r0 + c * SUB:r0 + (c + 1) * SUB, :], NT,
                             preferred_element_type=F32) for c in range(1, nb)]
    return s_main, s_ext


def _softmax(s, i):
    s_main, s_ext = s
    r0 = i * TQ
    nb = TQ // SUB
    row = lax.broadcasted_iota(jnp.int32, (SUB, SUB), 0)
    col = lax.broadcasted_iota(jnp.int32, (SUB, SUB), 1)
    tri = col <= row
    p_main, p_ext, ls = [], [[] for _ in range(1, nb)], []
    for b in range(nb):
        sm = s_main[b * SUB:(b + 1) * SUB, :]
        if b == 0:
            d = jnp.where(tri, sm[:, r0:], NEG)
            sm = jnp.concatenate([sm[:, :r0], d], axis=1) if r0 > 0 else d
        parts = [sm]
        for c in range(1, b + 1):
            e = s_ext[c - 1][(b - c) * SUB:(b - c + 1) * SUB, :]
            if c == b:
                e = jnp.where(tri, e, NEG)
            parts.append(e)
        sb = jnp.concatenate(parts, axis=1) if len(parts) > 1 else parts[0]
        m = jnp.max(sb, axis=1, keepdims=True)
        p = jnp.exp2(sb - m)
        nt = p.shape[1] // SUB
        tiles = [p[:, t * SUB:(t + 1) * SUB] for t in range(nt)]
        acc = None
        for t0 in range(0, nt, GRP):
            grp = tiles[t0:t0 + GRP]
            tot = grp[0]
            for g in grp[1:]:
                tot = tot + g
            acc = tot if acc is None else acc + tot
            last = t0 + len(grp) - 1
            if acc is not tiles[last]:
                tiles[last] = jnp.minimum(tiles[last], acc)
        p = jnp.concatenate(tiles, axis=1) if nt > 1 else tiles[0]
        ls.append(jnp.sum(acc, axis=1, keepdims=True))
        p_main.append(p[:, :r0 + SUB])
        for c in range(1, b + 1):
            p_ext[c - 1].append(p[:, r0 + c * SUB:r0 + (c + 1) * SUB])
    pm = jnp.concatenate(p_main, axis=0).astype(BF16)
    pe = [(jnp.concatenate(e, axis=0) if len(e) > 1 else e[0]).astype(BF16) for e in p_ext]
    return pm, pe, ls


def _pv(p, v, i):
    pm, pe, ls = p
    r0 = i * TQ
    nb = TQ // SUB
    o = jnp.dot(pm, v[0:r0 + SUB, :], preferred_element_type=F32)
    os_ = [o[b * SUB:(b + 1) * SUB] for b in range(nb)]
    for c in range(1, nb):
        oe = jnp.dot(pe[c - 1], v[r0 + c * SUB:r0 + (c + 1) * SUB, :], preferred_element_type=F32)
        for b in range(c, nb):
            os_[b] = os_[b] + oe[(b - c) * SUB:(b - c + 1) * SUB]
    return jnp.concatenate([os_[b] * _recip(ls[b]) for b in range(nb)], axis=0)


def _attn_pair(q_s, k_s, v_s, order, actions):
    sc, ctx = {}, {}

    def pair_ctx(i):
        return jnp.concatenate([ctx[(0, i)], ctx[(1, i)]], axis=1).astype(BF16)

    for tok in order.split():
        if tok[0] == 'S':
            h, i = int(tok[1]), int(tok[2])
            sc[(h, i)] = _qk(_Packed(q_s.at[h]), _Packed(k_s.at[h]), i)
        elif tok[0] == 'P':
            h, i = int(tok[1]), int(tok[2])
            ctx[(h, i)] = _pv(_softmax(sc.pop((h, i)), i), _Packed(v_s.at[h]), i)
        else:
            actions[tok[0]](int(tok[1:]), pair_ctx)


def _kernel(x_hbm, c_hbm, wq_hbm, wk_hbm, wv_hbm, wo_hbm, wr_hbm, wg_hbm, wu_hbm, wd_hbm,
            out_hbm,
            io_v, pt_v, c_v, xn_s, acc_s, mux_s, ctx_s, q_s, k_s, v_s,
            w_b, wo_v, wr_ref, wg_v, wu_v, wd_v,
            xsem, csem, wsem, osem_w, fsem, osem,
            *, S, M, C, D, NP, FF):
    ALL = slice(None)
    xn_p, c_p = _Packed(xn_s), _Packed(c_v)
    scale = (D ** -0.5) * math.log2(math.e)

    def xcopy(b):
        rows = pl.ds(pl.multiple_of(b * XB, XB), XB)
        return pltpu.make_async_copy(x_hbm.at[0, rows, :], io_v.at[rows, :], xsem.at[b])

    def ccopy(b):
        rows = pl.ds(pl.multiple_of(b * (XB // 2), XB // 2), XB // 2)
        return pltpu.make_async_copy(c_hbm.bitcast(U32).at[0, rows, :], c_v.at[rows, :], csem.at[b])

    KR, VR, QR = slice(0, C), slice(C, 2 * C), slice(2 * C, 2 * C + M)

    def wstart(jj, sl):
        for src, rows in ((wk_hbm, KR), (wv_hbm, VR), (wq_hbm, QR)):
            pltpu.make_async_copy(src.bitcast(U32).at[:, jj, :], w_b.at[sl, rows, :], wsem.at[sl]).start()

    def wwait(sl):
        pltpu.make_async_copy(w_b.at[sl], w_b.at[sl], wsem.at[sl]).wait()

    def wocopy(t):
        heads = pl.ds(0, 2) if t == 0 else pl.ds(2, 2 * NP - 2)
        return pltpu.make_async_copy(wo_hbm.bitcast(U32).at[heads], wo_v.at[heads], osem_w.at[t])

    def fcopy(t):
        if t == 0:
            return pltpu.make_async_copy(wg_hbm, wg_v, fsem.at[0])
        if t == 1:
            return pltpu.make_async_copy(wu_hbm, wu_v, fsem.at[1])
        if t == 2:
            return pltpu.make_async_copy(wd_hbm, wd_v.at[:, 0:M], fsem.at[2])
        return pltpu.make_async_copy(wr_hbm, wr_ref, fsem.at[3])

    def ocopy(g):
        rows = pl.ds(g * OB, OB)
        return pltpu.make_async_copy(io_v.at[rows, :], out_hbm.at[0, rows, :], osem.at[g])

    def project(dst, lhs, w32, rows, mult=None):
        y = jnp.dot(lhs, _unpack_pair(w32), preferred_element_type=F32)
        if mult is not None:
            y = y * mult
        _Packed(dst.at[0])[rows, ALL] = y[:, :D]
        _Packed(dst.at[1])[rows, ALL] = y[:, D:]

    NXB = S // XB
    wstart(0, 0)
    for b in range(NXB):
        ccopy(b).start()
        xcopy(b).start()
    wocopy(0).start()
    fcopy(3).start()
    wstart(1, 1)
    wwait(0)

    def first(b, carry):
        ccopy(b).wait()
        xcopy(b).wait()
        rows = pl.ds(pl.multiple_of(b * XB, XB), XB)
        xf = io_v[rows, :].astype(F32)
        mu = jnp.mean(xf, axis=1, keepdims=True)
        xc = xf - mu
        var = jnp.mean(xc * xc, axis=1, keepdims=True)
        xn = (xc * lax.rsqrt(var + 1e-5)).astype(BF16)
        prow = (b, XB)
        xn_p[prow, ALL] = xn
        acc_s[rows, :] = xc
        mux_s[rows, :] = jnp.broadcast_to(mu, (XB, 128))
        c = c_p[prow, ALL]
        project(k_s, c, w_b[0, KR, :], prow)
        project(v_s, c, w_b[0, VR, :], prow)
        project(q_s, xn, w_b[0, QR, :], prow, scale)
        return carry
    lax.fori_loop(0, S // XB, first, 0)
    wstart(2, 0)
    wocopy(1).start()
    for t in range(3):
        fcopy(t).start()
    wocopy(0).wait()

    def step(j, carry):
        slot = j & 1

        @pl.when(j == 1)
        def _():
            wocopy(1).wait()

        wwait(1 - slot)

        @pl.when(jnp.logical_and(j >= 1, j + 2 < NP))
        def _():
            wstart(j + 2, slot)

        wo = pltpu.bitcast(wo_v[pl.ds(2 * j, 2)].reshape(D, M), BF16)

        def oproj(ii, pair_ctx):
            acc_s[ii * TQ:(ii + 1) * TQ, :] += jnp.dot(pair_ctx(ii), wo, preferred_element_type=F32)

        def rows_of(code):
            return slice((code // 10) * TQ, (code % 10 + 1) * TQ)

        _attn_pair(q_s, k_s, v_s, ORDER_MAIN, {
            'O': oproj,
            'K': lambda code, _: project(k_s, c_p[rows_of(code), ALL], w_b[1 - slot, KR, :], rows_of(code)),
            'V': lambda code, _: project(v_s, c_p[rows_of(code), ALL], w_b[1 - slot, VR, :], rows_of(code)),
            'Q': lambda code, _: project(q_s, xn_p[rows_of(code), ALL], w_b[1 - slot, QR, :], rows_of(code), scale),
        })
        return carry
    lax.fori_loop(0, NP - 1, step, 0)

    for t in range(4):
        fcopy(t).wait()
    eps = jnp.asarray(1e-5, BF16).astype(F32)

    def last_head(h, carry):
        sc = {}
        for tok in ORDER_LAST.split():
            i = int(tok[1])
            if tok[0] == 'S':
                sc[i] = _qk(_Packed(q_s.at[h]), _Packed(k_s.at[h]), i)
            else:
                _Packed(ctx_s.at[h])[slice(i * TQ, (i + 1) * TQ), ALL] = _pv(
                    _softmax(sc.pop(i), i), _Packed(v_s.at[h]), i)
        return carry
    lax.fori_loop(0, 2, last_head, 0)

    CW = M // NCH
    RW = M // RG
    wr16 = [jnp.broadcast_to(wr_ref[t * RW:(t + 1) * RW].astype(F32).reshape(1, RW), (16, RW)).astype(BF16)
            for t in range(RG)]

    def oproj_part(r0, t):
        rows = slice(r0, r0 + EB)
        cols = slice(t * CW, (t + 1) * CW)
        return (acc_s[rows, cols]
                + jnp.dot(_Packed(ctx_s.at[0])[rows, ALL], pltpu.bitcast(wo_v[2 * NP - 2, :, cols], BF16),
                           preferred_element_type=F32)
                + jnp.dot(_Packed(ctx_s.at[1])[rows, ALL], pltpu.bitcast(wo_v[2 * NP - 1, :, cols], BF16),
                           preferred_element_type=F32))

    def ln2(r0, a):
        rows = slice(r0, r0 + EB)
        acc_s[rows, :] = a
        s1 = jnp.mean(a, axis=1, keepdims=True)
        var = jnp.maximum(jnp.mean(a * a, axis=1, keepdims=True) - s1 * s1, 0.0)
        ve = _rb(_rb(var) + eps)
        den = _rb(ve * lax.rsqrt(ve))
        inv = _recip(den)
        inv = inv * (2.0 - den * inv)
        mux = mux_s[rows, :]
        c1 = (_rb(mux + s1) - mux) * inv
        c2 = mux - c1
        a = acc_s[rows, :]
        t = a * inv
        xn_p[rows, ALL] = t - jnp.concatenate([c1] * (M // 128), axis=1)
        io_v[rows, :] = ((a + t) + jnp.concatenate([c2] * (M // 128), axis=1)).astype(BF16)

    def router_part(r0, t):
        cols = slice(t * RW, (t + 1) * RW)
        return lax.dot_general(wr16[t], xn_p[slice(r0, r0 + EB), cols], NT, preferred_element_type=F32)

    neb = S // EB
    rparts = []
    for k in range(neb + RLAG):
        hp, rp = [], None
        for t in range(NCH):
            if k < neb:
                hp.append(oproj_part(k * EB, t))
            if k >= RLAG and t < RG:
                part = router_part((k - RLAG) * EB, t)[0:8, :]
                rp = part if rp is None else rp + part
        if k > 0 and k <= neb and (k * EB) % OB == 0:
            ocopy(k * EB // OB - 1).start()
        if k < neb:
            ln2(k * EB, jnp.concatenate(hp, axis=1))
        if k >= RLAG:
            rparts.append(rp)
    rrow = _rb(jnp.concatenate(rparts, axis=1))

    I32 = jnp.int32
    b16 = lax.shift_right_logical(pltpu.bitcast(rrow, I32), 16)
    rank = jnp.where(b16 >= 0x8000, 0x10000 - b16, 0x8000 + b16)
    lane = lax.broadcasted_iota(I32, rrow.shape, 1)
    key = pltpu.bitcast(rank * S + (S - 1 - lane) + 0x20000000, F32)
    k1 = jnp.max(key, axis=1, keepdims=True)
    k2 = jnp.max(jnp.where(key == k1, 0.0, key), axis=1, keepdims=True)
    i1 = (S - 1) - (pltpu.bitcast(k1, I32)[0, 0] & (S - 1))
    i2 = (S - 1) - (pltpu.bitcast(k2, I32)[0, 0] & (S - 1))
    m1 = jnp.max(jnp.where(key == k1, rrow, -jnp.inf), axis=1, keepdims=True)[0:1, :]
    m2 = jnp.max(jnp.where(key == k2, rrow, -jnp.inf), axis=1, keepdims=True)[0:1, :]
    q1 = jnp.clip(i1 >> 4, 0, S // 16 - 1)
    q2 = jnp.clip(i2 >> 4, 0, S // 16 - 1)
    g1 = pl.multiple_of(q1 * 16, 16)
    g2 = pl.multiple_of(q2 * 16, 16)

    rid = lax.broadcasted_iota(jnp.int32, (16, M), 0)

    def pick(q, i):
        blk = pltpu.bitcast(xn_s[pl.ds(pl.multiple_of(q * 8, 8), 8), :], BF16).astype(F32)
        return jnp.sum(jnp.where(rid == i - q * 16, blk, 0.0), axis=0, keepdims=True)

    xs = jnp.where(rid == 0, pick(q1, i1), pick(q2, i2))
    xsb = xs.astype(BF16)
    ocopy(0).wait()
    nch = FF // FC
    acts, y = [], None
    for t in range(nch + 1):
        if t < nch:
            cols = slice(t * FC, (t + 1) * FC)
            a = _rb(jnp.dot(xsb, wg_v[:, cols], preferred_element_type=F32))
            u = _rb(jnp.dot(xsb, wu_v[:, cols], preferred_element_type=F32))
            g = _rb(a * _rb(jax.nn.sigmoid(a)))
            acts.append((g * u).astype(BF16))
        if t > 0:
            yt = jnp.dot(acts[t - 1], wd_v[(t - 1) * FC:t * FC, 0:M], preferred_element_type=F32)
            y = yt if y is None else y + yt
    rsel = jnp.where(rid == 0, m1, m2)
    y = _rb(_rb(y) * _rb(jax.nn.sigmoid(rsel)))
    upd = _rb(xs + y)

    for k, gg in enumerate((g1, g2)):
        rows = pl.ds(gg, 16)
        hb = _rb(acc_s[rows, :] + jnp.concatenate([mux_s[rows, :]] * (M // 128), axis=1))
        val = jnp.where(rid == i1 - gg, hb + upd[0:1, :],
                        jnp.where(rid == i2 - gg, hb + upd[1:2, :], io_v[rows, :].astype(F32)))
        pt_v[k] = val.astype(BF16)

    def pcopy(g, k):
        return pltpu.make_async_copy(pt_v.at[k], out_hbm.at[0, pl.ds(g, 16), :], osem.at[k])

    for b in range(1, S // OB):
        ocopy(b).wait()
    pcopy(g1, 0).start()

    @pl.when(g2 != g1)
    def _():
        pcopy(g2, 1).start()
        pcopy(g2, 1).wait()
    pcopy(g1, 0).wait()


def _compiler_params():
    vmem = 110 * 1024 * 1024
    try:
        return pltpu.CompilerParams(vmem_limit_bytes=vmem, disable_bounds_checks=True,
                                    disable_semaphore_checks=True)
    except TypeError:
        return pltpu.CompilerParams(vmem_limit_bytes=vmem, disable_bounds_checks=True)


@jax.jit
def pallas_sequential_preLN__compressed_kv_cla__moe_arch_mod__prompt_kernel(
    A_x: jax.Array,
    A_c_kv: jax.Array,
    A_w_q: jax.Array,
    A_w_uk: jax.Array,
    A_w_uv: jax.Array,
    A_w_o: jax.Array,
    B_x: jax.Array,
    B_w_r: jax.Array,
    B_w_gate: jax.Array,
    B_w_up: jax.Array,
    B_w_down: jax.Array,
):
    _, S, M = A_x.shape
    C = A_c_kv.shape[2]
    H, D = A_w_q.shape[1], A_w_q.shape[2]
    FF = B_w_gate.shape[1]
    NP = H // 2
    any_spec = pl.BlockSpec(memory_space=pl.ANY)
    return pl.pallas_call(
        functools.partial(_kernel, S=S, M=M, C=C, D=D, NP=NP, FF=FF),
        in_specs=[
            any_spec, any_spec, any_spec, any_spec, any_spec, any_spec,
            any_spec, any_spec, any_spec, any_spec,
        ],
        out_specs=any_spec,
        out_shape=jax.ShapeDtypeStruct((1, S, M), BF16),
        scratch_shapes=[
            pltpu.VMEM((S, M), BF16),
            pltpu.VMEM((2, 16, M), BF16),
            pltpu.VMEM((S // 2, C), U32),
            pltpu.VMEM((S // 2, M), U32),
            pltpu.VMEM((S, M), F32),
            pltpu.VMEM((S, 128), F32),
            pltpu.VMEM((2, S // 2, D), U32),
            pltpu.VMEM((2, S // 2, D), U32),
            pltpu.VMEM((2, S // 2, D), U32),
            pltpu.VMEM((2, S // 2, D), U32),
            pltpu.VMEM((2, 2 * C + M, D), U32),
            pltpu.VMEM((H, D // 2, M), U32),
            pltpu.VMEM((M,), BF16),
            pltpu.VMEM((M, FF), BF16),
            pltpu.VMEM((M, FF), BF16),
            pltpu.VMEM((FF, M + 128), BF16),
            pltpu.SemaphoreType.DMA((S // XB,)),
            pltpu.SemaphoreType.DMA((S // XB,)),
            pltpu.SemaphoreType.DMA((2,)),
            pltpu.SemaphoreType.DMA((2,)),
            pltpu.SemaphoreType.DMA((4,)),
            pltpu.SemaphoreType.DMA((S // OB,)),
        ],
        compiler_params=_compiler_params(),
    )(A_x, A_c_kv, A_w_q, A_w_uk, A_w_uv, A_w_o, B_w_r, B_w_gate, B_w_up, B_w_down)
```

```python
import functools
import math

import jax
import jax.numpy as jnp
from jax import lax
import jax.experimental.pallas as pl
import jax.experimental.pallas.tpu as pltpu

F32 = jnp.float32
BF16 = jnp.bfloat16
U32 = jnp.uint32
NEG = -1e30
NT = (((1,), (1,)), ((), ()))
TQ = 512
SUB = 128
GRP = 4
XB = 256
EB = 128
OB = 512
NCH = 4
RG = 2
RLAG = 2
FC = 512

ORDER_MAIN = ("S03 S13 K33 P03 S02 P13 S12 P02 S01 Q23 S11 S00 P12 P01 P11 S10 K02 P00 P10 "
              "O3 O2 Q01 O1 V03 O0")
ORDER_LAST = "S2 S3 P2 S1 P3 S0 P1 P0"
QKORD, QKORD1, QKORDL, QKORDL1 = "01s2CcS3m", "01cCm2sS3", "m0123cCSs", "m012sScC3"


def _rb(v):
    return v.astype(BF16).astype(F32)


def _recip(l):
    return pl.reciprocal(l, approx=True)


def _unpack_pair(w32):
    lo = pltpu.bitcast(w32 << 16, F32)
    hi = pltpu.bitcast(w32 & jnp.uint32(0xFFFF0000), F32)
    return jnp.concatenate([lo, hi], axis=1).astype(BF16)


class _Packed:
    def __init__(self, ref):
        self.ref = ref

    @staticmethod
    def half(rows):
        if isinstance(rows, slice):
            return slice(rows.start // 2, rows.stop // 2)
        blk, size = rows
        return pl.ds(pl.multiple_of(blk * (size // 2), size // 2), size // 2)

    def __getitem__(self, idx):
        rows, cols = idx
        return pltpu.bitcast(self.ref[self.half(rows), cols], BF16)

    def __setitem__(self, idx, val):
        rows, cols = idx
        self.ref[self.half(rows), cols] = pltpu.bitcast(val.astype(BF16), U32)


def _nt(a, b):
    return lax.dot_general(a, b, NT, preferred_element_type=F32)


def _rows(*parts):
    return jnp.concatenate(parts, axis=0)


def _qk(q, k, i, qkord):
    r0 = i * TQ
    HB = SUB // 2

    def qr(a, b):
        return q[r0 + a * HB:r0 + b * HB, :]

    def kr(a, b):
        return k[r0 + a * HB:r0 + b * HB, :]

    jobs = {
        'c': lambda: _nt(kr(0, 1), _rows(qr(0, 1), qr(2, 3))),
        'C': lambda: _nt(kr(4, 5), _rows(qr(4, 5), qr(6, 7))),
        's': lambda: _nt(qr(2, 3), _rows(kr(2, 3), kr(1, 2))),
        'S': lambda: _nt(qr(6, 7), _rows(kr(6, 7), kr(5, 6))),
        '0': lambda: _nt(_rows(qr(1, 2), qr(3, 8)), kr(0, 2)),
        '1': lambda: _nt(qr(3, 8), kr(2, 4)),
        '2': lambda: _nt(_rows(qr(5, 6), qr(7, 8)), kr(4, 6)),
        '3': lambda: _nt(qr(7, 8), kr(6, 8)),
        'm': lambda: _nt(qr(0, 8), k[0:r0, :]) if r0 > 0 else None,
    }
    res = {ch: jobs[ch]() for ch in qkord}
    co, sh, al = [res['c'], res['C']], [res['s'], res['S']], [res[t] for t in '0123']
    cot = [_rows(co[0], co[1]).T, _rows(co[1], co[0]).T]
    row = lax.broadcasted_iota(jnp.int32, (SUB, SUB), 0)
    col = lax.broadcasted_iota(jnp.int32, (SUB, SUB), 1)
    tri = col <= row
    low = lax.broadcasted_iota(jnp.int32, (HB, SUB), 1) < HB
    tiles = [[None] * (b + 1) for b in range(4)]
    for u in range(2):
        a_lo, a_hi = al[2 * u], al[2 * u + 1]
        tiles[2 * u][2 * u] = jnp.where(tri, _rows(cot[u][0:HB], a_lo[0:HB]), NEG)
        tiles[2 * u + 1][2 * u] = _rows(jnp.where(low, cot[u][HB:SUB], sh[u]), a_lo[HB:SUB])
        tiles[2 * u + 1][2 * u + 1] = jnp.where(tri, _rows(sh[u], a_hi[0:HB]), NEG)
    for b in (2, 3):
        tiles[b][0] = al[0][(b - 1) * SUB:b * SUB]
        tiles[b][1] = al[1][(b - 2) * SUB + HB:(b - 1) * SUB + HB]
    return res['m'], tiles


def _softmax(s, i):
    s_main, s_tiles = s
    r0 = i * TQ
    nb = TQ // SUB
    p_main, p_ext, ls = [], [[] for _ in range(1, nb)], []
    for b in range(nb):
        parts = ([s_main[b * SUB:(b + 1) * SUB, :]] if r0 > 0 else []) + s_tiles[b]
        sb = jnp.concatenate(parts, axis=1) if len(parts) > 1 else parts[0]
        m = jnp.max(sb, axis=1, keepdims=True)
        p = jnp.exp2(sb - m)
        nt = p.shape[1] // SUB
        tiles = [p[:, t * SUB:(t + 1) * SUB] for t in range(nt)]
        acc = None
        for t0 in range(0, nt, GRP):
            grp = tiles[t0:t0 + GRP]
            tot = grp[0]
            for g in grp[1:]:
                tot = tot + g
            acc = tot if acc is None else acc + tot
            last = t0 + len(grp) - 1
            if acc is not tiles[last]:
                tiles[last] = jnp.minimum(tiles[last], acc)
        p = jnp.concatenate(tiles, axis=1) if nt > 1 else tiles[0]
        ls.append(jnp.sum(acc, axis=1, keepdims=True))
        p_main.append(p[:, :r0 + SUB])
        for c in range(1, b + 1):
            p_ext[c - 1].append(p[:, r0 + c * SUB:r0 + (c + 1) * SUB])
    pm = jnp.concatenate(p_main, axis=0).astype(BF16)
    pe = [(jnp.concatenate(e, axis=0) if len(e) > 1 else e[0]).astype(BF16) for e in p_ext]
    return pm, pe, ls


def _pv(p, v, i):
    pm, pe, ls = p
    r0 = i * TQ
    nb = TQ // SUB
    o = jnp.dot(pm, v[0:r0 + SUB, :], preferred_element_type=F32)
    os_ = [o[b * SUB:(b + 1) * SUB] for b in range(nb)]
    for c in range(1, nb):
        oe = jnp.dot(pe[c - 1], v[r0 + c * SUB:r0 + (c + 1) * SUB, :], preferred_element_type=F32)
        for b in range(c, nb):
            os_[b] = os_[b] + oe[(b - c) * SUB:(b - c + 1) * SUB]
    return jnp.concatenate([os_[b] * _recip(ls[b]) for b in range(nb)], axis=0)


def _attn_pair(q_s, k_s, v_s, order, actions):
    sc, ctx = {}, {}

    def pair_ctx(i):
        return jnp.concatenate([ctx[(0, i)], ctx[(1, i)]], axis=1).astype(BF16)

    for tok in order.split():
        if tok[0] == 'S':
            h, i = int(tok[1]), int(tok[2])
            sc[(h, i)] = _qk(_Packed(q_s.at[h]), _Packed(k_s.at[h]), i, QKORD if (sc or ctx) else QKORD1)
        elif tok[0] == 'P':
            h, i = int(tok[1]), int(tok[2])
            ctx[(h, i)] = _pv(_softmax(sc.pop((h, i)), i), _Packed(v_s.at[h]), i)
        else:
            actions[tok[0]](int(tok[1:]), pair_ctx)


def _kernel(x_hbm, c_hbm, wq_hbm, wk_hbm, wv_hbm, wo_hbm, wr_hbm, wg_hbm, wu_hbm, wd_hbm,
            out_hbm,
            io_v, pt_v, c_v, xn_s, acc_s, mux_s, ctx_s, q_s, k_s, v_s,
            w_b, wo_v, wr_ref, wg_v, wu_v, wd_v,
            xsem, csem, wsem, osem_w, fsem, osem,
            *, S, M, C, D, NP, FF):
    ALL = slice(None)
    xn_p, c_p = _Packed(xn_s), _Packed(c_v)
    scale = (D ** -0.5) * math.log2(math.e)

    def xcopy(b):
        rows = pl.ds(pl.multiple_of(b * XB, XB), XB)
        return pltpu.make_async_copy(x_hbm.at[0, rows, :], io_v.at[rows, :], xsem.at[b])

    def ccopy(b):
        rows = pl.ds(pl.multiple_of(b * (XB // 2), XB // 2), XB // 2)
        return pltpu.make_async_copy(c_hbm.bitcast(U32).at[0, rows, :], c_v.at[rows, :], csem.at[b])

    KR, VR, QR = slice(0, C), slice(C, 2 * C), slice(2 * C, 2 * C + M)

    def wstart(jj, sl):
        for src, rows in ((wk_hbm, KR), (wv_hbm, VR), (wq_hbm, QR)):
            pltpu.make_async_copy(src.bitcast(U32).at[:, jj, :], w_b.at[sl, rows, :], wsem.at[sl]).start()

    def wwait(sl):
        pltpu.make_async_copy(w_b.at[sl], w_b.at[sl], wsem.at[sl]).wait()

    def wocopy(t):
        heads = pl.ds(0, 2) if t == 0 else pl.ds(2, 2 * NP - 2)
        return pltpu.make_async_copy(wo_hbm.bitcast(U32).at[heads], wo_v.at[heads], osem_w.at[t])

    def fcopy(t):
        if t == 0:
            return pltpu.make_async_copy(wg_hbm, wg_v, fsem.at[0])
        if t == 1:
            return pltpu.make_async_copy(wu_hbm, wu_v, fsem.at[1])
        if t == 2:
            return pltpu.make_async_copy(wd_hbm, wd_v.at[:, 0:M], fsem.at[2])
        return pltpu.make_async_copy(wr_hbm, wr_ref, fsem.at[3])

    def ocopy(g):
        rows = pl.ds(g * OB, OB)
        return pltpu.make_async_copy(io_v.at[rows, :], out_hbm.at[0, rows, :], osem.at[g])

    def project(dst, lhs, w32, rows, mult=None):
        y = jnp.dot(lhs, _unpack_pair(w32), preferred_element_type=F32)
        if mult is not None:
            y = y * mult
        _Packed(dst.at[0])[rows, ALL] = y[:, :D]
        _Packed(dst.at[1])[rows, ALL] = y[:, D:]

    NXB = S // XB
    wstart(0, 0)
    for b in range(NXB):
        ccopy(b).start()
        xcopy(b).start()
    wocopy(0).start()
    fcopy(3).start()
    wstart(1, 1)
    wwait(0)

    def first(b, carry):
        ccopy(b).wait()
        xcopy(b).wait()
        rows = pl.ds(pl.multiple_of(b * XB, XB), XB)
        xf = io_v[rows, :].astype(F32)
        mu = jnp.mean(xf, axis=1, keepdims=True)
        xc = xf - mu
        var = jnp.mean(xc * xc, axis=1, keepdims=True)
        xn = (xc * lax.rsqrt(var + 1e-5)).astype(BF16)
        prow = (b, XB)
        xn_p[prow, ALL] = xn
        acc_s[rows, :] = xc
        mux_s[rows, :] = jnp.broadcast_to(mu, (XB, 128))
        c = c_p[prow, ALL]
        project(k_s, c, w_b[0, KR, :], prow)
        project(v_s, c, w_b[0, VR, :], prow)
        project(q_s, xn, w_b[0, QR, :], prow, scale)
        return carry
    lax.fori_loop(0, S // XB, first, 0)
    wstart(2, 0)
    wocopy(1).start()
    for t in range(3):
        fcopy(t).start()
    wocopy(0).wait()

    def step(j, carry):
        slot = j & 1

        @pl.when(j == 1)
        def _():
            wocopy(1).wait()

        wwait(1 - slot)

        @pl.when(jnp.logical_and(j >= 1, j + 2 < NP))
        def _():
            wstart(j + 2, slot)

        wo = pltpu.bitcast(wo_v[pl.ds(2 * j, 2)].reshape(D, M), BF16)

        def oproj(ii, pair_ctx):
            acc_s[ii * TQ:(ii + 1) * TQ, :] += jnp.dot(pair_ctx(ii), wo, preferred_element_type=F32)

        def rows_of(code):
            return slice((code // 10) * TQ, (code % 10 + 1) * TQ)

        _attn_pair(q_s, k_s, v_s, ORDER_MAIN, {
            'O': oproj,
            'K': lambda code, _: project(k_s, c_p[rows_of(code), ALL], w_b[1 - slot, KR, :], rows_of(code)),
            'V': lambda code, _: project(v_s, c_p[rows_of(code), ALL], w_b[1 - slot, VR, :], rows_of(code)),
            'Q': lambda code, _: project(q_s, xn_p[rows_of(code), ALL], w_b[1 - slot, QR, :], rows_of(code), scale),
        })
        return carry
    lax.fori_loop(0, NP - 1, step, 0)

    for t in range(4):
        fcopy(t).wait()
    eps = jnp.asarray(1e-5, BF16).astype(F32)

    def last_head(h, carry):
        sc = {}
        for tok in ORDER_LAST.split():
            i = int(tok[1])
            if tok[0] == 'S':
                sc[i] = _qk(_Packed(q_s.at[h]), _Packed(k_s.at[h]), i, QKORDL1 if tok == ORDER_LAST.split()[0] else QKORDL)
            else:
                _Packed(ctx_s.at[h])[slice(i * TQ, (i + 1) * TQ), ALL] = _pv(
                    _softmax(sc.pop(i), i), _Packed(v_s.at[h]), i)
        return carry
    lax.fori_loop(0, 2, last_head, 0)

    CW = M // NCH
    RW = M // RG
    wr16 = [jnp.broadcast_to(wr_ref[t * RW:(t + 1) * RW].astype(F32).reshape(1, RW), (16, RW)).astype(BF16)
            for t in range(RG)]

    def oproj_part(r0, t):
        rows = slice(r0, r0 + EB)
        cols = slice(t * CW, (t + 1) * CW)
        return (acc_s[rows, cols]
                + jnp.dot(_Packed(ctx_s.at[0])[rows, ALL], pltpu.bitcast(wo_v[2 * NP - 2, :, cols], BF16),
                           preferred_element_type=F32)
                + jnp.dot(_Packed(ctx_s.at[1])[rows, ALL], pltpu.bitcast(wo_v[2 * NP - 1, :, cols], BF16),
                           preferred_element_type=F32))

    def ln2(r0, a):
        rows = slice(r0, r0 + EB)
        acc_s[rows, :] = a
        s1 = jnp.mean(a, axis=1, keepdims=True)
        var = jnp.maximum(jnp.mean(a * a, axis=1, keepdims=True) - s1 * s1, 0.0)
        ve = _rb(_rb(var) + eps)
        den = _rb(ve * lax.rsqrt(ve))
        inv = _recip(den)
        inv = inv * (2.0 - den * inv)
        mux = mux_s[rows, :]
        c1 = (_rb(mux + s1) - mux) * inv
        c2 = mux - c1
        a = acc_s[rows, :]
        t = a * inv
        xn_p[rows, ALL] = t - jnp.concatenate([c1] * (M // 128), axis=1)
        io_v[rows, :] = ((a + t) + jnp.concatenate([c2] * (M // 128), axis=1)).astype(BF16)

    def router_part(r0, t):
        cols = slice(t * RW, (t + 1) * RW)
        return lax.dot_general(wr16[t], xn_p[slice(r0, r0 + EB), cols], NT, preferred_element_type=F32)

    neb = S // EB
    rparts = []
    for k in range(neb + RLAG):
        hp, rp = [], None
        for t in range(NCH):
            if k < neb:
                hp.append(oproj_part(k * EB, t))
            if k >= RLAG and t < RG:
                part = router_part((k - RLAG) * EB, t)[0:8, :]
                rp = part if rp is None else rp + part
        if k > 0 and k <= neb and (k * EB) % OB == 0:
            ocopy(k * EB // OB - 1).start()
        if k < neb:
            ln2(k * EB, jnp.concatenate(hp, axis=1))
        if k >= RLAG:
            rparts.append(rp)
    rrow = _rb(jnp.concatenate(rparts, axis=1))

    I32 = jnp.int32
    b16 = lax.shift_right_logical(pltpu.bitcast(rrow, I32), 16)
    rank = jnp.where(b16 >= 0x8000, 0x10000 - b16, 0x8000 + b16)
    lane = lax.broadcasted_iota(I32, rrow.shape, 1)
    key = pltpu.bitcast(rank * S + (S - 1 - lane) + 0x20000000, F32)
    k1 = jnp.max(key, axis=1, keepdims=True)
    k2 = jnp.max(jnp.where(key == k1, 0.0, key), axis=1, keepdims=True)
    i1 = (S - 1) - (pltpu.bitcast(k1, I32)[0, 0] & (S - 1))
    i2 = (S - 1) - (pltpu.bitcast(k2, I32)[0, 0] & (S - 1))
    m1 = jnp.max(jnp.where(key == k1, rrow, -jnp.inf), axis=1, keepdims=True)[0:1, :]
    m2 = jnp.max(jnp.where(key == k2, rrow, -jnp.inf), axis=1, keepdims=True)[0:1, :]
    q1 = jnp.clip(i1 >> 4, 0, S // 16 - 1)
    q2 = jnp.clip(i2 >> 4, 0, S // 16 - 1)
    g1 = pl.multiple_of(q1 * 16, 16)
    g2 = pl.multiple_of(q2 * 16, 16)

    rid = lax.broadcasted_iota(jnp.int32, (16, M), 0)

    def pick(q, i):
        blk = pltpu.bitcast(xn_s[pl.ds(pl.multiple_of(q * 8, 8), 8), :], BF16).astype(F32)
        return jnp.sum(jnp.where(rid == i - q * 16, blk, 0.0), axis=0, keepdims=True)

    xs = jnp.where(rid == 0, pick(q1, i1), pick(q2, i2))
    xsb = xs.astype(BF16)
    ocopy(0).wait()
    nch = FF // FC
    acts, y = [], None
    for t in range(nch + 1):
        if t < nch:
            cols = slice(t * FC, (t + 1) * FC)
            a = _rb(jnp.dot(xsb, wg_v[:, cols], preferred_element_type=F32))
            u = _rb(jnp.dot(xsb, wu_v[:, cols], preferred_element_type=F32))
            g = _rb(a * _rb(jax.nn.sigmoid(a)))
            acts.append((g * u).astype(BF16))
        if t > 0:
            yt = jnp.dot(acts[t - 1], wd_v[(t - 1) * FC:t * FC, 0:M], preferred_element_type=F32)
            y = yt if y is None else y + yt
    rsel = jnp.where(rid == 0, m1, m2)
    y = _rb(_rb(y) * _rb(jax.nn.sigmoid(rsel)))
    upd = _rb(xs + y)

    for k, gg in enumerate((g1, g2)):
        rows = pl.ds(gg, 16)
        hb = _rb(acc_s[rows, :] + jnp.concatenate([mux_s[rows, :]] * (M // 128), axis=1))
        val = jnp.where(rid == i1 - gg, hb + upd[0:1, :],
                        jnp.where(rid == i2 - gg, hb + upd[1:2, :], io_v[rows, :].astype(F32)))
        pt_v[k] = val.astype(BF16)

    def pcopy(g, k):
        return pltpu.make_async_copy(pt_v.at[k], out_hbm.at[0, pl.ds(g, 16), :], osem.at[k])

    for b in range(1, S // OB):
        ocopy(b).wait()
    pcopy(g1, 0).start()

    @pl.when(g2 != g1)
    def _():
        pcopy(g2, 1).start()
        pcopy(g2, 1).wait()
    pcopy(g1, 0).wait()


def _compiler_params():
    vmem = 110 * 1024 * 1024
    try:
        return pltpu.CompilerParams(vmem_limit_bytes=vmem, disable_bounds_checks=True,
                                    disable_semaphore_checks=True)
    except TypeError:
        return pltpu.CompilerParams(vmem_limit_bytes=vmem, disable_bounds_checks=True)


@jax.jit
def pallas_sequential_preLN__compressed_kv_cla__moe_arch_mod__prompt_kernel(
    A_x: jax.Array,
    A_c_kv: jax.Array,
    A_w_q: jax.Array,
    A_w_uk: jax.Array,
    A_w_uv: jax.Array,
    A_w_o: jax.Array,
    B_x: jax.Array,
    B_w_r: jax.Array,
    B_w_gate: jax.Array,
    B_w_up: jax.Array,
    B_w_down: jax.Array,
):
    _, S, M = A_x.shape
    C = A_c_kv.shape[2]
    H, D = A_w_q.shape[1], A_w_q.shape[2]
    FF = B_w_gate.shape[1]
    NP = H // 2
    any_spec = pl.BlockSpec(memory_space=pl.ANY)
    return pl.pallas_call(
        functools.partial(_kernel, S=S, M=M, C=C, D=D, NP=NP, FF=FF),
        in_specs=[
            any_spec, any_spec, any_spec, any_spec, any_spec, any_spec,
            any_spec, any_spec, any_spec, any_spec,
        ],
        out_specs=any_spec,
        out_shape=jax.ShapeDtypeStruct((1, S, M), BF16),
        scratch_shapes=[
            pltpu.VMEM((S, M), BF16),
            pltpu.VMEM((2, 16, M), BF16),
            pltpu.VMEM((S // 2, C), U32),
            pltpu.VMEM((S // 2, M), U32),
            pltpu.VMEM((S, M), F32),
            pltpu.VMEM((S, 128), F32),
            pltpu.VMEM((2, S // 2, D), U32),
            pltpu.VMEM((2, S // 2, D), U32),
            pltpu.VMEM((2, S // 2, D), U32),
            pltpu.VMEM((2, S // 2, D), U32),
            pltpu.VMEM((2, 2 * C + M, D), U32),
            pltpu.VMEM((H, D // 2, M), U32),
            pltpu.VMEM((M,), BF16),
            pltpu.VMEM((M, FF), BF16),
            pltpu.VMEM((M, FF), BF16),
            pltpu.VMEM((FF, M + 128), BF16),
            pltpu.SemaphoreType.DMA((S // XB,)),
            pltpu.SemaphoreType.DMA((S // XB,)),
            pltpu.SemaphoreType.DMA((2,)),
            pltpu.SemaphoreType.DMA((2,)),
            pltpu.SemaphoreType.DMA((4,)),
            pltpu.SemaphoreType.DMA((S // OB,)),
        ],
        compiler_params=_compiler_params(),
    )(A_x, A_c_kv, A_w_q, A_w_uk, A_w_uv, A_w_o, B_w_r, B_w_gate, B_w_up, B_w_down)
```

```python
import functools
import math

import jax
import jax.numpy as jnp
from jax import lax
import jax.experimental.pallas as pl
import jax.experimental.pallas.tpu as pltpu

F32 = jnp.float32
BF16 = jnp.bfloat16
U32 = jnp.uint32
NEG = -1e30
NT = (((1,), (1,)), ((), ()))
TQ = 512
SUB = 128
GRP = 4
XB = 256
EB = 128
OB = 512
NCH = 4
RG = 2
RLAG = 2
FC = 512

ORDER_MAIN = ("S03 S13 K33 P03 S02 P13 S12 P02 S01 Q23 S11 S00 P12 P01 P11 S10 K02 P00 P10 "
              "O3 O2 Q01 O1 V03 O0")
ORDER_LAST = "S3 S2 P3 S1 P2 S0 P1 P0"
QKORD, QKORD1, QKORDL, QKORDL1 = "01s2CcS3m", "01cCm2sS3", "01mS2cCs3", "Ccm2s10S3"


def _rb(v):
    return v.astype(BF16).astype(F32)


def _recip(l):
    return pl.reciprocal(l, approx=True)


def _unpack_pair(w32):
    lo = pltpu.bitcast(w32 << 16, F32)
    hi = pltpu.bitcast(w32 & jnp.uint32(0xFFFF0000), F32)
    return jnp.concatenate([lo, hi], axis=1).astype(BF16)


class _Packed:
    def __init__(self, ref):
        self.ref = ref

    @staticmethod
    def half(rows):
        if isinstance(rows, slice):
            return slice(rows.start // 2, rows.stop // 2)
        blk, size = rows
        return pl.ds(pl.multiple_of(blk * (size // 2), size // 2), size // 2)

    def __getitem__(self, idx):
        rows, cols = idx
        return pltpu.bitcast(self.ref[self.half(rows), cols], BF16)

    def __setitem__(self, idx, val):
        rows, cols = idx
        self.ref[self.half(rows), cols] = pltpu.bitcast(val.astype(BF16), U32)


def _nt(a, b):
    return lax.dot_general(a, b, NT, preferred_element_type=F32)


def _rows(*parts):
    return jnp.concatenate(parts, axis=0)


def _qk(q, k, i, qkord):
    r0 = i * TQ
    HB = SUB // 2

    def qr(a, b):
        return q[r0 + a * HB:r0 + b * HB, :]

    def kr(a, b):
        return k[r0 + a * HB:r0 + b * HB, :]

    jobs = {
        'c': lambda: _nt(kr(0, 1), _rows(qr(0, 1), qr(2, 3))),
        'C': lambda: _nt(kr(4, 5), _rows(qr(4, 5), qr(6, 7))),
        's': lambda: _nt(qr(2, 3), _rows(kr(2, 3), kr(1, 2))),
        'S': lambda: _nt(qr(6, 7), _rows(kr(6, 7), kr(5, 6))),
        '0': lambda: _nt(_rows(qr(1, 2), qr(3, 8)), kr(0, 2)),
        '1': lambda: _nt(qr(3, 8), kr(2, 4)),
        '2': lambda: _nt(_rows(qr(5, 6), qr(7, 8)), kr(4, 6)),
        '3': lambda: _nt(qr(7, 8), kr(6, 8)),
        'm': lambda: _nt(qr(0, 8), k[0:r0, :]) if r0 > 0 else None,
    }
    res = {ch: jobs[ch]() for ch in qkord}
    co, sh, al = [res['c'], res['C']], [res['s'], res['S']], [res[t] for t in '0123']
    cot = [_rows(co[0], co[1]).T, _rows(co[1], co[0]).T]
    row = lax.broadcasted_iota(jnp.int32, (SUB, SUB), 0)
    col = lax.broadcasted_iota(jnp.int32, (SUB, SUB), 1)
    tri = col <= row
    low = lax.broadcasted_iota(jnp.int32, (HB, SUB), 1) < HB
    tiles = [[None] * (b + 1) for b in range(4)]
    for u in range(2):
        a_lo, a_hi = al[2 * u], al[2 * u + 1]
        tiles[2 * u][2 * u] = jnp.where(tri, _rows(cot[u][0:HB], a_lo[0:HB]), NEG)
        tiles[2 * u + 1][2 * u] = _rows(jnp.where(low, cot[u][HB:SUB], sh[u]), a_lo[HB:SUB])
        tiles[2 * u + 1][2 * u + 1] = jnp.where(tri, _rows(sh[u], a_hi[0:HB]), NEG)
    for b in (2, 3):
        tiles[b][0] = al[0][(b - 1) * SUB:b * SUB]
        tiles[b][1] = al[1][(b - 2) * SUB + HB:(b - 1) * SUB + HB]
    return res['m'], tiles


def _softmax(s, i):
    s_main, s_tiles = s
    r0 = i * TQ
    nb = TQ // SUB
    p_main, p_ext, ls = [], [[] for _ in range(1, nb)], []
    for b in range(nb):
        parts = ([s_main[b * SUB:(b + 1) * SUB, :]] if r0 > 0 else []) + s_tiles[b]
        sb = jnp.concatenate(parts, axis=1) if len(parts) > 1 else parts[0]
        m = jnp.max(sb, axis=1, keepdims=True)
        p = jnp.exp2(sb - m)
        nt = p.shape[1] // SUB
        tiles = [p[:, t * SUB:(t + 1) * SUB] for t in range(nt)]
        acc = None
        for t0 in range(0, nt, GRP):
            grp = tiles[t0:t0 + GRP]
            tot = grp[0]
            for g in grp[1:]:
                tot = tot + g
            acc = tot if acc is None else acc + tot
            last = t0 + len(grp) - 1
            if acc is not tiles[last]:
                tiles[last] = jnp.minimum(tiles[last], acc)
        p = jnp.concatenate(tiles, axis=1) if nt > 1 else tiles[0]
        ls.append(jnp.sum(acc, axis=1, keepdims=True))
        p_main.append(p[:, :r0 + SUB])
        for c in range(1, b + 1):
            p_ext[c - 1].append(p[:, r0 + c * SUB:r0 + (c + 1) * SUB])
    pm = jnp.concatenate(p_main, axis=0).astype(BF16)
    pe = [(jnp.concatenate(e, axis=0) if len(e) > 1 else e[0]).astype(BF16) for e in p_ext]
    return pm, pe, ls


def _pv(p, v, i):
    pm, pe, ls = p
    r0 = i * TQ
    nb = TQ // SUB
    o = jnp.dot(pm, v[0:r0 + SUB, :], preferred_element_type=F32)
    os_ = [o[b * SUB:(b + 1) * SUB] for b in range(nb)]
    for c in range(1, nb):
        oe = jnp.dot(pe[c - 1], v[r0 + c * SUB:r0 + (c + 1) * SUB, :], preferred_element_type=F32)
        for b in range(c, nb):
            os_[b] = os_[b] + oe[(b - c) * SUB:(b - c + 1) * SUB]
    return jnp.concatenate([os_[b] * _recip(ls[b]) for b in range(nb)], axis=0)


def _attn_pair(q_s, k_s, v_s, order, actions):
    sc, ctx = {}, {}

    def pair_ctx(i):
        return jnp.concatenate([ctx[(0, i)], ctx[(1, i)]], axis=1).astype(BF16)

    for tok in order.split():
        if tok[0] == 'S':
            h, i = int(tok[1]), int(tok[2])
            sc[(h, i)] = _qk(_Packed(q_s.at[h]), _Packed(k_s.at[h]), i, QKORD if (sc or ctx) else QKORD1)
        elif tok[0] == 'P':
            h, i = int(tok[1]), int(tok[2])
            ctx[(h, i)] = _pv(_softmax(sc.pop((h, i)), i), _Packed(v_s.at[h]), i)
        else:
            actions[tok[0]](int(tok[1:]), pair_ctx)


def _kernel(x_hbm, c_hbm, wq_hbm, wk_hbm, wv_hbm, wo_hbm, wr_hbm, wg_hbm, wu_hbm, wd_hbm,
            out_hbm,
            io_v, pt_v, c_v, xn_s, acc_s, mux_s, ctx_s, q_s, k_s, v_s,
            w_b, wo_v, wr_ref, wg_v, wu_v, wd_v,
            xsem, csem, w0sem, wsem, osem_w, fsem, osem,
            *, S, M, C, D, NP, FF):
    ALL = slice(None)
    xn_p, c_p = _Packed(xn_s), _Packed(c_v)
    scale = (D ** -0.5) * math.log2(math.e)

    def xcopy(b):
        rows = pl.ds(pl.multiple_of(b * XB, XB), XB)
        return pltpu.make_async_copy(x_hbm.at[0, rows, :], io_v.at[rows, :], xsem.at[b])

    def ccopy(b):
        rows = pl.ds(pl.multiple_of(b * (XB // 2), XB // 2), XB // 2)
        return pltpu.make_async_copy(c_hbm.bitcast(U32).at[0, rows, :], c_v.at[rows, :], csem.at[b])

    KR, VR, QR = slice(0, C), slice(C, 2 * C), slice(2 * C, 2 * C + M)

    def wstart(jj, sl):
        for src, rows in ((wk_hbm, KR), (wv_hbm, VR), (wq_hbm, QR)):
            pltpu.make_async_copy(src.bitcast(U32).at[:, jj, :], w_b.at[sl, rows, :], wsem.at[sl]).start()

    def wwait(sl):
        pltpu.make_async_copy(w_b.at[sl], w_b.at[sl], wsem.at[sl]).wait()

    def wocopy(t):
        heads = pl.ds(0, 2) if t == 0 else pl.ds(2, 2 * NP - 2)
        return pltpu.make_async_copy(wo_hbm.bitcast(U32).at[heads], wo_v.at[heads], osem_w.at[t])

    def fcopy(t):
        if t == 0:
            return pltpu.make_async_copy(wg_hbm, wg_v, fsem.at[0])
        if t == 1:
            return pltpu.make_async_copy(wu_hbm, wu_v, fsem.at[1])
        if t == 2:
            return pltpu.make_async_copy(wd_hbm, wd_v.at[:, 0:M], fsem.at[2])
        return pltpu.make_async_copy(wr_hbm, wr_ref, fsem.at[3])

    def ocopy(g):
        rows = pl.ds(g * OB, OB)
        return pltpu.make_async_copy(io_v.at[rows, :], out_hbm.at[0, rows, :], osem.at[g])

    def project(dst, lhs, w32, rows, mult=None):
        y = jnp.dot(lhs, _unpack_pair(w32), preferred_element_type=F32)
        if mult is not None:
            y = y * mult
        _Packed(dst.at[0])[rows, ALL] = y[:, :D]
        _Packed(dst.at[1])[rows, ALL] = y[:, D:]

    NXB = S // XB

    def w0copy(t):
        src, rows = ((wk_hbm, KR), (wv_hbm, VR), (wq_hbm, QR))[t]
        return pltpu.make_async_copy(src.bitcast(U32).at[:, 0, :], w_b.at[0, rows, :], w0sem.at[t])

    w0copy(0).start()
    ccopy(0).start()
    w0copy(1).start()
    xcopy(0).start()
    w0copy(2).start()
    for b in range(1, NXB):
        ccopy(b).start()
        xcopy(b).start()
    wocopy(0).start()
    fcopy(3).start()
    wstart(1, 1)

    def ln1(b):
        rows = pl.ds(pl.multiple_of(b * XB, XB), XB)
        xf = io_v[rows, :].astype(F32)
        mu = jnp.mean(xf, axis=1, keepdims=True)
        xc = xf - mu
        var = jnp.mean(xc * xc, axis=1, keepdims=True)
        xn = (xc * lax.rsqrt(var + 1e-5)).astype(BF16)
        xn_p[(b, XB), ALL] = xn
        acc_s[rows, :] = xc
        mux_s[rows, :] = jnp.broadcast_to(mu, (XB, 128))
        return xn

    r0 = slice(0, XB)
    w0copy(0).wait()
    ccopy(0).wait()
    project(k_s, c_p[r0, ALL], w_b[0, KR, :], r0)
    w0copy(1).wait()
    xcopy(0).wait()
    ln1(0)
    project(v_s, c_p[r0, ALL], w_b[0, VR, :], r0)
    w0copy(2).wait()
    project(q_s, xn_p[r0, ALL], w_b[0, QR, :], r0, scale)

    def first(b, carry):
        ccopy(b).wait()
        xcopy(b).wait()
        xn = ln1(b)
        prow = (b, XB)
        c = c_p[prow, ALL]
        project(k_s, c, w_b[0, KR, :], prow)
        project(v_s, c, w_b[0, VR, :], prow)
        project(q_s, xn, w_b[0, QR, :], prow, scale)
        return carry
    lax.fori_loop(1, NXB, first, 0)
    wstart(2, 0)
    wocopy(1).start()
    for t in range(3):
        fcopy(t).start()
    wocopy(0).wait()

    def step(j, carry):
        slot = j & 1

        @pl.when(j == 1)
        def _():
            wocopy(1).wait()

        wwait(1 - slot)

        @pl.when(jnp.logical_and(j >= 1, j + 2 < NP))
        def _():
            wstart(j + 2, slot)

        wo = pltpu.bitcast(wo_v[pl.ds(2 * j, 2)].reshape(D, M), BF16)

        def oproj(ii, pair_ctx):
            acc_s[ii * TQ:(ii + 1) * TQ, :] += jnp.dot(pair_ctx(ii), wo, preferred_element_type=F32)

        def rows_of(code):
            return slice((code // 10) * TQ, (code % 10 + 1) * TQ)

        _attn_pair(q_s, k_s, v_s, ORDER_MAIN, {
            'O': oproj,
            'K': lambda code, _: project(k_s, c_p[rows_of(code), ALL], w_b[1 - slot, KR, :], rows_of(code)),
            'V': lambda code, _: project(v_s, c_p[rows_of(code), ALL], w_b[1 - slot, VR, :], rows_of(code)),
            'Q': lambda code, _: project(q_s, xn_p[rows_of(code), ALL], w_b[1 - slot, QR, :], rows_of(code), scale),
        })
        return carry
    lax.fori_loop(0, NP - 1, step, 0)

    for t in range(4):
        fcopy(t).wait()
    eps = jnp.asarray(1e-5, BF16).astype(F32)

    def last_head(h, carry):
        sc = {}
        for tok in ORDER_LAST.split():
            i = int(tok[1])
            if tok[0] == 'S':
                sc[i] = _qk(_Packed(q_s.at[h]), _Packed(k_s.at[h]), i, QKORDL1 if tok == ORDER_LAST.split()[0] else QKORDL)
            else:
                _Packed(ctx_s.at[h])[slice(i * TQ, (i + 1) * TQ), ALL] = _pv(
                    _softmax(sc.pop(i), i), _Packed(v_s.at[h]), i)
        return carry
    lax.fori_loop(0, 2, last_head, 0)

    CW = M // NCH
    RW = M // RG
    wr16 = [jnp.broadcast_to(wr_ref[t * RW:(t + 1) * RW].astype(F32).reshape(1, RW), (16, RW)).astype(BF16)
            for t in range(RG)]

    def oproj_part(r0, t):
        rows = slice(r0, r0 + EB)
        cols = slice(t * CW, (t + 1) * CW)
        return (acc_s[rows, cols]
                + jnp.dot(_Packed(ctx_s.at[0])[rows, ALL], pltpu.bitcast(wo_v[2 * NP - 2, :, cols], BF16),
                           preferred_element_type=F32)
                + jnp.dot(_Packed(ctx_s.at[1])[rows, ALL], pltpu.bitcast(wo_v[2 * NP - 1, :, cols], BF16),
                           preferred_element_type=F32))

    def ln2(r0, a):
        rows = slice(r0, r0 + EB)
        acc_s[rows, :] = a
        s1 = jnp.mean(a, axis=1, keepdims=True)
        var = jnp.maximum(jnp.mean(a * a, axis=1, keepdims=True) - s1 * s1, 0.0)
        ve = _rb(_rb(var) + eps)
        den = _rb(ve * lax.rsqrt(ve))
        inv = _recip(den)
        inv = inv * (2.0 - den * inv)
        mux = mux_s[rows, :]
        c1 = (_rb(mux + s1) - mux) * inv
        c2 = mux - c1
        a = acc_s[rows, :]
        t = a * inv
        xn_p[rows, ALL] = t - jnp.concatenate([c1] * (M // 128), axis=1)
        io_v[rows, :] = ((a + t) + jnp.concatenate([c2] * (M // 128), axis=1)).astype(BF16)

    def router_part(r0, t):
        cols = slice(t * RW, (t + 1) * RW)
        return lax.dot_general(wr16[t], xn_p[slice(r0, r0 + EB), cols], NT, preferred_element_type=F32)

    neb = S // EB
    rparts = []
    for k in range(neb + RLAG):
        hp, rp = [], None
        for t in range(NCH):
            if k < neb:
                hp.append(oproj_part(k * EB, t))
            if k >= RLAG and t < RG:
                part = router_part((k - RLAG) * EB, t)[0:8, :]
                rp = part if rp is None else rp + part
        if k > 0 and k <= neb and (k * EB) % OB == 0:
            ocopy(k * EB // OB - 1).start()
        if k < neb:
            ln2(k * EB, jnp.concatenate(hp, axis=1))
        if k >= RLAG:
            rparts.append(rp)
    rrow = _rb(jnp.concatenate(rparts, axis=1))

    I32 = jnp.int32
    b16 = lax.shift_right_logical(pltpu.bitcast(rrow, I32), 16)
    rank = jnp.where(b16 >= 0x8000, 0x10000 - b16, 0x8000 + b16)
    lane = lax.broadcasted_iota(I32, rrow.shape, 1)
    key = pltpu.bitcast(rank * S + (S - 1 - lane) + 0x20000000, F32)
    k1 = jnp.max(key, axis=1, keepdims=True)
    k2 = jnp.max(jnp.where(key == k1, 0.0, key), axis=1, keepdims=True)
    i1 = (S - 1) - (pltpu.bitcast(k1, I32)[0, 0] & (S - 1))
    i2 = (S - 1) - (pltpu.bitcast(k2, I32)[0, 0] & (S - 1))
    m1 = jnp.max(jnp.where(key == k1, rrow, -jnp.inf), axis=1, keepdims=True)[0:1, :]
    m2 = jnp.max(jnp.where(key == k2, rrow, -jnp.inf), axis=1, keepdims=True)[0:1, :]
    q1 = jnp.clip(i1 >> 4, 0, S // 16 - 1)
    q2 = jnp.clip(i2 >> 4, 0, S // 16 - 1)
    g1 = pl.multiple_of(q1 * 16, 16)
    g2 = pl.multiple_of(q2 * 16, 16)

    rid = lax.broadcasted_iota(jnp.int32, (16, M), 0)

    def pick(q, i):
        blk = pltpu.bitcast(xn_s[pl.ds(pl.multiple_of(q * 8, 8), 8), :], BF16).astype(F32)
        return jnp.sum(jnp.where(rid == i - q * 16, blk, 0.0), axis=0, keepdims=True)

    xs = jnp.where(rid == 0, pick(q1, i1), pick(q2, i2))
    xsb = xs.astype(BF16)
    ocopy(0).wait()
    nch = FF // FC
    acts, y = [], None
    for t in range(nch + 1):
        if t < nch:
            cols = slice(t * FC, (t + 1) * FC)
            a = _rb(jnp.dot(xsb, wg_v[:, cols], preferred_element_type=F32))
            u = _rb(jnp.dot(xsb, wu_v[:, cols], preferred_element_type=F32))
            g = _rb(a * _rb(jax.nn.sigmoid(a)))
            acts.append((g * u).astype(BF16))
        if t > 0:
            yt = jnp.dot(acts[t - 1], wd_v[(t - 1) * FC:t * FC, 0:M], preferred_element_type=F32)
            y = yt if y is None else y + yt
    rsel = jnp.where(rid == 0, m1, m2)
    y = _rb(_rb(y) * _rb(jax.nn.sigmoid(rsel)))
    upd = _rb(xs + y)

    for k, gg in enumerate((g1, g2)):
        rows = pl.ds(gg, 16)
        hb = _rb(acc_s[rows, :] + jnp.concatenate([mux_s[rows, :]] * (M // 128), axis=1))
        val = jnp.where(rid == i1 - gg, hb + upd[0:1, :],
                        jnp.where(rid == i2 - gg, hb + upd[1:2, :], io_v[rows, :].astype(F32)))
        pt_v[k] = val.astype(BF16)

    def pcopy(g, k):
        return pltpu.make_async_copy(pt_v.at[k], out_hbm.at[0, pl.ds(g, 16), :], osem.at[k])

    for b in range(1, S // OB):
        ocopy(b).wait()
    pcopy(g1, 0).start()

    @pl.when(g2 != g1)
    def _():
        pcopy(g2, 1).start()
        pcopy(g2, 1).wait()
    pcopy(g1, 0).wait()


def _compiler_params():
    vmem = 110 * 1024 * 1024
    try:
        return pltpu.CompilerParams(vmem_limit_bytes=vmem, disable_bounds_checks=True,
                                    disable_semaphore_checks=True)
    except TypeError:
        return pltpu.CompilerParams(vmem_limit_bytes=vmem, disable_bounds_checks=True)


@jax.jit
def pallas_sequential_preLN__compressed_kv_cla__moe_arch_mod__prompt_kernel(
    A_x: jax.Array,
    A_c_kv: jax.Array,
    A_w_q: jax.Array,
    A_w_uk: jax.Array,
    A_w_uv: jax.Array,
    A_w_o: jax.Array,
    B_x: jax.Array,
    B_w_r: jax.Array,
    B_w_gate: jax.Array,
    B_w_up: jax.Array,
    B_w_down: jax.Array,
):
    _, S, M = A_x.shape
    C = A_c_kv.shape[2]
    H, D = A_w_q.shape[1], A_w_q.shape[2]
    FF = B_w_gate.shape[1]
    NP = H // 2
    any_spec = pl.BlockSpec(memory_space=pl.ANY)
    return pl.pallas_call(
        functools.partial(_kernel, S=S, M=M, C=C, D=D, NP=NP, FF=FF),
        in_specs=[
            any_spec, any_spec, any_spec, any_spec, any_spec, any_spec,
            any_spec, any_spec, any_spec, any_spec,
        ],
        out_specs=any_spec,
        out_shape=jax.ShapeDtypeStruct((1, S, M), BF16),
        scratch_shapes=[
            pltpu.VMEM((S, M), BF16),
            pltpu.VMEM((2, 16, M), BF16),
            pltpu.VMEM((S // 2, C), U32),
            pltpu.VMEM((S // 2, M), U32),
            pltpu.VMEM((S, M), F32),
            pltpu.VMEM((S, 128), F32),
            pltpu.VMEM((2, S // 2, D), U32),
            pltpu.VMEM((2, S // 2, D), U32),
            pltpu.VMEM((2, S // 2, D), U32),
            pltpu.VMEM((2, S // 2, D), U32),
            pltpu.VMEM((2, 2 * C + M, D), U32),
            pltpu.VMEM((H, D // 2, M), U32),
            pltpu.VMEM((M,), BF16),
            pltpu.VMEM((M, FF), BF16),
            pltpu.VMEM((M, FF), BF16),
            pltpu.VMEM((FF, M + 128), BF16),
            pltpu.SemaphoreType.DMA((S // XB,)),
            pltpu.SemaphoreType.DMA((S // XB,)),
            pltpu.SemaphoreType.DMA((3,)),
            pltpu.SemaphoreType.DMA((2,)),
            pltpu.SemaphoreType.DMA((2,)),
            pltpu.SemaphoreType.DMA((4,)),
            pltpu.SemaphoreType.DMA((S // OB,)),
        ],
        compiler_params=_compiler_params(),
    )(A_x, A_c_kv, A_w_q, A_w_uk, A_w_uv, A_w_o, B_w_r, B_w_gate, B_w_up, B_w_down)
```

```python
import functools
import math

import jax
import jax.numpy as jnp
from jax import lax
import jax.experimental.pallas as pl
import jax.experimental.pallas.tpu as pltpu

F32 = jnp.float32
BF16 = jnp.bfloat16
U32 = jnp.uint32
NEG = -1e30
NT = (((1,), (1,)), ((), ()))
TQ = 512
SUB = 128
GRP = 4
KB0 = 288
NK0 = 4
NXB = 4
QS = 2
EB = 128
OB = 512
NCH = 4
RG = 2
RLAG = 2
FC = 512

ORDER_MAIN = ("S03 S13 K33 P03 S02 P13 S12 P02 S01 Q23 S11 S00 P12 P01 P11 S10 K02 P00 P10 "
              "O3 O2 Q01 O1 V03 O0")
ORDER_LAST = "S3 S2 P3 S1 P2 S0 P1 P0"
QKORD, QKORD1, QKORDL, QKORDL1 = "01s2CcS3m", "01cCm2sS3", "01mS2cCs3", "Ccm2s10S3"


def _rb(v):
    return v.astype(BF16).astype(F32)


def _recip(l):
    return pl.reciprocal(l, approx=True)


def _unpack_pair(w32):
    lo = pltpu.bitcast(w32 << 16, F32)
    hi = pltpu.bitcast(w32 & jnp.uint32(0xFFFF0000), F32)
    return jnp.concatenate([lo, hi], axis=1).astype(BF16)


class _Packed:
    def __init__(self, ref):
        self.ref = ref

    @staticmethod
    def half(rows):
        if isinstance(rows, slice):
            return slice(rows.start // 2, rows.stop // 2)
        grp, size = rows
        return pl.ds(pl.multiple_of(grp * 8, 8), size // 2)

    def __getitem__(self, idx):
        rows, cols = idx
        return pltpu.bitcast(self.ref[self.half(rows), cols], BF16)

    def __setitem__(self, idx, val):
        rows, cols = idx
        self.ref[self.half(rows), cols] = pltpu.bitcast(val.astype(BF16), U32)


def _nt(a, b):
    return lax.dot_general(a, b, NT, preferred_element_type=F32)


def _rows(*parts):
    return jnp.concatenate(parts, axis=0)


def _qk(q, k, i, qkord):
    r0 = i * TQ
    HB = SUB // 2

    def qr(a, b):
        return q[r0 + a * HB:r0 + b * HB, :]

    def kr(a, b):
        return k[r0 + a * HB:r0 + b * HB, :]

    jobs = {
        'c': lambda: _nt(kr(0, 1), _rows(qr(0, 1), qr(2, 3))),
        'C': lambda: _nt(kr(4, 5), _rows(qr(4, 5), qr(6, 7))),
        's': lambda: _nt(qr(2, 3), _rows(kr(2, 3), kr(1, 2))),
        'S': lambda: _nt(qr(6, 7), _rows(kr(6, 7), kr(5, 6))),
        '0': lambda: _nt(_rows(qr(1, 2), qr(3, 8)), kr(0, 2)),
        '1': lambda: _nt(qr(3, 8), kr(2, 4)),
        '2': lambda: _nt(_rows(qr(5, 6), qr(7, 8)), kr(4, 6)),
        '3': lambda: _nt(qr(7, 8), kr(6, 8)),
        'm': lambda: _nt(qr(0, 8), k[0:r0, :]) if r0 > 0 else None,
    }
    res = {ch: jobs[ch]() for ch in qkord}
    co, sh, al = [res['c'], res['C']], [res['s'], res['S']], [res[t] for t in '0123']
    cot = [_rows(co[0], co[1]).T, _rows(co[1], co[0]).T]
    row = lax.broadcasted_iota(jnp.int32, (SUB, SUB), 0)
    col = lax.broadcasted_iota(jnp.int32, (SUB, SUB), 1)
    tri = col <= row
    low = lax.broadcasted_iota(jnp.int32, (HB, SUB), 1) < HB
    tiles = [[None] * (b + 1) for b in range(4)]
    for u in range(2):
        a_lo, a_hi = al[2 * u], al[2 * u + 1]
        tiles[2 * u][2 * u] = jnp.where(tri, _rows(cot[u][0:HB], a_lo[0:HB]), NEG)
        tiles[2 * u + 1][2 * u] = _rows(jnp.where(low, cot[u][HB:SUB], sh[u]), a_lo[HB:SUB])
        tiles[2 * u + 1][2 * u + 1] = jnp.where(tri, _rows(sh[u], a_hi[0:HB]), NEG)
    for b in (2, 3):
        tiles[b][0] = al[0][(b - 1) * SUB:b * SUB]
        tiles[b][1] = al[1][(b - 2) * SUB + HB:(b - 1) * SUB + HB]
    return res['m'], tiles


def _softmax(s, i):
    s_main, s_tiles = s
    r0 = i * TQ
    nb = TQ // SUB
    p_main, p_ext, ls = [], [[] for _ in range(1, nb)], []
    for b in range(nb):
        parts = ([s_main[b * SUB:(b + 1) * SUB, :]] if r0 > 0 else []) + s_tiles[b]
        sb = jnp.concatenate(parts, axis=1) if len(parts) > 1 else parts[0]
        m = jnp.max(sb, axis=1, keepdims=True)
        p = jnp.exp2(sb - m)
        nt = p.shape[1] // SUB
        tiles = [p[:, t * SUB:(t + 1) * SUB] for t in range(nt)]
        acc = None
        for t0 in range(0, nt, GRP):
            grp = tiles[t0:t0 + GRP]
            tot = grp[0]
            for g in grp[1:]:
                tot = tot + g
            acc = tot if acc is None else acc + tot
            last = t0 + len(grp) - 1
            if acc is not tiles[last]:
                tiles[last] = jnp.minimum(tiles[last], acc)
        p = jnp.concatenate(tiles, axis=1) if nt > 1 else tiles[0]
        ls.append(jnp.sum(acc, axis=1, keepdims=True))
        p_main.append(p[:, :r0 + SUB])
        for c in range(1, b + 1):
            p_ext[c - 1].append(p[:, r0 + c * SUB:r0 + (c + 1) * SUB])
    pm = jnp.concatenate(p_main, axis=0).astype(BF16)
    pe = [(jnp.concatenate(e, axis=0) if len(e) > 1 else e[0]).astype(BF16) for e in p_ext]
    return pm, pe, ls


def _pv(p, v, i):
    pm, pe, ls = p
    r0 = i * TQ
    nb = TQ // SUB
    o = jnp.dot(pm, v[0:r0 + SUB, :], preferred_element_type=F32)
    os_ = [o[b * SUB:(b + 1) * SUB] for b in range(nb)]
    for c in range(1, nb):
        oe = jnp.dot(pe[c - 1], v[r0 + c * SUB:r0 + (c + 1) * SUB, :], preferred_element_type=F32)
        for b in range(c, nb):
            os_[b] = os_[b] + oe[(b - c) * SUB:(b - c + 1) * SUB]
    return jnp.concatenate([os_[b] * _recip(ls[b]) for b in range(nb)], axis=0)


def _attn_pair(q_s, k_s, v_s, order, actions):
    sc, ctx = {}, {}

    def pair_ctx(i):
        return jnp.concatenate([ctx[(0, i)], ctx[(1, i)]], axis=1).astype(BF16)

    for tok in order.split():
        if tok[0] == 'S':
            h, i = int(tok[1]), int(tok[2])
            sc[(h, i)] = _qk(_Packed(q_s.at[h]), _Packed(k_s.at[h]), i, QKORD if (sc or ctx) else QKORD1)
        elif tok[0] == 'P':
            h, i = int(tok[1]), int(tok[2])
            ctx[(h, i)] = _pv(_softmax(sc.pop((h, i)), i), _Packed(v_s.at[h]), i)
        else:
            actions[tok[0]](int(tok[1:]), pair_ctx)


def _kernel(x_hbm, c_hbm, wq_hbm, wk_hbm, wv_hbm, wo_hbm, wr_hbm, wg_hbm, wu_hbm, wd_hbm,
            out_hbm,
            io_v, pt_v, c_v, xn_s, acc_s, mux_s, ctx_s, q_s, k_s, v_s,
            w_b, wo_v, wr_ref, wg_v, wu_v, wd_v,
            xsem, csem, w0sem, wsem, osem_w, fsem, osem,
            *, S, M, C, D, NP, FF):
    ALL = slice(None)
    xn_p, c_p = _Packed(xn_s), _Packed(c_v)
    scale = (D ** -0.5) * math.log2(math.e)

    XB = S // NXB
    KB = (S - NK0 * KB0) // NXB

    def cchunk0(b):
        return b * (KB0 // 16), KB0

    def cchunk(b):
        return NK0 * KB0 // 16 + b * (KB // 16), KB

    def xrows(b):
        return pl.ds(pl.multiple_of(b * XB, XB), XB)

    def xcopy(b):
        return pltpu.make_async_copy(x_hbm.at[0, xrows(b), :], io_v.at[xrows(b), :], xsem.at[b])

    def ccopy(ch, k):
        rows = _Packed.half(ch)
        return pltpu.make_async_copy(c_hbm.bitcast(U32).at[0, rows, :], c_v.at[rows, :], csem.at[k])

    KR, VR, QR = slice(0, C), slice(C, 2 * C), slice(2 * C, 2 * C + M)

    def wstart(jj, sl):
        for src, rows in ((wk_hbm, KR), (wv_hbm, VR), (wq_hbm, QR)):
            pltpu.make_async_copy(src.bitcast(U32).at[:, jj, :], w_b.at[sl, rows, :], wsem.at[sl]).start()

    def wwait(sl):
        pltpu.make_async_copy(w_b.at[sl], w_b.at[sl], wsem.at[sl]).wait()

    def wocopy(t):
        heads = pl.ds(0, 2) if t == 0 else pl.ds(2, 2 * NP - 2)
        return pltpu.make_async_copy(wo_hbm.bitcast(U32).at[heads], wo_v.at[heads], osem_w.at[t])

    def fcopy(t):
        if t == 0:
            return pltpu.make_async_copy(wg_hbm, wg_v, fsem.at[0])
        if t == 1:
            return pltpu.make_async_copy(wu_hbm, wu_v, fsem.at[1])
        if t == 2:
            return pltpu.make_async_copy(wd_hbm, wd_v.at[:, 0:M], fsem.at[2])
        return pltpu.make_async_copy(wr_hbm, wr_ref, fsem.at[3])

    def ocopy(g):
        rows = pl.ds(g * OB, OB)
        return pltpu.make_async_copy(io_v.at[rows, :], out_hbm.at[0, rows, :], osem.at[g])

    def project(dst, lhs, w32, rows, mult=None):
        y = jnp.dot(lhs, _unpack_pair(w32), preferred_element_type=F32)
        if mult is not None:
            y = y * mult
        _Packed(dst.at[0])[rows, ALL] = y[:, :D]
        _Packed(dst.at[1])[rows, ALL] = y[:, D:]

    def w0copy(t):
        src, rows = ((wk_hbm, KR), (wv_hbm, VR), (wq_hbm, QR))[t]
        return pltpu.make_async_copy(src.bitcast(U32).at[:, 0, :], w_b.at[0, rows, :], w0sem.at[t])

    w0copy(0).start()
    w0copy(1).start()
    for b in range(NK0):
        ccopy(cchunk0(b), b).start()
    w0copy(2).start()
    for b in range(NXB):
        xcopy(b).start()
        ccopy(cchunk(b), NK0 + b).start()
    wocopy(0).start()
    fcopy(3).start()
    wstart(1, 1)

    def kv(ch):
        c = c_p[ch, ALL]
        project(k_s, c, w_b[0, KR, :], ch)
        project(v_s, c, w_b[0, VR, :], ch)

    def kv_ahead(b, carry):
        ccopy(cchunk0(b), b).wait()
        kv(cchunk0(b))
        return carry
    w0copy(0).wait()
    w0copy(1).wait()
    lax.fori_loop(0, NK0, kv_ahead, 0)
    w0copy(2).wait()

    def first(b, carry):
        xcopy(b).wait()
        ccopy(cchunk(b), NK0 + b).wait()
        HQ = XB // QS
        xns = []
        for u in range(QS):
            rows = pl.ds(pl.multiple_of(b * XB + u * HQ, HQ), HQ)
            xf = io_v[rows, :].astype(F32)
            mu = jnp.mean(xf, axis=1, keepdims=True)
            xc = xf - mu
            var = jnp.mean(xc * xc, axis=1, keepdims=True)
            xn = (xc * lax.rsqrt(var + 1e-5)).astype(BF16)
            xn_p[((b * QS + u) * (HQ // 16), HQ), ALL] = xn
            acc_s[rows, :] = xc
            mux_s[rows, :] = jnp.broadcast_to(mu, (HQ, 128))
            xns.append(xn)
        kv(cchunk(b))
        for u in range(QS):
            project(q_s, xns[u], w_b[0, QR, :], ((b * QS + u) * (HQ // 16), HQ), scale)
        return carry
    lax.fori_loop(0, NXB, first, 0)
    wstart(2, 0)
    wocopy(1).start()
    for t in range(3):
        fcopy(t).start()
    wocopy(0).wait()

    def step(j, carry):
        slot = j & 1

        @pl.when(j == 1)
        def _():
            wocopy(1).wait()

        wwait(1 - slot)

        @pl.when(jnp.logical_and(j >= 1, j + 2 < NP))
        def _():
            wstart(j + 2, slot)

        wo = pltpu.bitcast(wo_v[pl.ds(2 * j, 2)].reshape(D, M), BF16)

        def oproj(ii, pair_ctx):
            acc_s[ii * TQ:(ii + 1) * TQ, :] += jnp.dot(pair_ctx(ii), wo, preferred_element_type=F32)

        def rows_of(code):
            return slice((code // 10) * TQ, (code % 10 + 1) * TQ)

        _attn_pair(q_s, k_s, v_s, ORDER_MAIN, {
            'O': oproj,
            'K': lambda code, _: project(k_s, c_p[rows_of(code), ALL], w_b[1 - slot, KR, :], rows_of(code)),
            'V': lambda code, _: project(v_s, c_p[rows_of(code), ALL], w_b[1 - slot, VR, :], rows_of(code)),
            'Q': lambda code, _: project(q_s, xn_p[rows_of(code), ALL], w_b[1 - slot, QR, :], rows_of(code), scale),
        })
        return carry
    lax.fori_loop(0, NP - 1, step, 0)

    for t in range(4):
        fcopy(t).wait()
    eps = jnp.asarray(1e-5, BF16).astype(F32)

    def last_head(h, carry):
        sc = {}
        for tok in ORDER_LAST.split():
            i = int(tok[1])
            if tok[0] == 'S':
                sc[i] = _qk(_Packed(q_s.at[h]), _Packed(k_s.at[h]), i, QKORDL1 if tok == ORDER_LAST.split()[0] else QKORDL)
            else:
                _Packed(ctx_s.at[h])[slice(i * TQ, (i + 1) * TQ), ALL] = _pv(
                    _softmax(sc.pop(i), i), _Packed(v_s.at[h]), i)
        return carry
    lax.fori_loop(0, 2, last_head, 0)

    CW = M // NCH
    RW = M // RG
    wr16 = [jnp.broadcast_to(wr_ref[t * RW:(t + 1) * RW].astype(F32).reshape(1, RW), (16, RW)).astype(BF16)
            for t in range(RG)]

    def oproj_part(r0, t):
        rows = slice(r0, r0 + EB)
        cols = slice(t * CW, (t + 1) * CW)
        return (acc_s[rows, cols]
                + jnp.dot(_Packed(ctx_s.at[0])[rows, ALL], pltpu.bitcast(wo_v[2 * NP - 2, :, cols], BF16),
                           preferred_element_type=F32)
                + jnp.dot(_Packed(ctx_s.at[1])[rows, ALL], pltpu.bitcast(wo_v[2 * NP - 1, :, cols], BF16),
                           preferred_element_type=F32))

    def ln2(r0, a):
        rows = slice(r0, r0 + EB)
        acc_s[rows, :] = a
        s1 = jnp.mean(a, axis=1, keepdims=True)
        var = jnp.maximum(jnp.mean(a * a, axis=1, keepdims=True) - s1 * s1, 0.0)
        ve = _rb(_rb(var) + eps)
        den = _rb(ve * lax.rsqrt(ve))
        inv = _recip(den)
        inv = inv * (2.0 - den * inv)
        mux = mux_s[rows, :]
        c1 = (_rb(mux + s1) - mux) * inv
        c2 = mux - c1
        a = acc_s[rows, :]
        t = a * inv
        xn_p[rows, ALL] = t - jnp.concatenate([c1] * (M // 128), axis=1)
        io_v[rows, :] = ((a + t) + jnp.concatenate([c2] * (M // 128), axis=1)).astype(BF16)

    def router_part(r0, t):
        cols = slice(t * RW, (t + 1) * RW)
        return lax.dot_general(wr16[t], xn_p[slice(r0, r0 + EB), cols], NT, preferred_element_type=F32)

    neb = S // EB
    rparts = []
    for k in range(neb + RLAG):
        hp, rp = [], None
        for t in range(NCH):
            if k < neb:
                hp.append(oproj_part(k * EB, t))
            if k >= RLAG and t < RG:
                part = router_part((k - RLAG) * EB, t)[0:8, :]
                rp = part if rp is None else rp + part
        if k > 0 and k <= neb and (k * EB) % OB == 0:
            ocopy(k * EB // OB - 1).start()
        if k < neb:
            ln2(k * EB, jnp.concatenate(hp, axis=1))
        if k >= RLAG:
            rparts.append(rp)
    rrow = _rb(jnp.concatenate(rparts, axis=1))

    I32 = jnp.int32
    b16 = lax.shift_right_logical(pltpu.bitcast(rrow, I32), 16)
    rank = jnp.where(b16 >= 0x8000, 0x10000 - b16, 0x8000 + b16)
    lane = lax.broadcasted_iota(I32, rrow.shape, 1)
    key = pltpu.bitcast(rank * S + (S - 1 - lane) + 0x20000000, F32)
    k1 = jnp.max(key, axis=1, keepdims=True)
    k2 = jnp.max(jnp.where(key == k1, 0.0, key), axis=1, keepdims=True)
    i1 = (S - 1) - (pltpu.bitcast(k1, I32)[0, 0] & (S - 1))
    i2 = (S - 1) - (pltpu.bitcast(k2, I32)[0, 0] & (S - 1))
    m1 = jnp.max(jnp.where(key == k1, rrow, -jnp.inf), axis=1, keepdims=True)[0:1, :]
    m2 = jnp.max(jnp.where(key == k2, rrow, -jnp.inf), axis=1, keepdims=True)[0:1, :]
    q1 = jnp.clip(i1 >> 4, 0, S // 16 - 1)
    q2 = jnp.clip(i2 >> 4, 0, S // 16 - 1)
    g1 = pl.multiple_of(q1 * 16, 16)
    g2 = pl.multiple_of(q2 * 16, 16)

    rid = lax.broadcasted_iota(jnp.int32, (16, M), 0)

    def pick(q, i):
        blk = pltpu.bitcast(xn_s[pl.ds(pl.multiple_of(q * 8, 8), 8), :], BF16).astype(F32)
        return jnp.sum(jnp.where(rid == i - q * 16, blk, 0.0), axis=0, keepdims=True)

    xs = jnp.where(rid == 0, pick(q1, i1), pick(q2, i2))
    xsb = xs.astype(BF16)
    ocopy(0).wait()
    nch = FF // FC
    acts, y = [], None
    for t in range(nch + 1):
        if t < nch:
            cols = slice(t * FC, (t + 1) * FC)
            a = _rb(jnp.dot(xsb, wg_v[:, cols], preferred_element_type=F32))
            u = _rb(jnp.dot(xsb, wu_v[:, cols], preferred_element_type=F32))
            g = _rb(a * _rb(jax.nn.sigmoid(a)))
            acts.append((g * u).astype(BF16))
        if t > 0:
            yt = jnp.dot(acts[t - 1], wd_v[(t - 1) * FC:t * FC, 0:M], preferred_element_type=F32)
            y = yt if y is None else y + yt
    rsel = jnp.where(rid == 0, m1, m2)
    y = _rb(_rb(y) * _rb(jax.nn.sigmoid(rsel)))
    upd = _rb(xs + y)

    for k, gg in enumerate((g1, g2)):
        rows = pl.ds(gg, 16)
        hb = _rb(acc_s[rows, :] + jnp.concatenate([mux_s[rows, :]] * (M // 128), axis=1))
        val = jnp.where(rid == i1 - gg, hb + upd[0:1, :],
                        jnp.where(rid == i2 - gg, hb + upd[1:2, :], io_v[rows, :].astype(F32)))
        pt_v[k] = val.astype(BF16)

    def pcopy(g, k):
        return pltpu.make_async_copy(pt_v.at[k], out_hbm.at[0, pl.ds(g, 16), :], osem.at[k])

    for b in range(1, S // OB):
        ocopy(b).wait()
    pcopy(g1, 0).start()

    @pl.when(g2 != g1)
    def _():
        pcopy(g2, 1).start()
        pcopy(g2, 1).wait()
    pcopy(g1, 0).wait()


def _compiler_params():
    vmem = 110 * 1024 * 1024
    try:
        return pltpu.CompilerParams(vmem_limit_bytes=vmem, disable_bounds_checks=True,
                                    disable_semaphore_checks=True)
    except TypeError:
        return pltpu.CompilerParams(vmem_limit_bytes=vmem, disable_bounds_checks=True)


@jax.jit
def pallas_sequential_preLN__compressed_kv_cla__moe_arch_mod__prompt_kernel(
    A_x: jax.Array,
    A_c_kv: jax.Array,
    A_w_q: jax.Array,
    A_w_uk: jax.Array,
    A_w_uv: jax.Array,
    A_w_o: jax.Array,
    B_x: jax.Array,
    B_w_r: jax.Array,
    B_w_gate: jax.Array,
    B_w_up: jax.Array,
    B_w_down: jax.Array,
):
    _, S, M = A_x.shape
    C = A_c_kv.shape[2]
    H, D = A_w_q.shape[1], A_w_q.shape[2]
    FF = B_w_gate.shape[1]
    NP = H // 2
    any_spec = pl.BlockSpec(memory_space=pl.ANY)
    return pl.pallas_call(
        functools.partial(_kernel, S=S, M=M, C=C, D=D, NP=NP, FF=FF),
        in_specs=[
            any_spec, any_spec, any_spec, any_spec, any_spec, any_spec,
            any_spec, any_spec, any_spec, any_spec,
        ],
        out_specs=any_spec,
        out_shape=jax.ShapeDtypeStruct((1, S, M), BF16),
        scratch_shapes=[
            pltpu.VMEM((S, M), BF16),
            pltpu.VMEM((2, 16, M), BF16),
            pltpu.VMEM((S // 2, C), U32),
            pltpu.VMEM((S // 2, M), U32),
            pltpu.VMEM((S, M), F32),
            pltpu.VMEM((S, 128), F32),
            pltpu.VMEM((2, S // 2, D), U32),
            pltpu.VMEM((2, S // 2, D), U32),
            pltpu.VMEM((2, S // 2, D), U32),
            pltpu.VMEM((2, S // 2, D), U32),
            pltpu.VMEM((2, 2 * C + M, D), U32),
            pltpu.VMEM((H, D // 2, M), U32),
            pltpu.VMEM((M,), BF16),
            pltpu.VMEM((M, FF), BF16),
            pltpu.VMEM((M, FF), BF16),
            pltpu.VMEM((FF, M + 128), BF16),
            pltpu.SemaphoreType.DMA((NXB,)),
            pltpu.SemaphoreType.DMA((NK0 + NXB,)),
            pltpu.SemaphoreType.DMA((3,)),
            pltpu.SemaphoreType.DMA((2,)),
            pltpu.SemaphoreType.DMA((2,)),
            pltpu.SemaphoreType.DMA((4,)),
            pltpu.SemaphoreType.DMA((S // OB,)),
        ],
        compiler_params=_compiler_params(),
    )(A_x, A_c_kv, A_w_q, A_w_uk, A_w_uv, A_w_o, B_w_r, B_w_gate, B_w_up, B_w_down)
```
